```python
import jax
import jax.numpy as jnp

def _softmax(x, axis=-1):
    return jax.nn.softmax(x, axis=axis)

def _gelu(x):
    return jax.nn.gelu(x, approximate=True)

def _silu(x):
    return jax.nn.silu(x)

def _sigmoid(x):
    return jax.nn.sigmoid(x)

def _layernorm(x, axis=-1, eps=1e-05):
    m = jnp.mean(x, axis=axis, keepdims=True)
    v = jnp.var(x, axis=axis, keepdims=True)
    return (x - m) / jnp.sqrt(v + eps)

def _scatter_add(tgt, idx, src, axis=0):
    return tgt.at[idx].add(src)

def _segment_sum(src, seg, n):
    return jax.ops.segment_sum(src, seg, n)

class _Rng:

    def __init__(self, key):
        self._k = key

    def _next(self):
        self._k, sub = jax.random.split(self._k)
        return sub

    def normal(self, shape):
        return jax.random.normal(self._next(), shape, dtype=jnp.bfloat16)

    def randint(self, lo, hi, shape):
        return jax.random.randint(self._next(), shape, lo, hi, dtype=jnp.int32)

    def uniform(self, shape, lo=0.0, hi=1.0):
        return jax.random.uniform(self._next(), shape, jnp.bfloat16, lo, hi)

    def permutation(self, n):
        return jax.random.permutation(self._next(), n)
kernel_name = 'concat_heads__memory_aug_recurrent_mem_tr__sliding_local_dilated__prompt'

def setup_inputs():
    _rng = _Rng(jax.random.key(int.from_bytes(__import__("os").urandom(4), "little")))
    _w = lambda a: (lambda t: t.astype(jnp.bfloat16) if jnp.issubdtype(t.dtype, jnp.floating) else t)(jnp.asarray(a))

    def _A_setup():
        B, S, Dm = (1, 2048, 1024)
        H, Dh = (32, 128)
        M, seg = (8, 32)
        seg = min(seg, S)
        S = S // seg * seg
        return {'x': _w((lambda *s: _rng.normal(s) * 0.05)(B, S, Dm)), 'mem0': _w((lambda *s: _rng.normal(s) * 0.05)(B, M, Dm)), 'Wq': _w((lambda *s: _rng.normal(s) * 0.05)(Dm, H, Dh) * Dm ** (-0.5)), 'Wk': _w((lambda *s: _rng.normal(s) * 0.05)(Dm, H, Dh) * Dm ** (-0.5)), 'Wv': _w((lambda *s: _rng.normal(s) * 0.05)(Dm, H, Dh) * Dm ** (-0.5)), 'Wo': _w((lambda *s: _rng.normal(s) * 0.05)(H, Dh, Dm) * (H * Dh) ** (-0.5)), 'seg_len': seg}
    _A_in = _A_setup()

    def _B_setup():
        B, S, D = (1, 2048, 1024)
        return {'x': _w((lambda *s: _rng.normal(s) * 0.05)(B, S, D)), 'wqkv': _w((lambda *s: _rng.normal(s) * 0.05)(D, 3 * D)), 'wo': _w((lambda *s: _rng.normal(s) * 0.05)(D, D))}
    _B_in = _B_setup()
    return {'A_x': _A_in['x'], 'A_mem0': _A_in['mem0'], 'A_Wq': _A_in['Wq'], 'A_Wk': _A_in['Wk'], 'A_Wv': _A_in['Wv'], 'A_Wo': _A_in['Wo'], 'A_seg_len': _A_in['seg_len'], 'B_x': _B_in['x'], 'B_wqkv': _B_in['wqkv'], 'B_wo': _B_in['wo']}

def reference(A_x, A_mem0, A_Wq, A_Wk, A_Wv, A_Wo, A_seg_len, B_x, B_wqkv, B_wo):

    def _A_ref(x, mem0, Wq, Wk, Wv, Wo, seg_len):
        B, S, Dm = x.shape
        H, Dh = (Wq.shape[1], Wq.shape[2])
        M = mem0.shape[1]
        scale = Dh ** (-0.5)
        n_seg = S // seg_len
        L = M + seg_len
        idx = jnp.arange(L)
        mask = (idx[:, None] < M) | (idx[:, None] >= idx[None, :])
        mem = mem0
        outs = []
        for s in range(n_seg):
            xs = x[:, s * seg_len:(s + 1) * seg_len, :].copy()
            h = jnp.concatenate([mem, xs], axis=1)
            q = jnp.einsum('btd,dhe->bhte', h, Wq)
            k = jnp.einsum('btd,dhe->bhte', h, Wk)
            v = jnp.einsum('btd,dhe->bhte', h, Wv)
            scores = jnp.einsum('bhqe,bhke->bhqk', q, k) * scale
            scores = jnp.where(mask[None, None], scores, -1000000000.0)
            p = _softmax(scores, axis=-1)
            o = jnp.einsum('bhqk,bhke->bhqe', p, v)
            o = jnp.einsum('bhte,hed->btd', o, Wo)
            mem = o[:, :M, :].copy()
            outs.append(o[:, M:, :])
        return jnp.concatenate(outs, axis=1)

    def _B_ref(x, wqkv, wo):
        B, S, D = x.shape
        H = 32
        Dh = D // H
        W, dil = (8, 2)
        qkv = (lambda x, *d: x.transpose(*d))((x @ wqkv).reshape(B, S, 3, H, Dh), 2, 0, 3, 1, 4)
        q, k, v = (qkv[0], qkv[1], qkv[2])
        scale = Dh ** (-0.5)
        pos = jnp.arange(S)
        off = jnp.arange(W) * dil
        idx = pos[:, None] - off[None, :]
        mask = idx >= 0
        idx_c = jnp.where(mask, idx, 0).reshape(-1)
        kg = k[:, :, idx_c, :].reshape(B, H, S, W, Dh)
        vg = v[:, :, idx_c, :].reshape(B, H, S, W, Dh)
        logits = jnp.einsum('bhsd,bhswd->bhsw', q, kg) * scale
        logits = jnp.where(mask[None, None, :, :], logits, -1000000000.0)
        attn = _softmax(logits, axis=-1)
        o = jnp.einsum('bhsw,bhswd->bhsd', attn, vg)
        return (lambda x, *d: x.transpose(*d))(o, 0, 2, 1, 3).reshape(B, S, D) @ wo
    a = _A_ref(A_x, A_mem0, A_Wq, A_Wk, A_Wv, A_Wo, A_seg_len)
    b = _B_ref(B_x, B_wqkv, B_wo)
    return jnp.concatenate([a, b], axis=-1)
```

```python
import functools

import jax
import jax.numpy as jnp
from jax import lax
from jax.experimental import pallas as pl
from jax.experimental.pallas import tpu as pltpu

_F32 = jnp.float32
_BF16 = jnp.bfloat16
_U32 = jnp.uint32
_NT = (((1,), (1,)), ((), ()))
_LOG2E = 1.4426950408889634
_MASKED = -1000000000.0

_B_HEADS = 32
_B_WIN = 8
_B_DIL = 2
_HALO = 16
_T = 128
_CH = 8

_D_QK = 1
_D_PV = 3
_O_CUTS = (8, 16, 24)


def _permute_b_columns(w_ref, r0, sec):
    lane = lax.broadcasted_iota(jnp.int32, (8, 128), 1)
    base = sec * 1024
    t = [w_ref[pl.ds(r0, 8), base + c * 128:base + (c + 1) * 128] for c in range(8)]
    for bit in range(3):
        s = 2 << bit
        low = (lane & s) == 0
        for c in range(8):
            if c & (1 << bit):
                continue
            lo, hi = t[c], t[c | (1 << bit)]
            t[c] = jnp.where(low, lo, pltpu.roll(hi, s, 1))
            t[c | (1 << bit)] = jnp.where(low, pltpu.roll(lo, 128 - s, 1), hi)
    for c in range(8):
        w_ref[pl.ds(r0, 8), base + c * 128:base + (c + 1) * 128] = t[c]


def _b_attention(q_ref, k_ref, v_ref, o_ref, first_block):
    scale = (1024 // _B_HEADS) ** -0.5
    lane = lax.broadcasted_iota(jnp.int32, (_CH, 128), 1)
    row = lax.broadcasted_iota(jnp.int32, (_CH, 128), 0)
    bit0 = (lane & 1) != 0
    bit4 = (lane & 16) != 0
    for r in range(0, _T, _CH):
        logits = [None] * _B_WIN
        for c in range(8):
            q = q_ref[c, r:r + _CH, :]
            for w in range(_B_WIN):
                a = _HALO + r - _B_DIL * w
                pr = q * k_ref[c, a:a + _CH, :]
                logits[w] = pr if logits[w] is None else logits[w] + pr
        for w in range(_B_WIN):
            x = logits[w]
            x = x + jnp.where(bit0, pltpu.roll(x, 1, 1), pltpu.roll(x, 127, 1))
            x = x + jnp.where(bit4, pltpu.roll(x, 16, 1), pltpu.roll(x, 112, 1))
            if first_block and r < _B_DIL * w:
                x = jnp.where(r + row >= _B_DIL * w, x, _MASKED / scale)
            logits[w] = x
        m = logits[0]
        for w in range(1, _B_WIN):
            m = jnp.maximum(m, logits[w])
        es = [jnp.exp2((x - m) * (scale * _LOG2E)) for x in logits]
        den = es[0]
        for w in range(1, _B_WIN):
            den = den + es[w]
        inv = 1.0 / den
        ps = [e * inv for e in es]
        for c in range(8):
            acc = None
            for w in range(_B_WIN):
                a = _HALO + r - _B_DIL * w
                pr = ps[w] * v_ref[c, a:a + _CH, :]
                acc = pr if acc is None else acc + pr
            o_ref[r:r + _CH, c * 128:(c + 1) * 128] = acc


def _kernel(ax_hbm, mem_hbm, wq_hbm, wk_hbm, wv_hbm, awo_hbm, bx_hbm, bw_hbm, bwo_hbm,
            out_hbm,
            xa, mem_v, wqkv, awo, xb, bw, bwo, outa, outb,
            qa, ka, va, qb, kb, vb, oa, ob, hbuf, ocat,
            sems, osems, *, seq, seg, n_mem, heads, dh):
    dm = 1024
    n_blk = seq // _T
    half = heads // 2

    bx_u = bx_hbm.bitcast(_U32)
    bw_u = bw_hbm.bitcast(_U32)
    bwo_u = bwo_hbm.bitcast(_U32)
    ax_u = ax_hbm.bitcast(_U32)
    awo_u = awo_hbm.bitcast(_U32)

    cp_xb0 = pltpu.make_async_copy(bx_u.at[0:_T // 2], xb.at[0:_T // 2], sems.at[0])
    cp_bw = [pltpu.make_async_copy(bw_u.at[:, s * dm:(s + 1) * dm],
                                   bw.at[:, s * dm:(s + 1) * dm], sems.at[1 + s])
             for s in range(3)]
    cp_xb1 = pltpu.make_async_copy(bx_u.at[_T // 2:], xb.at[_T // 2:], sems.at[4])
    cp_bwo = [pltpu.make_async_copy(bwo_u.at[:, j, :],
                                    bwo.at[(j % 8) * 8 + (j // 16) * 2 + (j // 8) % 2],
                                    sems.at[5])
              for j in range(64)]
    cp_w = [pltpu.make_async_copy(w.bitcast(_U32).at[:, par * half + j, :],
                                  wqkv.at[2 * j + par, :, m * dh:(m + 1) * dh],
                                  sems.at[6])
            for j in range(half) for par in range(2)
            for m, w in enumerate((wq_hbm, wk_hbm, wv_hbm))]
    cp_awo = pltpu.make_async_copy(awo_u, awo, sems.at[7])
    cp_xa = pltpu.make_async_copy(ax_u, xa, sems.at[8])
    cp_mem = pltpu.make_async_copy(mem_hbm, mem_v, sems.at[9])

    cp_xb0.start()
    for cp in cp_bw:
        cp.start()

    for s in range(3):
        cp_bw[s].wait()
        if s == 2:
            cp_xb1.start()
            for cp in cp_bwo:
                cp.start()

        def permute(i, carry, s=s):
            _permute_b_columns(bw, pl.multiple_of(i * 8, 8), s)
            return carry

        lax.fori_loop(0, dm // 16, permute, 0, unroll=4)

    def b_proj(r0, q_ref, k_ref, v_ref):
        x = pltpu.bitcast(xb[pl.ds(pl.multiple_of(r0 // 2, _T // 2), _T // 2), :], _BF16)
        for s, dst in enumerate((q_ref, k_ref, v_ref)):
            w = pltpu.bitcast(bw[:, s * dm:(s + 1) * dm], _BF16)
            y = jnp.dot(x, w, preferred_element_type=_F32)
            off = 0 if s == 0 else _HALO
            for c in range(8):
                dst[c, off:off + _T, :] = y[:, c * 128:(c + 1) * 128]

    def b_halo(src, dst):
        dst[:, 0:_HALO, :] = src[:, _T:_T + _HALO, :]

    def b_out(o_ref, r0):
        w = pltpu.bitcast(bwo[...].reshape(dm // 2, dm), _BF16)
        y = jnp.dot(o_ref[...], w, preferred_element_type=_F32)
        outb[pl.ds(pl.multiple_of(r0, _T), _T), :] = y.astype(_BF16)

    cp_xb0.wait()
    b_proj(0, qa, ka, va)
    ka[:, 0:_HALO, :] = jnp.broadcast_to(ka[:, _HALO:_HALO + 1, :], (8, _HALO, 128))
    va[:, 0:_HALO, :] = jnp.broadcast_to(va[:, _HALO:_HALO + 1, :], (8, _HALO, 128))

    cp_xb1.wait()
    for cp in cp_bwo:
        cp.wait()
    for cp in cp_w:
        cp.start()
    cp_awo.start()
    cp_xa.start()
    cp_mem.start()

    def b_step(r0, cur, nxt, first_block=False, last_block=False):
        if not last_block:
            b_halo(cur[1], nxt[1])
            b_halo(cur[2], nxt[2])
            b_proj(r0 + _T, nxt[0], nxt[1], nxt[2])
        _b_attention(cur[0], cur[1], cur[2], cur[3], first_block)
        b_out(cur[3], r0)

    set_a = (qa, ka, va, oa)
    set_b = (qb, kb, vb, ob)
    b_step(0, set_a, set_b, first_block=True)

    def b_body(i, carry):
        r0 = (2 * i + 1) * _T
        b_step(r0, set_b, set_a)
        b_step(r0 + _T, set_a, set_b)
        return carry

    lax.fori_loop(0, (n_blk - 2) // 2, b_body, 0)
    b_step(seq - _T, set_b, set_a, last_block=True)

    cp_outb = pltpu.make_async_copy(outb, out_hbm.at[:, dm:2 * dm], osems.at[0])
    cp_outb.start()

    for cp in cp_w:
        cp.wait()

    def split_heads(j, carry):
        even = wqkv[2 * j]
        odd = wqkv[2 * j + 1]
        wqkv[2 * j] = (even & 0xFFFF) | (odd << 16)
        wqkv[2 * j + 1] = (even >> 16) | ((odd >> 16) << 16)
        return carry

    lax.fori_loop(0, half, split_heads, 0)
    cp_awo.wait()
    cp_xa.wait()
    cp_mem.wait()

    rows = n_mem + seg
    scale = dh ** -0.5
    hbuf[0:n_mem, :] = mem_v[...].astype(_F32)

    def a_body(s, carry):
        qi = lax.broadcasted_iota(jnp.int32, (rows, 128), 0)
        ki = lax.broadcasted_iota(jnp.int32, (rows, 128), 1)
        real = ki < rows
        mask = ((qi < n_mem) | (qi >= ki)) & real
        fill = jnp.where(real, _MASKED, -jnp.inf).astype(_F32)
        pad = jnp.zeros((128 - rows, dh), _F32)

        xs = xa[pl.ds(pl.multiple_of(s * (seg // 2), seg // 2), seg // 2), :]
        hbuf[n_mem:rows, :] = pltpu.bitcast(xs, _BF16).astype(_F32)

        def project(h):
            return jnp.dot(hbuf[...], pltpu.bitcast(wqkv[h], _BF16),
                           preferred_element_type=_F32)

        def probs(qkv):
            k = jnp.concatenate([qkv[:, dh:2 * dh], pad], axis=0).astype(_BF16)
            sc = lax.dot_general(qkv[:, 0:dh], k, _NT, preferred_element_type=_F32)
            sc = jnp.where(mask, sc * scale, fill)
            e = jnp.exp(sc - jnp.max(sc, axis=-1, keepdims=True))
            return e / jnp.sum(e, axis=-1, keepdims=True)

        def values(p, qkv, h):
            v = jnp.concatenate([qkv[:, 2 * dh:3 * dh], pad], axis=0).astype(_BF16)
            ocat[:, h * dh:(h + 1) * dh] = jnp.dot(p, v, preferred_element_type=_F32)

        def out_proj(h0, h1):
            w = pltpu.bitcast(awo[h0 * dh // 2:h1 * dh // 2, :], _BF16)
            return jnp.dot(ocat[:, h0 * dh:h1 * dh], w, preferred_element_type=_F32)

        qkv, p = {}, {}
        acc, done = None, 0
        cuts = [c for c in _O_CUTS if c < heads]
        for t in range(heads + _D_PV):
            if t < heads:
                qkv[t] = project(t)
            elif cuts and cuts[0] <= t - _D_PV:
                part = out_proj(done, cuts[0])
                done = cuts.pop(0)
                acc = part if acc is None else acc + part
            if 0 <= t - _D_QK < heads:
                p[t - _D_QK] = probs(qkv[t - _D_QK])
            if 0 <= t - _D_PV < heads:
                values(p[t - _D_PV], qkv[t - _D_PV], t - _D_PV)
        for c in cuts + [heads]:
            part = out_proj(done, c)
            done = c
            acc = part if acc is None else acc + part

        hbuf[0:n_mem, :] = acc[0:n_mem]
        r0 = pl.multiple_of(s * seg, seg)
        outa[pl.ds(r0, seg), :] = acc[n_mem:rows].astype(_BF16)
        pltpu.make_async_copy(outa.at[pl.ds(r0, seg)],
                              out_hbm.at[pl.ds(r0, seg), 0:dm], osems.at[1]).start()
        return carry

    lax.fori_loop(0, seq // seg, a_body, 0)
    cp_outb.wait()
    pltpu.make_async_copy(outa, out_hbm.at[:, 0:dm], osems.at[1]).wait()


@functools.partial(jax.jit, static_argnames=("A_seg_len",))
def pallas_concat_heads__memory_aug_recurrent_mem_tr__sliding_local_dilated__prompt_kernel(
    A_x: jax.Array,
    A_mem0: jax.Array,
    A_Wq: jax.Array,
    A_Wk: jax.Array,
    A_Wv: jax.Array,
    A_Wo: jax.Array,
    A_seg_len: int,
    B_x: jax.Array,
    B_wqkv: jax.Array,
    B_wo: jax.Array,
):
    batch, seq, dm = A_x.shape
    heads, dh = A_Wq.shape[1], A_Wq.shape[2]
    n_mem = A_mem0.shape[1]
    seg = int(A_seg_len)
    assert batch == 1 and dm == 1024 and dh == 128 and heads % 8 == 0
    assert B_x.shape == (1, seq, dm) and B_wqkv.shape == (dm, 3 * dm)
    assert seg % 16 == 0 and seq % seg == 0 and n_mem % 8 == 0 and n_mem + seg <= 128
    assert seq % (2 * _T) == 0
    rows = n_mem + seg

    q_buf = pltpu.VMEM((8, _T, 128), _F32)
    kv_buf = pltpu.VMEM((8, _HALO + _T, 128), _F32)
    o_buf = pltpu.VMEM((_T, dm), _F32)
    out = pl.pallas_call(
        functools.partial(_kernel, seq=seq, seg=seg, n_mem=n_mem, heads=heads, dh=dh),
        out_shape=jax.ShapeDtypeStruct((seq, 2 * dm), _BF16),
        in_specs=[pl.BlockSpec(memory_space=pl.ANY)] * 9,
        out_specs=pl.BlockSpec(memory_space=pl.ANY),
        scratch_shapes=[
            pltpu.VMEM((seq // 2, dm), _U32),
            pltpu.VMEM((n_mem, dm), _BF16),
            pltpu.VMEM((heads, dm // 2, 3 * dh), _U32),
            pltpu.VMEM((heads * dh // 2, dm), _U32),
            pltpu.VMEM((seq // 2, dm), _U32),
            pltpu.VMEM((dm // 2, 3 * dm), _U32),
            pltpu.VMEM((64, 8, dm), _U32),
            pltpu.VMEM((seq, dm), _BF16),
            pltpu.VMEM((seq, dm), _BF16),
            q_buf, kv_buf, kv_buf, q_buf, kv_buf, kv_buf, o_buf, o_buf,
            pltpu.VMEM((rows, dm), _F32),
            pltpu.VMEM((rows, heads * dh), _F32),
            pltpu.SemaphoreType.DMA((10,)),
            pltpu.SemaphoreType.DMA((2,)),
        ],
        compiler_params=pltpu.CompilerParams(vmem_limit_bytes=110 * 1024 * 1024),
    )(
        A_x.reshape(seq, dm),
        A_mem0.reshape(n_mem, dm),
        A_Wq.reshape(dm // 2, 2 * heads, dh),
        A_Wk.reshape(dm // 2, 2 * heads, dh),
        A_Wv.reshape(dm // 2, 2 * heads, dh),
        A_Wo.reshape(heads * dh, dm),
        B_x.reshape(seq, dm),
        B_wqkv,
        B_wo.reshape(8, dm // 8, dm),
    )
    return out.reshape(1, seq, 2 * dm)
```

```python
import functools

import jax
import jax.numpy as jnp
from jax import lax
from jax.experimental import pallas as pl
from jax.experimental.pallas import tpu as pltpu

_F32 = jnp.float32
_BF16 = jnp.bfloat16
_U32 = jnp.uint32
_NT = (((1,), (1,)), ((), ()))
_LOG2E = 1.4426950408889634
_MASKED = -1000000000.0

_B_HEADS = 32
_B_WIN = 8
_B_DIL = 2
_HALO = 16
_T = 128
_CH = 8

_D_QK = 1
_D_PV = 3
_O_CUTS = (8, 16, 24)


def _permute_b_columns(src_ref, dst_ref, sec):
    field = (lax.broadcasted_iota(jnp.int32, (8, 128), 1) >> 1) & 7
    bits = [(field & (1 << b)) != 0 for b in range(3)]
    base = sec * 1024
    for r in range(0, src_ref.shape[0], 8):
        t = [src_ref[r:r + 8, base + c * 128:base + (c + 1) * 128] for c in range(8)]
        t = [t[c] if c == 0 else pltpu.roll(t[c], 2 * c, 1) for c in range(8)]
        t = [t[-c % 8] for c in range(8)]
        for b in range(3):
            t = [jnp.where(bits[b], t[(c - (1 << b)) % 8], t[c]) for c in range(8)]
        for c in range(8):
            y = t[c] if c == 0 else pltpu.roll(t[c], 128 - 2 * c, 1)
            dst_ref[r:r + 8, c * 128:(c + 1) * 128] = y


def _b_attention(q_ref, k_ref, v_ref, o_ref, first_block):
    scale = (1024 // _B_HEADS) ** -0.5
    lane = lax.broadcasted_iota(jnp.int32, (_CH, 128), 1)
    row = lax.broadcasted_iota(jnp.int32, (_CH, 128), 0)
    bit0 = (lane & 1) != 0
    bit4 = (lane & 16) != 0
    for r in range(0, _T, _CH):
        logits = [None] * _B_WIN
        for c in range(8):
            q = q_ref[c, r:r + _CH, :]
            for w in range(_B_WIN):
                a = _HALO + r - _B_DIL * w
                pr = q * k_ref[c, a:a + _CH, :]
                logits[w] = pr if logits[w] is None else logits[w] + pr
        for w in range(_B_WIN):
            x = logits[w]
            x = x + jnp.where(bit0, pltpu.roll(x, 1, 1), pltpu.roll(x, 127, 1))
            x = x + jnp.where(bit4, pltpu.roll(x, 16, 1), pltpu.roll(x, 112, 1))
            if first_block and r < _B_DIL * w:
                x = jnp.where(r + row >= _B_DIL * w, x, _MASKED / scale)
            logits[w] = x
        m = logits[0]
        for w in range(1, _B_WIN):
            m = jnp.maximum(m, logits[w])
        es = [jnp.exp2((x - m) * (scale * _LOG2E)) for x in logits]
        den = es[0]
        for w in range(1, _B_WIN):
            den = den + es[w]
        inv = 1.0 / den
        ps = [e * inv for e in es]
        for c in range(8):
            acc = None
            for w in range(_B_WIN):
                a = _HALO + r - _B_DIL * w
                pr = ps[w] * v_ref[c, a:a + _CH, :]
                acc = pr if acc is None else acc + pr
            o_ref[r:r + _CH, c * 128:(c + 1) * 128] = acc


def _kernel(ax_hbm, mem_hbm, wq_hbm, wk_hbm, wv_hbm, awo_hbm, bx_hbm, bw_hbm, bwo_hbm,
            out_hbm,
            xa, mem_v, wqkv, awo, xb, bw_raw, bwq, bwk, bwv, bwo, outa, outb,
            qa, ka, va, qb, kb, vb, oa, ob, hbuf, ocat,
            sems, wsems, osems, *, seq, seg, n_mem, heads, dh):
    dm = 1024
    n_blk = seq // _T
    half = heads // 2
    bw = (bwq, bwk, bwv)

    bx_u = bx_hbm.bitcast(_U32)
    bw_u = bw_hbm.bitcast(_U32)
    bwo_u = bwo_hbm.bitcast(_U32)
    ax_u = ax_hbm.bitcast(_U32)
    awo_u = awo_hbm.bitcast(_U32)

    n_head_blk = 4
    cp_xb0 = pltpu.make_async_copy(bx_u.at[0:_T // 2], xb.at[0:_T // 2], sems.at[0])
    cp_bw = [pltpu.make_async_copy(bw_u.at[:, s * dm:(s + 1) * dm],
                                   bw_raw.at[:, s * dm:(s + 1) * dm], sems.at[1 + s])
             for s in range(3)]
    cp_xb1 = pltpu.make_async_copy(bx_u.at[_T // 2:n_head_blk * _T // 2],
                                   xb.at[_T // 2:n_head_blk * _T // 2], sems.at[4])
    cp_xb2 = pltpu.make_async_copy(bx_u.at[n_head_blk * _T // 2:],
                                   xb.at[n_head_blk * _T // 2:], sems.at[6])
    cp_bwo = [pltpu.make_async_copy(bwo_u.at[:, j, :],
                                    bwo.at[(j % 8) * 8 + (j // 16) * 2 + (j // 8) % 2],
                                    sems.at[5])
              for j in range(64)]
    cp_awo = pltpu.make_async_copy(awo_u, awo, sems.at[7])
    cp_xa = pltpu.make_async_copy(ax_u, xa, sems.at[8])
    cp_mem = pltpu.make_async_copy(mem_hbm, mem_v, sems.at[9])

    n_grp = n_blk // 2
    per_grp = half // n_grp

    def cp_w(g):
        return [pltpu.make_async_copy(
                    w.bitcast(_U32).at[:, par * half + g * per_grp + j, :],
                    wqkv.at[2 * (g * per_grp + j) + par, :, m * dh:(m + 1) * dh],
                    wsems.at[g])
                for j in range(per_grp) for par in range(2)
                for m, w in enumerate((wq_hbm, wk_hbm, wv_hbm))]

    def split_heads(g):
        for j in range(per_grp):
            h = 2 * (g * per_grp + j)
            even = wqkv[h]
            odd = wqkv[h + 1]
            wqkv[h] = (even & 0xFFFF) | (odd << 16)
            wqkv[h + 1] = (even >> 16) | ((odd >> 16) << 16)

    cp_xb0.start()
    for cp in cp_bw:
        cp.start()
    cp_xb1.start()

    def b_proj_section(r0, s, dst):
        x = pltpu.bitcast(xb[pl.ds(pl.multiple_of(r0 // 2, _T // 2), _T // 2), :], _BF16)
        y = jnp.dot(x, pltpu.bitcast(bw[s][...], _BF16), preferred_element_type=_F32)
        off = 0 if s == 0 else _HALO
        for c in range(8):
            dst[c, off:off + _T, :] = y[:, c * 128:(c + 1) * 128]

    def b_proj(r0, q_ref, k_ref, v_ref):
        for s, dst in enumerate((q_ref, k_ref, v_ref)):
            b_proj_section(r0, s, dst)

    def b_halo(src, dst):
        dst[:, 0:_HALO, :] = src[:, _T:_T + _HALO, :]

    def b_out(o_ref, r0):
        w = pltpu.bitcast(bwo[...].reshape(dm // 2, dm), _BF16)
        y = jnp.dot(o_ref[...], w, preferred_element_type=_F32)
        outb[pl.ds(pl.multiple_of(r0, _T), _T), :] = y.astype(_BF16)

    cp_bw[0].wait()
    _permute_b_columns(bw_raw, bw[0], 0)
    cp_xb0.wait()
    cp_bw[1].wait()
    for cp in cp_bwo:
        cp.start()
    b_proj_section(0, 0, qa)
    _permute_b_columns(bw_raw, bw[1], 1)
    cp_bw[2].wait()
    for cp in cp_w(0):
        cp.start()
    cp_xb2.start()
    b_proj_section(0, 1, ka)
    _permute_b_columns(bw_raw, bw[2], 2)
    b_proj_section(0, 2, va)
    ka[:, 0:_HALO, :] = jnp.broadcast_to(ka[:, _HALO:_HALO + 1, :], (8, _HALO, 128))
    va[:, 0:_HALO, :] = jnp.broadcast_to(va[:, _HALO:_HALO + 1, :], (8, _HALO, 128))

    cp_xb1.wait()
    for cp in cp_bwo:
        cp.wait()
    for cp in cp_w(1):
        cp.start()
    cp_awo.start()
    cp_xa.start()
    cp_mem.start()

    def b_step(r0, cur, nxt, first_block=False, last_block=False):
        if not last_block:
            b_halo(cur[1], nxt[1])
            b_halo(cur[2], nxt[2])
            b_proj(r0 + _T, nxt[0], nxt[1], nxt[2])
        _b_attention(cur[0], cur[1], cur[2], cur[3], first_block)
        b_out(cur[3], r0)

    set_a = (qa, ka, va, oa)
    set_b = (qb, kb, vb, ob)
    b_step(0, set_a, set_b, first_block=True)

    cp_xb2.wait()

    def b_body(i, carry):
        @pl.when(i + 2 < n_grp)
        def _():
            for cp in cp_w(i + 2):
                cp.start()

        for cp in cp_w(i):
            cp.wait()
        r0 = (2 * i + 1) * _T
        b_step(r0, set_b, set_a)
        split_heads(i)
        b_step(r0 + _T, set_a, set_b)
        return carry

    lax.fori_loop(0, n_grp - 1, b_body, 0)
    for cp in cp_w(n_grp - 1):
        cp.wait()
    b_step(seq - _T, set_b, set_a, last_block=True)
    split_heads(n_grp - 1)

    cp_outb = pltpu.make_async_copy(outb, out_hbm.at[:, dm:2 * dm], osems.at[0])
    cp_outb.start()

    cp_awo.wait()
    cp_xa.wait()
    cp_mem.wait()

    rows = n_mem + seg
    scale = dh ** -0.5
    hbuf[0:n_mem, :] = mem_v[...].astype(_F32)

    def a_body(s, carry):
        qi = lax.broadcasted_iota(jnp.int32, (rows, 128), 0)
        ki = lax.broadcasted_iota(jnp.int32, (rows, 128), 1)
        real = ki < rows
        mask = ((qi < n_mem) | (qi >= ki)) & real
        fill = jnp.where(real, _MASKED, -jnp.inf).astype(_F32)
        pad = jnp.zeros((128 - rows, dh), _F32)

        xs = xa[pl.ds(pl.multiple_of(s * (seg // 2), seg // 2), seg // 2), :]
        hbuf[n_mem:rows, :] = pltpu.bitcast(xs, _BF16).astype(_F32)

        def project(h):
            return jnp.dot(hbuf[...], pltpu.bitcast(wqkv[h], _BF16),
                           preferred_element_type=_F32)

        def probs(qkv):
            k = jnp.concatenate([qkv[:, dh:2 * dh], pad], axis=0).astype(_BF16)
            sc = lax.dot_general(qkv[:, 0:dh], k, _NT, preferred_element_type=_F32)
            sc = jnp.where(mask, sc * scale, fill)
            e = jnp.exp(sc - jnp.max(sc, axis=-1, keepdims=True))
            return e / jnp.sum(e, axis=-1, keepdims=True)

        def values(p, qkv, h):
            v = jnp.concatenate([qkv[:, 2 * dh:3 * dh], pad], axis=0).astype(_BF16)
            ocat[:, h * dh:(h + 1) * dh] = jnp.dot(p, v, preferred_element_type=_F32)

        def out_proj(h0, h1):
            w = pltpu.bitcast(awo[h0 * dh // 2:h1 * dh // 2, :], _BF16)
            return jnp.dot(ocat[:, h0 * dh:h1 * dh], w, preferred_element_type=_F32)

        qkv, p = {}, {}
        acc, done = None, 0
        cuts = [c for c in _O_CUTS if c < heads]
        for t in range(heads + _D_PV):
            if t < heads:
                qkv[t] = project(t)
            elif cuts and cuts[0] <= t - _D_PV:
                part = out_proj(done, cuts[0])
                done = cuts.pop(0)
                acc = part if acc is None else acc + part
            if 0 <= t - _D_QK < heads:
                p[t - _D_QK] = probs(qkv[t - _D_QK])
            if 0 <= t - _D_PV < heads:
                values(p[t - _D_PV], qkv[t - _D_PV], t - _D_PV)
        for c in cuts + [heads]:
            part = out_proj(done, c)
            done = c
            acc = part if acc is None else acc + part

        hbuf[0:n_mem, :] = acc[0:n_mem]
        r0 = pl.multiple_of(s * seg, seg)
        outa[pl.ds(r0, seg), :] = acc[n_mem:rows].astype(_BF16)
        pltpu.make_async_copy(outa.at[pl.ds(r0, seg)],
                              out_hbm.at[pl.ds(r0, seg), 0:dm], osems.at[1]).start()
        return carry

    lax.fori_loop(0, seq // seg, a_body, 0)
    cp_outb.wait()
    pltpu.make_async_copy(outa, out_hbm.at[:, 0:dm], osems.at[1]).wait()


@functools.partial(jax.jit, static_argnames=("A_seg_len",))
def pallas_concat_heads__memory_aug_recurrent_mem_tr__sliding_local_dilated__prompt_kernel(
    A_x: jax.Array,
    A_mem0: jax.Array,
    A_Wq: jax.Array,
    A_Wk: jax.Array,
    A_Wv: jax.Array,
    A_Wo: jax.Array,
    A_seg_len: int,
    B_x: jax.Array,
    B_wqkv: jax.Array,
    B_wo: jax.Array,
):
    batch, seq, dm = A_x.shape
    heads, dh = A_Wq.shape[1], A_Wq.shape[2]
    n_mem = A_mem0.shape[1]
    seg = int(A_seg_len)
    assert batch == 1 and dm == 1024 and dh == 128 and heads % 8 == 0
    assert B_x.shape == (1, seq, dm) and B_wqkv.shape == (dm, 3 * dm)
    assert seg % 16 == 0 and seq % seg == 0 and n_mem % 8 == 0 and n_mem + seg <= 128
    assert seq % (2 * _T) == 0 and (heads // 2) % (seq // (2 * _T)) == 0
    rows = n_mem + seg

    q_buf = pltpu.VMEM((8, _T, 128), _F32)
    kv_buf = pltpu.VMEM((8, _HALO + _T, 128), _F32)
    o_buf = pltpu.VMEM((_T, dm), _F32)
    out = pl.pallas_call(
        functools.partial(_kernel, seq=seq, seg=seg, n_mem=n_mem, heads=heads, dh=dh),
        out_shape=jax.ShapeDtypeStruct((seq, 2 * dm), _BF16),
        in_specs=[pl.BlockSpec(memory_space=pl.ANY)] * 9,
        out_specs=pl.BlockSpec(memory_space=pl.ANY),
        scratch_shapes=[
            pltpu.VMEM((seq // 2, dm), _U32),
            pltpu.VMEM((n_mem, dm), _BF16),
            pltpu.VMEM((heads, dm // 2, 3 * dh), _U32),
            pltpu.VMEM((heads * dh // 2, dm), _U32),
            pltpu.VMEM((seq // 2, dm), _U32),
            pltpu.VMEM((dm // 2, 3 * dm), _U32),
            pltpu.VMEM((dm // 2, dm), _U32),
            pltpu.VMEM((dm // 2, dm), _U32),
            pltpu.VMEM((dm // 2, dm), _U32),
            pltpu.VMEM((64, 8, dm), _U32),
            pltpu.VMEM((seq, dm), _BF16),
            pltpu.VMEM((seq, dm), _BF16),
            q_buf, kv_buf, kv_buf, q_buf, kv_buf, kv_buf, o_buf, o_buf,
            pltpu.VMEM((rows, dm), _F32),
            pltpu.VMEM((rows, heads * dh), _F32),
            pltpu.SemaphoreType.DMA((10,)),
            pltpu.SemaphoreType.DMA((seq // (2 * _T),)),
            pltpu.SemaphoreType.DMA((2,)),
        ],
        compiler_params=pltpu.CompilerParams(vmem_limit_bytes=110 * 1024 * 1024),
    )(
        A_x.reshape(seq, dm),
        A_mem0.reshape(n_mem, dm),
        A_Wq.reshape(dm // 2, 2 * heads, dh),
        A_Wk.reshape(dm // 2, 2 * heads, dh),
        A_Wv.reshape(dm // 2, 2 * heads, dh),
        A_Wo.reshape(heads * dh, dm),
        B_x.reshape(seq, dm),
        B_wqkv,
        B_wo.reshape(8, dm // 8, dm),
    )
    return out.reshape(1, seq, 2 * dm)
```

```python
import functools

import jax
import jax.numpy as jnp
from jax import lax
from jax.experimental import pallas as pl
from jax.experimental.pallas import tpu as pltpu

_F32 = jnp.float32
_BF16 = jnp.bfloat16
_U32 = jnp.uint32
_NT = (((1,), (1,)), ((), ()))
_LOG2E = 1.4426950408889634
_MASKED = -1000000000.0

_B_HEADS = 32
_B_WIN = 8
_B_DIL = 2
_HALO = 16
_T = 128
_SPAN = 0.85
_CH = 8

_D_QK = 1
_D_PV = 3
_O_CUTS = (8, 16, 24)


def _permute_b_columns(src_ref, dst_ref, sec):
    rows, lag = 16, 2
    field = (lax.broadcasted_iota(jnp.int32, (rows, 128), 1) >> 1) & 7
    bits = [(field & (1 << b)) != 0 for b in range(3)]
    base = sec * 1024

    def spread(r):
        t = [src_ref[r:r + rows, base + c * 128:base + (c + 1) * 128] for c in range(8)]
        return [t[c] if c == 0 else pltpu.roll(t[c], 2 * c, 1) for c in range(8)]

    def exchange(t):
        t = [t[-c % 8] for c in range(8)]
        for b in range(3):
            t = [jnp.where(bits[b], t[(c - (1 << b)) % 8], t[c]) for c in range(8)]
        return [t[c] if c == 0 else pltpu.roll(t[c], 128 - 2 * c, 1) for c in range(8)]

    n = src_ref.shape[0] // rows
    first, second = {}, {}
    for i in range(n + 2 * lag):
        if i < n:
            first[i] = spread(i * rows)
        if 0 <= i - lag < n:
            second[i - lag] = exchange(first.pop(i - lag))
        if 0 <= i - 2 * lag < n:
            r = (i - 2 * lag) * rows
            for c, y in enumerate(second.pop(i - 2 * lag)):
                dst_ref[r:r + rows, c * 128:(c + 1) * 128] = y


def _b_logits(q_ref, k_ref, r, first_block, never):
    scale = (1024 // _B_HEADS) ** -0.5
    lane = lax.broadcasted_iota(jnp.int32, (_CH, 128), 1)
    row = lax.broadcasted_iota(jnp.int32, (_CH, 128), 0)
    bit0 = (lane & 1) != 0
    bit4 = (lane & 16) != 0
    logits = [None] * _B_WIN
    for c in range(8):
        q = q_ref[c, r:r + _CH, :]
        if never is not None:
            q = jnp.where(never, 0.0, q)
        for w in range(_B_WIN):
            a = _HALO + r - _B_DIL * w
            pr = q * k_ref[c, a:a + _CH, :]
            logits[w] = pr if logits[w] is None else logits[w] + pr
    for w in range(_B_WIN):
        x = logits[w]
        x = x + jnp.where(bit0, pltpu.roll(x, 1, 1), pltpu.roll(x, 127, 1))
        x = x + jnp.where(bit4, pltpu.roll(x, 16, 1), pltpu.roll(x, 112, 1))
        if first_block and r < _B_DIL * w:
            x = jnp.where(r + row >= _B_DIL * w, x, _MASKED / scale)
        logits[w] = x
    return logits


def _b_values(logits, v_ref, o_ref, r):
    scale = (1024 // _B_HEADS) ** -0.5
    m = logits[0]
    for w in range(1, _B_WIN):
        m = jnp.maximum(m, logits[w])
    es = [jnp.exp2((x - m) * (scale * _LOG2E)) for x in logits]
    den = es[0]
    for w in range(1, _B_WIN):
        den = den + es[w]
    inv = 1.0 / den
    ps = [e * inv for e in es]
    for c in range(8):
        acc = None
        for w in range(_B_WIN):
            a = _HALO + r - _B_DIL * w
            pr = ps[w] * v_ref[c, a:a + _CH, :]
            acc = pr if acc is None else acc + pr
        o_ref[r:r + _CH, c * 128:(c + 1) * 128] = acc


def _paced(zero_ref, mxu_jobs, *vpu_streams, span=1.0):
    jobs = [((i + 1.0) / len(mxu_jobs), 0, f) for i, f in enumerate(mxu_jobs)]
    jobs += [(span * (i + 0.5) / len(s), 1, f)
             for s in vpu_streams for i, f in enumerate(s)]
    never = None
    for _, is_vpu, f in sorted(jobs, key=lambda j: j[:2]):
        if is_vpu:
            f(never)
        else:
            y = pltpu.bitcast(f()[-8:, :], _U32)
            never = (y & zero_ref[...]) != 0


def _kernel(ax_hbm, mem_hbm, wq_hbm, wk_hbm, wv_hbm, awo_hbm, bx_hbm, bw_hbm, bwo_hbm,
            out_hbm,
            xa, mem_v, wqkv, awo, xb, bw_raw, bwq, bwk, bwv, bwo, outa, outb,
            qa, ka, va, qb, kb, vb, oa, ob, hbuf, ocat, zero,
            sems, wsems, osems, *, seq, seg, n_mem, heads, dh):
    dm = 1024
    n_blk = seq // _T
    half = heads // 2
    bw = (bwq, bwk, bwv)

    bx_u = bx_hbm.bitcast(_U32)
    bw_u = bw_hbm.bitcast(_U32)
    bwo_u = bwo_hbm.bitcast(_U32)
    ax_u = ax_hbm.bitcast(_U32)
    awo_u = awo_hbm.bitcast(_U32)

    n_head_blk = 4
    cp_xb0 = pltpu.make_async_copy(bx_u.at[0:_T // 2], xb.at[0:_T // 2], sems.at[0])
    cp_bw = [pltpu.make_async_copy(bw_u.at[:, s * dm:(s + 1) * dm],
                                   bw_raw.at[:, s * dm:(s + 1) * dm], sems.at[1 + s])
             for s in range(3)]
    cp_xb1 = pltpu.make_async_copy(bx_u.at[_T // 2:n_head_blk * _T // 2],
                                   xb.at[_T // 2:n_head_blk * _T // 2], sems.at[4])
    cp_xb2 = pltpu.make_async_copy(bx_u.at[n_head_blk * _T // 2:],
                                   xb.at[n_head_blk * _T // 2:], sems.at[6])
    cp_bwo = [pltpu.make_async_copy(bwo_u.at[:, j, :],
                                    bwo.at[(j % 8) * 8 + (j // 16) * 2 + (j // 8) % 2],
                                    sems.at[5])
              for j in range(64)]
    cp_awo = pltpu.make_async_copy(awo_u, awo, sems.at[7])
    cp_xa = pltpu.make_async_copy(ax_u, xa, sems.at[8])
    cp_mem = pltpu.make_async_copy(mem_hbm, mem_v, sems.at[9])

    n_grp = n_blk // 2
    per_grp = half // n_grp

    def cp_w(g):
        return [pltpu.make_async_copy(
                    w.bitcast(_U32).at[:, par * half + g * per_grp + j, :],
                    wqkv.at[2 * (g * per_grp + j) + par, :, m * dh:(m + 1) * dh],
                    wsems.at[g])
                for j in range(per_grp) for par in range(2)
                for m, w in enumerate((wq_hbm, wk_hbm, wv_hbm))]

    def split_heads(g):
        def job(j, r, never):
            h = 2 * (g * per_grp + j)
            low = jnp.full((8, 128), 0xFFFF, _U32)
            sh = jnp.full((8, 128), 16, _U32)
            if never is not None:
                low = jnp.where(never, sh, low)
                sh = jnp.where(never, low, sh)
            for rr in range(r, r + 32, 8):
                for m in range(3):
                    even = wqkv[h, rr:rr + 8, m * dh:(m + 1) * dh]
                    odd = wqkv[h + 1, rr:rr + 8, m * dh:(m + 1) * dh]
                    wqkv[h, rr:rr + 8, m * dh:(m + 1) * dh] = (even & low) | (odd << sh)
                    wqkv[h + 1, rr:rr + 8, m * dh:(m + 1) * dh] = (
                        (even >> sh) | ((odd >> sh) << sh))
        return [functools.partial(job, j, r)
                for j in range(per_grp) for r in range(0, dm // 2, 32)]

    cp_xb0.start()
    zero[...] = jnp.zeros(zero.shape, _U32)
    for cp in cp_bw:
        cp.start()
    cp_xb1.start()

    def b_proj(r0, s, dst):
        def job(c):
            x = xb[pl.ds(pl.multiple_of(r0 // 2, _T // 2), _T // 2), :]
            w = bw[s][:, c * 128:(c + 1) * 128]
            off = 0 if s == 0 else _HALO
            y = jnp.dot(pltpu.bitcast(x, _BF16), pltpu.bitcast(w, _BF16),
                        preferred_element_type=_F32)
            dst[c, off:off + _T, :] = y
            return y
        return [functools.partial(job, c) for c in range(8)]

    def b_halo(src, dst):
        dst[:, 0:_HALO, :] = src[:, _T:_T + _HALO, :]

    def b_out(o_ref, r0):
        def job(c):
            w = bwo[:, :, c * 128:(c + 1) * 128].reshape(dm // 2, 128)
            y = jnp.dot(o_ref[...], pltpu.bitcast(w, _BF16), preferred_element_type=_F32)
            outb[pl.ds(pl.multiple_of(r0, _T), _T), c * 128:(c + 1) * 128] = y.astype(_BF16)
            return y
        return [functools.partial(job, c) for c in range(8)]

    def b_attention(bufs, first_block):
        pending = {}

        def logits(r, never):
            pending[r] = _b_logits(bufs[0], bufs[1], r, first_block, never)

        def values(r, never):
            _b_values(pending.pop(r), bufs[2], bufs[3], r)

        starts = list(range(0, _T, _CH))
        jobs = []
        for i in range(len(starts) + 1):
            if i < len(starts):
                jobs.append(functools.partial(logits, starts[i]))
            if i >= 1:
                jobs.append(functools.partial(values, starts[i - 1]))
        return jobs

    cp_bw[0].wait()
    _permute_b_columns(bw_raw, bw[0], 0)
    cp_xb0.wait()
    cp_bw[1].wait()
    for cp in cp_bwo:
        cp.start()
    _paced(zero, b_proj(0, 0, qa))
    _permute_b_columns(bw_raw, bw[1], 1)
    cp_bw[2].wait()
    for cp in cp_w(0):
        cp.start()
    cp_xb2.start()
    _paced(zero, b_proj(0, 1, ka))
    _permute_b_columns(bw_raw, bw[2], 2)
    _paced(zero, b_proj(0, 2, va))
    ka[:, 0:_HALO, :] = jnp.broadcast_to(ka[:, _HALO:_HALO + 1, :], (8, _HALO, 128))
    va[:, 0:_HALO, :] = jnp.broadcast_to(va[:, _HALO:_HALO + 1, :], (8, _HALO, 128))

    cp_xb1.wait()
    for cp in cp_bwo:
        cp.wait()
    for cp in cp_w(1):
        cp.start()
    cp_awo.start()
    cp_xa.start()
    cp_mem.start()

    def b_step(r0, cur, nxt, extra=(), first_block=False, last_block=False):
        mxu = []
        if not first_block:
            mxu += b_out(nxt[3], r0 - _T)
        if not last_block:
            b_halo(cur[1], nxt[1])
            b_halo(cur[2], nxt[2])
            for s in range(3):
                mxu += b_proj(r0 + _T, s, nxt[s])
        _paced(zero, mxu, b_attention(cur, first_block), list(extra), span=_SPAN)

    set_a = (qa, ka, va, oa)
    set_b = (qb, kb, vb, ob)
    b_step(0, set_a, set_b, first_block=True)

    cp_xb2.wait()

    def b_body(i, carry):
        @pl.when(i + 2 < n_grp)
        def _():
            for cp in cp_w(i + 2):
                cp.start()

        for cp in cp_w(i):
            cp.wait()
        r0 = (2 * i + 1) * _T
        split = split_heads(i)
        b_step(r0, set_b, set_a, split[:len(split) // 2])
        b_step(r0 + _T, set_a, set_b, split[len(split) // 2:])
        return carry

    lax.fori_loop(0, n_grp - 1, b_body, 0)
    for cp in cp_w(n_grp - 1):
        cp.wait()
    b_step(seq - _T, set_b, set_a, split_heads(n_grp - 1), last_block=True)
    _paced(zero, b_out(ob, seq - _T))

    cp_outb = pltpu.make_async_copy(outb, out_hbm.at[:, dm:2 * dm], osems.at[0])
    cp_outb.start()

    cp_awo.wait()
    cp_xa.wait()
    cp_mem.wait()

    rows = n_mem + seg
    scale = dh ** -0.5
    hbuf[0:n_mem, :] = mem_v[...].astype(_F32)

    def a_body(s, carry):
        qi = lax.broadcasted_iota(jnp.int32, (rows, 128), 0)
        ki = lax.broadcasted_iota(jnp.int32, (rows, 128), 1)
        real = ki < rows
        mask = ((qi < n_mem) | (qi >= ki)) & real
        fill = jnp.where(real, _MASKED, -jnp.inf).astype(_F32)
        pad = jnp.zeros((128 - rows, dh), _F32)

        xs = xa[pl.ds(pl.multiple_of(s * (seg // 2), seg // 2), seg // 2), :]
        hbuf[n_mem:rows, :] = pltpu.bitcast(xs, _BF16).astype(_F32)

        def project(h):
            return jnp.dot(hbuf[...], pltpu.bitcast(wqkv[h], _BF16),
                           preferred_element_type=_F32)

        def probs(qkv):
            k = jnp.concatenate([qkv[:, dh:2 * dh], pad], axis=0).astype(_BF16)
            sc = lax.dot_general(qkv[:, 0:dh], k, _NT, preferred_element_type=_F32)
            sc = jnp.where(mask, sc * scale, fill)
            e = jnp.exp(sc - jnp.max(sc, axis=-1, keepdims=True))
            return e / jnp.sum(e, axis=-1, keepdims=True)

        def values(p, qkv, h):
            v = jnp.concatenate([qkv[:, 2 * dh:3 * dh], pad], axis=0).astype(_BF16)
            ocat[:, h * dh:(h + 1) * dh] = jnp.dot(p, v, preferred_element_type=_F32)

        def out_proj(h0, h1):
            w = pltpu.bitcast(awo[h0 * dh // 2:h1 * dh // 2, :], _BF16)
            return jnp.dot(ocat[:, h0 * dh:h1 * dh], w, preferred_element_type=_F32)

        qkv, p = {}, {}
        acc, done = None, 0
        cuts = [c for c in _O_CUTS if c < heads]
        for t in range(heads + _D_PV):
            if t < heads:
                qkv[t] = project(t)
            elif cuts and cuts[0] <= t - _D_PV:
                part = out_proj(done, cuts[0])
                done = cuts.pop(0)
                acc = part if acc is None else acc + part
            if 0 <= t - _D_QK < heads:
                p[t - _D_QK] = probs(qkv[t - _D_QK])
            if 0 <= t - _D_PV < heads:
                values(p[t - _D_PV], qkv[t - _D_PV], t - _D_PV)
        for c in cuts + [heads]:
            part = out_proj(done, c)
            done = c
            acc = part if acc is None else acc + part

        hbuf[0:n_mem, :] = acc[0:n_mem]
        r0 = pl.multiple_of(s * seg, seg)
        outa[pl.ds(r0, seg), :] = acc[n_mem:rows].astype(_BF16)
        pltpu.make_async_copy(outa.at[pl.ds(r0, seg)],
                              out_hbm.at[pl.ds(r0, seg), 0:dm], osems.at[1]).start()
        return carry

    lax.fori_loop(0, seq // seg, a_body, 0)
    cp_outb.wait()
    pltpu.make_async_copy(outa, out_hbm.at[:, 0:dm], osems.at[1]).wait()


@functools.partial(jax.jit, static_argnames=("A_seg_len",))
def pallas_concat_heads__memory_aug_recurrent_mem_tr__sliding_local_dilated__prompt_kernel(
    A_x: jax.Array,
    A_mem0: jax.Array,
    A_Wq: jax.Array,
    A_Wk: jax.Array,
    A_Wv: jax.Array,
    A_Wo: jax.Array,
    A_seg_len: int,
    B_x: jax.Array,
    B_wqkv: jax.Array,
    B_wo: jax.Array,
):
    batch, seq, dm = A_x.shape
    heads, dh = A_Wq.shape[1], A_Wq.shape[2]
    n_mem = A_mem0.shape[1]
    seg = int(A_seg_len)
    assert batch == 1 and dm == 1024 and dh == 128 and heads % 8 == 0
    assert B_x.shape == (1, seq, dm) and B_wqkv.shape == (dm, 3 * dm)
    assert seg % 16 == 0 and seq % seg == 0 and n_mem % 8 == 0 and n_mem + seg <= 128
    assert seq % (2 * _T) == 0 and (heads // 2) % (seq // (2 * _T)) == 0
    rows = n_mem + seg

    q_buf = pltpu.VMEM((8, _T, 128), _F32)
    kv_buf = pltpu.VMEM((8, _HALO + _T, 128), _F32)
    o_buf = pltpu.VMEM((_T, dm), _F32)
    out = pl.pallas_call(
        functools.partial(_kernel, seq=seq, seg=seg, n_mem=n_mem, heads=heads, dh=dh),
        out_shape=jax.ShapeDtypeStruct((seq, 2 * dm), _BF16),
        in_specs=[pl.BlockSpec(memory_space=pl.ANY)] * 9,
        out_specs=pl.BlockSpec(memory_space=pl.ANY),
        scratch_shapes=[
            pltpu.VMEM((seq // 2, dm), _U32),
            pltpu.VMEM((n_mem, dm), _BF16),
            pltpu.VMEM((heads, dm // 2, 3 * dh), _U32),
            pltpu.VMEM((heads * dh // 2, dm), _U32),
            pltpu.VMEM((seq // 2, dm), _U32),
            pltpu.VMEM((dm // 2, 3 * dm), _U32),
            pltpu.VMEM((dm // 2, dm), _U32),
            pltpu.VMEM((dm // 2, dm), _U32),
            pltpu.VMEM((dm // 2, dm), _U32),
            pltpu.VMEM((64, 8, dm), _U32),
            pltpu.VMEM((seq, dm), _BF16),
            pltpu.VMEM((seq, dm), _BF16),
            q_buf, kv_buf, kv_buf, q_buf, kv_buf, kv_buf, o_buf, o_buf,
            pltpu.VMEM((rows, dm), _F32),
            pltpu.VMEM((rows, heads * dh), _F32),
            pltpu.VMEM((8, 128), _U32),
            pltpu.SemaphoreType.DMA((10,)),
            pltpu.SemaphoreType.DMA((seq // (2 * _T),)),
            pltpu.SemaphoreType.DMA((2,)),
        ],
        compiler_params=pltpu.CompilerParams(vmem_limit_bytes=110 * 1024 * 1024),
    )(
        A_x.reshape(seq, dm),
        A_mem0.reshape(n_mem, dm),
        A_Wq.reshape(dm // 2, 2 * heads, dh),
        A_Wk.reshape(dm // 2, 2 * heads, dh),
        A_Wv.reshape(dm // 2, 2 * heads, dh),
        A_Wo.reshape(heads * dh, dm),
        B_x.reshape(seq, dm),
        B_wqkv,
        B_wo.reshape(8, dm // 8, dm),
    )
    return out.reshape(1, seq, 2 * dm)
```

```python
import functools

import jax
import jax.numpy as jnp
from jax import lax
from jax.experimental import pallas as pl
from jax.experimental.pallas import tpu as pltpu

_F32 = jnp.float32
_BF16 = jnp.bfloat16
_U32 = jnp.uint32
_NT = (((1,), (1,)), ((), ()))
_LOG2E = 1.4426950408889634
_MASKED = -1000000000.0

_B_HEADS = 32
_B_WIN = 8
_B_DIL = 2
_HALO = 16
_T = 128
_SPAN = 0.85
_CH = 8

_D_QK = 1
_D_PV = 3
_O_CUTS = (8, 16, 24)


def _permute_b_columns(src_ref, dst_ref, sec):
    rows, lag = 16, 2
    field = (lax.broadcasted_iota(jnp.int32, (rows, 128), 1) >> 1) & 7
    bits = [(field & (1 << b)) != 0 for b in range(3)]
    base = sec * 1024

    def spread(r):
        t = [src_ref[r:r + rows, base + c * 128:base + (c + 1) * 128] for c in range(8)]
        return [t[c] if c == 0 else pltpu.roll(t[c], 2 * c, 1) for c in range(8)]

    def exchange(t):
        t = [t[-c % 8] for c in range(8)]
        for b in range(3):
            t = [jnp.where(bits[b], t[(c - (1 << b)) % 8], t[c]) for c in range(8)]
        return [t[c] if c == 0 else pltpu.roll(t[c], 128 - 2 * c, 1) for c in range(8)]

    n = src_ref.shape[0] // rows
    first, second = {}, {}
    for i in range(n + 2 * lag):
        if i < n:
            first[i] = spread(i * rows)
        if 0 <= i - lag < n:
            second[i - lag] = exchange(first.pop(i - lag))
        if 0 <= i - 2 * lag < n:
            r = (i - 2 * lag) * rows
            for c, y in enumerate(second.pop(i - 2 * lag)):
                dst_ref[r:r + rows, c * 128:(c + 1) * 128] = y


def _b_logits(q_ref, k_ref, r, first_block, never):
    scale = (1024 // _B_HEADS) ** -0.5
    lane = lax.broadcasted_iota(jnp.int32, (_CH, 128), 1)
    row = lax.broadcasted_iota(jnp.int32, (_CH, 128), 0)
    bit0 = (lane & 1) != 0
    bit4 = (lane & 16) != 0
    logits = [None] * _B_WIN
    for c in range(8):
        q = q_ref[c, r:r + _CH, :]
        if never is not None:
            q = jnp.where(never, 0.0, q)
        for w in range(_B_WIN):
            a = _HALO + r - _B_DIL * w
            pr = q * k_ref[c, a:a + _CH, :]
            logits[w] = pr if logits[w] is None else logits[w] + pr
    for w in range(_B_WIN):
        x = logits[w]
        x = x + jnp.where(bit0, pltpu.roll(x, 1, 1), pltpu.roll(x, 127, 1))
        x = x + jnp.where(bit4, pltpu.roll(x, 16, 1), pltpu.roll(x, 112, 1))
        if first_block and r < _B_DIL * w:
            x = jnp.where(r + row >= _B_DIL * w, x, _MASKED / scale)
        logits[w] = x
    return logits


def _b_values(logits, v_ref, o_ref, r):
    scale = (1024 // _B_HEADS) ** -0.5
    m = logits[0]
    for w in range(1, _B_WIN):
        m = jnp.maximum(m, logits[w])
    es = [jnp.exp2((x - m) * (scale * _LOG2E)) for x in logits]
    den = es[0]
    for w in range(1, _B_WIN):
        den = den + es[w]
    inv = 1.0 / den
    ps = [e * inv for e in es]
    for c in range(8):
        acc = None
        for w in range(_B_WIN):
            a = _HALO + r - _B_DIL * w
            pr = ps[w] * v_ref[c, a:a + _CH, :]
            acc = pr if acc is None else acc + pr
        o_ref[r:r + _CH, c * 128:(c + 1) * 128] = acc


def _paced(zero_ref, mxu_jobs, *vpu_streams, span=1.0):
    jobs = [((i + 1.0) / len(mxu_jobs), 0, f) for i, f in enumerate(mxu_jobs)]
    jobs += [(span * (i + 0.5) / len(s), 1, f)
             for s in vpu_streams for i, f in enumerate(s)]
    never = None
    for _, is_vpu, f in sorted(jobs, key=lambda j: j[:2]):
        if is_vpu:
            f(never)
        else:
            y = pltpu.bitcast(f()[-8:, :], _U32)
            never = (y & zero_ref[...]) != 0


def _kernel(ax_hbm, mem_hbm, wq_hbm, wk_hbm, wv_hbm, awo_hbm, bx_hbm, bw_hbm, bwo_hbm,
            out_hbm,
            xa, mem_v, wqkv, awo, xb, bw_raw, bwq, bwk, bwv, bwo, outa, outb,
            qa, ka, va, qb, kb, vb, oa, ob, hbuf, ocat, zero,
            sems, wsems, xsems, osems, *, seq, seg, n_mem, heads, dh):
    dm = 1024
    n_blk = seq // _T
    half = heads // 2
    bw = (bwq, bwk, bwv)

    bx_u = bx_hbm.bitcast(_U32)
    bw_u = bw_hbm.bitcast(_U32)
    bwo_u = bwo_hbm.bitcast(_U32)
    ax_u = ax_hbm.bitcast(_U32)
    awo_u = awo_hbm.bitcast(_U32)


    def cp_xb(g):
        rows = pl.ds(pl.multiple_of(g * _T, _T), _T)
        return pltpu.make_async_copy(bx_u.at[rows], xb.at[rows], xsems.at[g])

    cp_bw = [pltpu.make_async_copy(bw_u.at[:, s * dm:(s + 1) * dm],
                                   bw_raw.at[:, s * dm:(s + 1) * dm], sems.at[1 + s])
             for s in range(3)]
    cp_bwo = [pltpu.make_async_copy(bwo_u.at[:, j, :],
                                    bwo.at[(j % 8) * 8 + (j // 16) * 2 + (j // 8) % 2],
                                    sems.at[5])
              for j in range(64)]
    cp_mem = pltpu.make_async_copy(mem_hbm, mem_v, sems.at[9])

    n_grp = n_blk // 2
    per_grp = half // n_grp

    def cp_w(g):
        return [pltpu.make_async_copy(
                    w.bitcast(_U32).at[:, par * half + g * per_grp + j, :],
                    wqkv.at[2 * (g * per_grp + j) + par, :, m * dh:(m + 1) * dh],
                    wsems.at[g])
                for j in range(per_grp) for par in range(2)
                for m, w in enumerate((wq_hbm, wk_hbm, wv_hbm))]

    def start_a_slice(g):
        for src_ref, dst_ref, sem in ((awo_u, awo, sems.at[7]), (ax_u, xa, sems.at[8])):
            n = dst_ref.shape[0] // n_grp
            rows = pl.ds(pl.multiple_of(g * n, n), n)
            pltpu.make_async_copy(src_ref.at[rows], dst_ref.at[rows], sem).start()

    def split_heads(g):
        def job(j, r, never):
            h = 2 * (g * per_grp + j)
            low = jnp.full((8, 128), 0xFFFF, _U32)
            sh = jnp.full((8, 128), 16, _U32)
            if never is not None:
                low = jnp.where(never, sh, low)
                sh = jnp.where(never, low, sh)
            for rr in range(r, r + 32, 8):
                for m in range(3):
                    even = wqkv[h, rr:rr + 8, m * dh:(m + 1) * dh]
                    odd = wqkv[h + 1, rr:rr + 8, m * dh:(m + 1) * dh]
                    wqkv[h, rr:rr + 8, m * dh:(m + 1) * dh] = (even & low) | (odd << sh)
                    wqkv[h + 1, rr:rr + 8, m * dh:(m + 1) * dh] = (
                        (even >> sh) | ((odd >> sh) << sh))
        return [functools.partial(job, j, r)
                for j in range(per_grp) for r in range(0, dm // 2, 32)]

    cp_xb(0).start()
    zero[...] = jnp.zeros(zero.shape, _U32)
    for cp in cp_bw:
        cp.start()

    def b_proj(r0, s, dst):
        def job(c):
            x = xb[pl.ds(pl.multiple_of(r0 // 2, _T // 2), _T // 2), :]
            w = bw[s][:, c * 128:(c + 1) * 128]
            off = 0 if s == 0 else _HALO
            y = jnp.dot(pltpu.bitcast(x, _BF16), pltpu.bitcast(w, _BF16),
                        preferred_element_type=_F32)
            dst[c, off:off + _T, :] = y
            return y
        return [functools.partial(job, c) for c in range(8)]

    def b_halo(src, dst):
        dst[:, 0:_HALO, :] = src[:, _T:_T + _HALO, :]

    def b_out(o_ref, r0):
        def job(c):
            w = bwo[:, :, c * 128:(c + 1) * 128].reshape(dm // 2, 128)
            y = jnp.dot(o_ref[...], pltpu.bitcast(w, _BF16), preferred_element_type=_F32)
            outb[pl.ds(pl.multiple_of(r0, _T), _T), c * 128:(c + 1) * 128] = y.astype(_BF16)
            return y
        return [functools.partial(job, c) for c in range(8)]

    def b_attention(bufs, first_block):
        pending = {}

        def logits(r, never):
            pending[r] = _b_logits(bufs[0], bufs[1], r, first_block, never)

        def values(r, never):
            _b_values(pending.pop(r), bufs[2], bufs[3], r)

        starts = list(range(0, _T, _CH))
        jobs = []
        for i in range(len(starts) + 1):
            if i < len(starts):
                jobs.append(functools.partial(logits, starts[i]))
            if i >= 1:
                jobs.append(functools.partial(values, starts[i - 1]))
        return jobs

    cp_bw[0].wait()
    _permute_b_columns(bw_raw, bw[0], 0)
    cp_xb(0).wait()
    cp_bw[1].wait()
    for cp in cp_bwo:
        cp.start()
    cp_xb(1).start()
    _paced(zero, b_proj(0, 0, qa))
    _permute_b_columns(bw_raw, bw[1], 1)
    cp_bw[2].wait()
    for cp in cp_w(0):
        cp.start()
    _paced(zero, b_proj(0, 1, ka))
    _permute_b_columns(bw_raw, bw[2], 2)
    _paced(zero, b_proj(0, 2, va))
    ka[:, 0:_HALO, :] = jnp.broadcast_to(ka[:, _HALO:_HALO + 1, :], (8, _HALO, 128))
    va[:, 0:_HALO, :] = jnp.broadcast_to(va[:, _HALO:_HALO + 1, :], (8, _HALO, 128))

    for cp in cp_bwo:
        cp.wait()
    for cp in cp_w(1):
        cp.start()
    cp_xb(2).start()
    cp_mem.start()

    def b_step(r0, cur, nxt, extra=(), first_block=False, last_block=False):
        mxu = []
        if not first_block:
            mxu += b_out(nxt[3], r0 - _T)
        if not last_block:
            b_halo(cur[1], nxt[1])
            b_halo(cur[2], nxt[2])
            for s in range(3):
                mxu += b_proj(r0 + _T, s, nxt[s])
        _paced(zero, mxu, b_attention(cur, first_block), list(extra), span=_SPAN)

    set_a = (qa, ka, va, oa)
    set_b = (qb, kb, vb, ob)
    b_step(0, set_a, set_b, first_block=True)

    def b_body(i, carry):
        @pl.when(i + 2 < n_grp)
        def _():
            for cp in cp_w(i + 2):
                cp.start()

        @pl.when(i + 3 < n_grp)
        def _():
            cp_xb(i + 3).start()

        start_a_slice(i)
        cp_xb(i + 1).wait()
        for cp in cp_w(i):
            cp.wait()
        r0 = (2 * i + 1) * _T
        split = split_heads(i)
        b_step(r0, set_b, set_a, split[:len(split) // 2])
        b_step(r0 + _T, set_a, set_b, split[len(split) // 2:])
        return carry

    lax.fori_loop(0, n_grp - 1, b_body, 0)
    start_a_slice(n_grp - 1)
    for cp in cp_w(n_grp - 1):
        cp.wait()
    b_step(seq - _T, set_b, set_a, split_heads(n_grp - 1), last_block=True)
    _paced(zero, b_out(ob, seq - _T))

    cp_outb = pltpu.make_async_copy(outb, out_hbm.at[:, dm:2 * dm], osems.at[0])
    cp_outb.start()

    pltpu.make_async_copy(awo_u, awo, sems.at[7]).wait()
    pltpu.make_async_copy(ax_u, xa, sems.at[8]).wait()
    cp_mem.wait()

    rows = n_mem + seg
    scale = dh ** -0.5
    hbuf[0:n_mem, :] = mem_v[...].astype(_F32)

    def a_body(s, carry):
        qi = lax.broadcasted_iota(jnp.int32, (rows, 128), 0)
        ki = lax.broadcasted_iota(jnp.int32, (rows, 128), 1)
        real = ki < rows
        mask = ((qi < n_mem) | (qi >= ki)) & real
        fill = jnp.where(real, _MASKED, -jnp.inf).astype(_F32)
        pad = jnp.zeros((128 - rows, dh), _F32)

        xs = xa[pl.ds(pl.multiple_of(s * (seg // 2), seg // 2), seg // 2), :]
        hbuf[n_mem:rows, :] = pltpu.bitcast(xs, _BF16).astype(_F32)

        def project(h):
            return jnp.dot(hbuf[...], pltpu.bitcast(wqkv[h], _BF16),
                           preferred_element_type=_F32)

        def probs(qkv):
            k = jnp.concatenate([qkv[:, dh:2 * dh], pad], axis=0).astype(_BF16)
            sc = lax.dot_general(qkv[:, 0:dh], k, _NT, preferred_element_type=_F32)
            sc = jnp.where(mask, sc * scale, fill)
            e = jnp.exp(sc - jnp.max(sc, axis=-1, keepdims=True))
            return e / jnp.sum(e, axis=-1, keepdims=True)

        def values(p, qkv, h):
            v = jnp.concatenate([qkv[:, 2 * dh:3 * dh], pad], axis=0).astype(_BF16)
            ocat[:, h * dh:(h + 1) * dh] = jnp.dot(p, v, preferred_element_type=_F32)

        def out_proj(h0, h1):
            w = pltpu.bitcast(awo[h0 * dh // 2:h1 * dh // 2, :], _BF16)
            return jnp.dot(ocat[:, h0 * dh:h1 * dh], w, preferred_element_type=_F32)

        qkv, p = {}, {}
        acc, done = None, 0
        cuts = [c for c in _O_CUTS if c < heads]
        for t in range(heads + _D_PV):
            if t < heads:
                qkv[t] = project(t)
            elif cuts and cuts[0] <= t - _D_PV:
                part = out_proj(done, cuts[0])
                done = cuts.pop(0)
                acc = part if acc is None else acc + part
            if 0 <= t - _D_QK < heads:
                p[t - _D_QK] = probs(qkv[t - _D_QK])
            if 0 <= t - _D_PV < heads:
                values(p[t - _D_PV], qkv[t - _D_PV], t - _D_PV)
        for c in cuts + [heads]:
            part = out_proj(done, c)
            done = c
            acc = part if acc is None else acc + part

        hbuf[0:n_mem, :] = acc[0:n_mem]
        r0 = pl.multiple_of(s * seg, seg)
        outa[pl.ds(r0, seg), :] = acc[n_mem:rows].astype(_BF16)
        pltpu.make_async_copy(outa.at[pl.ds(r0, seg)],
                              out_hbm.at[pl.ds(r0, seg), 0:dm], osems.at[1]).start()
        return carry

    lax.fori_loop(0, seq // seg, a_body, 0)
    cp_outb.wait()
    pltpu.make_async_copy(outa, out_hbm.at[:, 0:dm], osems.at[1]).wait()


@functools.partial(jax.jit, static_argnames=("A_seg_len",))
def pallas_concat_heads__memory_aug_recurrent_mem_tr__sliding_local_dilated__prompt_kernel(
    A_x: jax.Array,
    A_mem0: jax.Array,
    A_Wq: jax.Array,
    A_Wk: jax.Array,
    A_Wv: jax.Array,
    A_Wo: jax.Array,
    A_seg_len: int,
    B_x: jax.Array,
    B_wqkv: jax.Array,
    B_wo: jax.Array,
):
    batch, seq, dm = A_x.shape
    heads, dh = A_Wq.shape[1], A_Wq.shape[2]
    n_mem = A_mem0.shape[1]
    seg = int(A_seg_len)
    assert batch == 1 and dm == 1024 and dh == 128 and heads % 8 == 0
    assert B_x.shape == (1, seq, dm) and B_wqkv.shape == (dm, 3 * dm)
    assert seg % 16 == 0 and seq % seg == 0 and n_mem % 8 == 0 and n_mem + seg <= 128
    assert seq % (2 * _T) == 0 and (heads // 2) % (seq // (2 * _T)) == 0
    rows = n_mem + seg

    q_buf = pltpu.VMEM((8, _T, 128), _F32)
    kv_buf = pltpu.VMEM((8, _HALO + _T, 128), _F32)
    o_buf = pltpu.VMEM((_T, dm), _F32)
    out = pl.pallas_call(
        functools.partial(_kernel, seq=seq, seg=seg, n_mem=n_mem, heads=heads, dh=dh),
        out_shape=jax.ShapeDtypeStruct((seq, 2 * dm), _BF16),
        in_specs=[pl.BlockSpec(memory_space=pl.ANY)] * 9,
        out_specs=pl.BlockSpec(memory_space=pl.ANY),
        scratch_shapes=[
            pltpu.VMEM((seq // 2, dm), _U32),
            pltpu.VMEM((n_mem, dm), _BF16),
            pltpu.VMEM((heads, dm // 2, 3 * dh), _U32),
            pltpu.VMEM((heads * dh // 2, dm), _U32),
            pltpu.VMEM((seq // 2, dm), _U32),
            pltpu.VMEM((dm // 2, 3 * dm), _U32),
            pltpu.VMEM((dm // 2, dm), _U32),
            pltpu.VMEM((dm // 2, dm), _U32),
            pltpu.VMEM((dm // 2, dm), _U32),
            pltpu.VMEM((64, 8, dm), _U32),
            pltpu.VMEM((seq, dm), _BF16),
            pltpu.VMEM((seq, dm), _BF16),
            q_buf, kv_buf, kv_buf, q_buf, kv_buf, kv_buf, o_buf, o_buf,
            pltpu.VMEM((rows, dm), _F32),
            pltpu.VMEM((rows, heads * dh), _F32),
            pltpu.VMEM((8, 128), _U32),
            pltpu.SemaphoreType.DMA((10,)),
            pltpu.SemaphoreType.DMA((seq // (2 * _T),)),
            pltpu.SemaphoreType.DMA((seq // (2 * _T),)),
            pltpu.SemaphoreType.DMA((2,)),
        ],
        compiler_params=pltpu.CompilerParams(vmem_limit_bytes=110 * 1024 * 1024),
    )(
        A_x.reshape(seq, dm),
        A_mem0.reshape(n_mem, dm),
        A_Wq.reshape(dm // 2, 2 * heads, dh),
        A_Wk.reshape(dm // 2, 2 * heads, dh),
        A_Wv.reshape(dm // 2, 2 * heads, dh),
        A_Wo.reshape(heads * dh, dm),
        B_x.reshape(seq, dm),
        B_wqkv,
        B_wo.reshape(8, dm // 8, dm),
    )
    return out.reshape(1, seq, 2 * dm)
```

```python
import functools

import jax
import jax.numpy as jnp
from jax import lax
from jax.experimental import pallas as pl
from jax.experimental.pallas import tpu as pltpu

_F32 = jnp.float32
_BF16 = jnp.bfloat16
_U32 = jnp.uint32
_NT = (((1,), (1,)), ((), ()))
_LOG2E = 1.4426950408889634
_MASKED = -1000000000.0

_B_HEADS = 32
_B_WIN = 8
_B_DIL = 2
_HALO = 16
_T = 128
_SPAN = 0.85
_CH = 8

_A_UNROLL = 2


def _permute_b_columns(src_ref, dst_ref, sec):
    rows, lag = 16, 2
    field = (lax.broadcasted_iota(jnp.int32, (rows, 128), 1) >> 1) & 7
    bits = [(field & (1 << b)) != 0 for b in range(3)]
    base = sec * 1024

    def spread(r):
        t = [src_ref[r:r + rows, base + c * 128:base + (c + 1) * 128] for c in range(8)]
        return [t[c] if c == 0 else pltpu.roll(t[c], 2 * c, 1) for c in range(8)]

    def exchange(t):
        t = [t[-c % 8] for c in range(8)]
        for b in range(3):
            t = [jnp.where(bits[b], t[(c - (1 << b)) % 8], t[c]) for c in range(8)]
        return [t[c] if c == 0 else pltpu.roll(t[c], 128 - 2 * c, 1) for c in range(8)]

    n = src_ref.shape[0] // rows
    first, second = {}, {}
    for i in range(n + 2 * lag):
        if i < n:
            first[i] = spread(i * rows)
        if 0 <= i - lag < n:
            second[i - lag] = exchange(first.pop(i - lag))
        if 0 <= i - 2 * lag < n:
            r = (i - 2 * lag) * rows
            for c, y in enumerate(second.pop(i - 2 * lag)):
                dst_ref[r:r + rows, c * 128:(c + 1) * 128] = y


def _b_logits(q_ref, k_ref, r, first_block, never):
    scale = (1024 // _B_HEADS) ** -0.5
    lane = lax.broadcasted_iota(jnp.int32, (_CH, 128), 1)
    row = lax.broadcasted_iota(jnp.int32, (_CH, 128), 0)
    bit0 = (lane & 1) != 0
    bit4 = (lane & 16) != 0
    logits = [None] * _B_WIN
    for c in range(8):
        q = q_ref[c, r:r + _CH, :]
        if never is not None:
            q = jnp.where(never, 0.0, q)
        for w in range(_B_WIN):
            a = _HALO + r - _B_DIL * w
            pr = q * k_ref[c, a:a + _CH, :]
            logits[w] = pr if logits[w] is None else logits[w] + pr
    for w in range(_B_WIN):
        x = logits[w]
        x = x + jnp.where(bit0, pltpu.roll(x, 1, 1), pltpu.roll(x, 127, 1))
        x = x + jnp.where(bit4, pltpu.roll(x, 16, 1), pltpu.roll(x, 112, 1))
        if first_block and r < _B_DIL * w:
            x = jnp.where(r + row >= _B_DIL * w, x, _MASKED / scale)
        logits[w] = x
    return logits


def _b_values(logits, v_ref, o_ref, r):
    scale = (1024 // _B_HEADS) ** -0.5
    m = logits[0]
    for w in range(1, _B_WIN):
        m = jnp.maximum(m, logits[w])
    es = [jnp.exp2((x - m) * (scale * _LOG2E)) for x in logits]
    den = es[0]
    for w in range(1, _B_WIN):
        den = den + es[w]
    inv = 1.0 / den
    ps = [e * inv for e in es]
    for c in range(8):
        acc = None
        for w in range(_B_WIN):
            a = _HALO + r - _B_DIL * w
            pr = ps[w] * v_ref[c, a:a + _CH, :]
            acc = pr if acc is None else acc + pr
        o_ref[r:r + _CH, c * 128:(c + 1) * 128] = acc


def _paced(zero_ref, mxu_jobs, *vpu_streams, span=1.0):
    jobs = [((i + 1.0) / len(mxu_jobs), 0, f) for i, f in enumerate(mxu_jobs)]
    jobs += [(span * (i + 0.5) / len(s), 1, f)
             for s in vpu_streams for i, f in enumerate(s)]
    never = None
    for _, is_vpu, f in sorted(jobs, key=lambda j: j[:2]):
        if is_vpu:
            f(never)
        else:
            y = pltpu.bitcast(f()[-8:, :], _U32)
            never = (y & zero_ref[...]) != 0


def _kernel(ax_hbm, mem_hbm, wq_hbm, wk_hbm, wv_hbm, awo_hbm, bx_hbm, bw_hbm, bwo_hbm,
            out_hbm,
            xa, mem_v, wqkv, awo, xb, bw_raw, bwq, bwk, bwv, bwo, outa, outb,
            qa, ka, va, qb, kb, vb, oa, ob, hbuf, zero,
            sems, wsems, xsems, osems, *, seq, seg, n_mem, heads, dh):
    dm = 1024
    n_blk = seq // _T
    half = heads // 2
    bw = (bwq, bwk, bwv)

    bx_u = bx_hbm.bitcast(_U32)
    bw_u = bw_hbm.bitcast(_U32)
    bwo_u = bwo_hbm.bitcast(_U32)
    ax_u = ax_hbm.bitcast(_U32)
    awo_u = awo_hbm.bitcast(_U32)


    def cp_xb(g):
        rows = pl.ds(pl.multiple_of(g * _T, _T), _T)
        return pltpu.make_async_copy(bx_u.at[rows], xb.at[rows], xsems.at[g])

    cp_bw = [pltpu.make_async_copy(bw_u.at[:, s * dm:(s + 1) * dm],
                                   bw_raw.at[:, s * dm:(s + 1) * dm], sems.at[1 + s])
             for s in range(3)]
    cp_bwo = [pltpu.make_async_copy(bwo_u.at[:, j, :],
                                    bwo.at[(j % 8) * 8 + (j // 16) * 2 + (j // 8) % 2],
                                    sems.at[5])
              for j in range(64)]
    cp_mem = pltpu.make_async_copy(mem_hbm, mem_v, sems.at[9])

    n_grp = n_blk // 2
    per_grp = half // n_grp

    def cp_w(g):
        return [pltpu.make_async_copy(
                    w.bitcast(_U32).at[:, par * half + g * per_grp + j, :],
                    wqkv.at[2 * (g * per_grp + j) + par, :, m * dh:(m + 1) * dh],
                    wsems.at[g])
                for j in range(per_grp) for par in range(2)
                for m, w in enumerate((wq_hbm, wk_hbm, wv_hbm))]

    def start_a_slice(g):
        for src_ref, dst_ref, sem in ((awo_u, awo, sems.at[7]), (ax_u, xa, sems.at[8])):
            n = dst_ref.shape[0] // n_grp
            rows = pl.ds(pl.multiple_of(g * n, n), n)
            pltpu.make_async_copy(src_ref.at[rows], dst_ref.at[rows], sem).start()

    def split_heads(g):
        def job(j, r, never):
            h = 2 * (g * per_grp + j)
            low = jnp.full((8, 128), 0xFFFF, _U32)
            sh = jnp.full((8, 128), 16, _U32)
            if never is not None:
                low = jnp.where(never, sh, low)
                sh = jnp.where(never, low, sh)
            for rr in range(r, r + 32, 8):
                for m in range(3):
                    even = wqkv[h, rr:rr + 8, m * dh:(m + 1) * dh]
                    odd = wqkv[h + 1, rr:rr + 8, m * dh:(m + 1) * dh]
                    wqkv[h, rr:rr + 8, m * dh:(m + 1) * dh] = (even & low) | (odd << sh)
                    wqkv[h + 1, rr:rr + 8, m * dh:(m + 1) * dh] = (
                        (even >> sh) | ((odd >> sh) << sh))
        return [functools.partial(job, j, r)
                for j in range(per_grp) for r in range(0, dm // 2, 32)]

    cp_xb(0).start()
    zero[...] = jnp.zeros(zero.shape, _U32)
    for cp in cp_bw:
        cp.start()

    def b_proj(r0, s, dst):
        def job(c):
            x = xb[pl.ds(pl.multiple_of(r0 // 2, _T // 2), _T // 2), :]
            w = bw[s][:, c * 128:(c + 1) * 128]
            off = 0 if s == 0 else _HALO
            y = jnp.dot(pltpu.bitcast(x, _BF16), pltpu.bitcast(w, _BF16),
                        preferred_element_type=_F32)
            dst[c, off:off + _T, :] = y
            return y
        return [functools.partial(job, c) for c in range(8)]

    def b_halo(src, dst):
        dst[:, 0:_HALO, :] = src[:, _T:_T + _HALO, :]

    def b_out(o_ref, r0):
        def job(c):
            w = bwo[:, :, c * 128:(c + 1) * 128].reshape(dm // 2, 128)
            y = jnp.dot(o_ref[...], pltpu.bitcast(w, _BF16), preferred_element_type=_F32)
            outb[pl.ds(pl.multiple_of(r0, _T), _T), c * 128:(c + 1) * 128] = y.astype(_BF16)
            return y
        return [functools.partial(job, c) for c in range(8)]

    def b_attention(bufs, first_block):
        pending = {}

        def logits(r, never):
            pending[r] = _b_logits(bufs[0], bufs[1], r, first_block, never)

        def values(r, never):
            _b_values(pending.pop(r), bufs[2], bufs[3], r)

        starts = list(range(0, _T, _CH))
        jobs = []
        for i in range(len(starts) + 1):
            if i < len(starts):
                jobs.append(functools.partial(logits, starts[i]))
            if i >= 1:
                jobs.append(functools.partial(values, starts[i - 1]))
        return jobs

    cp_bw[0].wait()
    _permute_b_columns(bw_raw, bw[0], 0)
    cp_xb(0).wait()
    cp_bw[1].wait()
    for cp in cp_bwo:
        cp.start()
    cp_xb(1).start()
    _paced(zero, b_proj(0, 0, qa))
    _permute_b_columns(bw_raw, bw[1], 1)
    cp_bw[2].wait()
    for cp in cp_w(0):
        cp.start()
    _paced(zero, b_proj(0, 1, ka))
    _permute_b_columns(bw_raw, bw[2], 2)
    _paced(zero, b_proj(0, 2, va))
    ka[:, 0:_HALO, :] = jnp.broadcast_to(ka[:, _HALO:_HALO + 1, :], (8, _HALO, 128))
    va[:, 0:_HALO, :] = jnp.broadcast_to(va[:, _HALO:_HALO + 1, :], (8, _HALO, 128))

    for cp in cp_bwo:
        cp.wait()
    for cp in cp_w(1):
        cp.start()
    cp_xb(2).start()
    cp_mem.start()

    def b_step(r0, cur, nxt, extra=(), first_block=False, last_block=False):
        mxu = []
        if not first_block:
            mxu += b_out(nxt[3], r0 - _T)
        if not last_block:
            b_halo(cur[1], nxt[1])
            b_halo(cur[2], nxt[2])
            for s in range(3):
                mxu += b_proj(r0 + _T, s, nxt[s])
        _paced(zero, mxu, b_attention(cur, first_block), list(extra), span=_SPAN)

    set_a = (qa, ka, va, oa)
    set_b = (qb, kb, vb, ob)
    b_step(0, set_a, set_b, first_block=True)

    def b_body(i, carry):
        @pl.when(i + 2 < n_grp)
        def _():
            for cp in cp_w(i + 2):
                cp.start()

        @pl.when(i + 3 < n_grp)
        def _():
            cp_xb(i + 3).start()

        start_a_slice(i)
        cp_xb(i + 1).wait()
        for cp in cp_w(i):
            cp.wait()
        r0 = (2 * i + 1) * _T
        split = split_heads(i)
        b_step(r0, set_b, set_a, split[:len(split) // 2])
        b_step(r0 + _T, set_a, set_b, split[len(split) // 2:])
        return carry

    lax.fori_loop(0, n_grp - 1, b_body, 0)
    start_a_slice(n_grp - 1)
    for cp in cp_w(n_grp - 1):
        cp.wait()
    b_step(seq - _T, set_b, set_a, split_heads(n_grp - 1), last_block=True)
    _paced(zero, b_out(ob, seq - _T))

    cp_outb = pltpu.make_async_copy(outb, out_hbm.at[:, dm:2 * dm], osems.at[0])
    cp_outb.start()

    pltpu.make_async_copy(awo_u, awo, sems.at[7]).wait()
    pltpu.make_async_copy(ax_u, xa, sems.at[8]).wait()
    cp_mem.wait()

    rows = n_mem + seg
    scale = dh ** -0.5
    hbuf[0:n_mem, :] = mem_v[...].astype(_F32)

    def a_step(s):
        qi = lax.broadcasted_iota(jnp.int32, (rows, 128), 0)
        ki = lax.broadcasted_iota(jnp.int32, (rows, 128), 1)
        real = ki < rows
        mask = ((qi < n_mem) | (qi >= ki)) & real
        fill = jnp.where(real, _MASKED, -jnp.inf).astype(_F32)
        pad = jnp.zeros((128 - rows, dh), _F32)

        xs = xa[pl.ds(pl.multiple_of(s * (seg // 2), seg // 2), seg // 2), :]
        hbuf[n_mem:rows, :] = pltpu.bitcast(xs, _BF16).astype(_F32)

        def project(h):
            return jnp.dot(hbuf[...], pltpu.bitcast(wqkv[h], _BF16),
                           preferred_element_type=_F32)

        def probs(qkv):
            k = jnp.concatenate([qkv[:, dh:2 * dh], pad], axis=0).astype(_BF16)
            sc = lax.dot_general(qkv[:, 0:dh], k, _NT, preferred_element_type=_F32)
            sc = jnp.where(mask, sc * scale, fill)
            e = jnp.exp(sc - jnp.max(sc, axis=-1, keepdims=True))
            return e / jnp.sum(e, axis=-1, keepdims=True)

        def values(p, qkv):
            v = jnp.concatenate([qkv[:, 2 * dh:3 * dh], pad], axis=0).astype(_BF16)
            return jnp.dot(p, v, preferred_element_type=_F32)

        def out_proj(g):
            h0, h1 = g * heads // 4, (g + 1) * heads // 4
            w = pltpu.bitcast(awo[h0 * dh // 2:h1 * dh // 2, :], _BF16)
            lhs = jnp.concatenate([o[h] for h in range(h0, h1)], axis=1)
            return jnp.dot(lhs, w, preferred_element_type=_F32)

        qkv, p, o = {}, {}, {}
        acc = None
        for t in range(heads + 3):
            if t < heads:
                qkv[t] = project(t)
            else:
                part = out_proj(t - heads)
                acc = part if acc is None else acc + part
            if 1 <= t <= heads:
                p[t - 1] = probs(qkv[t - 1])
            if t >= 3:
                o[t - 3] = values(p[t - 3], qkv[t - 3])
        acc = acc + out_proj(3)

        hbuf[0:n_mem, :] = acc[0:n_mem]
        outa[pl.ds(pl.multiple_of(s * seg, seg), seg), :] = acc[n_mem:rows].astype(_BF16)

    def a_body(i, carry):
        for u in range(_A_UNROLL):
            a_step(i * _A_UNROLL + u)
        n = _A_UNROLL * seg
        done = pl.ds(pl.multiple_of(i * n, n), n)
        pltpu.make_async_copy(outa.at[done], out_hbm.at[done, 0:dm], osems.at[1]).start()
        return carry

    lax.fori_loop(0, seq // (seg * _A_UNROLL), a_body, 0)
    cp_outb.wait()
    pltpu.make_async_copy(outa, out_hbm.at[:, 0:dm], osems.at[1]).wait()


@functools.partial(jax.jit, static_argnames=("A_seg_len",))
def pallas_concat_heads__memory_aug_recurrent_mem_tr__sliding_local_dilated__prompt_kernel(
    A_x: jax.Array,
    A_mem0: jax.Array,
    A_Wq: jax.Array,
    A_Wk: jax.Array,
    A_Wv: jax.Array,
    A_Wo: jax.Array,
    A_seg_len: int,
    B_x: jax.Array,
    B_wqkv: jax.Array,
    B_wo: jax.Array,
):
    batch, seq, dm = A_x.shape
    heads, dh = A_Wq.shape[1], A_Wq.shape[2]
    n_mem = A_mem0.shape[1]
    seg = int(A_seg_len)
    assert batch == 1 and dm == 1024 and dh == 128 and heads % 8 == 0
    assert B_x.shape == (1, seq, dm) and B_wqkv.shape == (dm, 3 * dm)
    assert seg % 16 == 0 and seq % (seg * _A_UNROLL) == 0 and n_mem % 8 == 0 and n_mem + seg <= 128
    assert seq % (2 * _T) == 0 and (heads // 2) % (seq // (2 * _T)) == 0
    rows = n_mem + seg

    q_buf = pltpu.VMEM((8, _T, 128), _F32)
    kv_buf = pltpu.VMEM((8, _HALO + _T, 128), _F32)
    o_buf = pltpu.VMEM((_T, dm), _F32)
    out = pl.pallas_call(
        functools.partial(_kernel, seq=seq, seg=seg, n_mem=n_mem, heads=heads, dh=dh),
        out_shape=jax.ShapeDtypeStruct((seq, 2 * dm), _BF16),
        in_specs=[pl.BlockSpec(memory_space=pl.ANY)] * 9,
        out_specs=pl.BlockSpec(memory_space=pl.ANY),
        scratch_shapes=[
            pltpu.VMEM((seq // 2, dm), _U32),
            pltpu.VMEM((n_mem, dm), _BF16),
            pltpu.VMEM((heads, dm // 2, 3 * dh), _U32),
            pltpu.VMEM((heads * dh // 2, dm), _U32),
            pltpu.VMEM((seq // 2, dm), _U32),
            pltpu.VMEM((dm // 2, 3 * dm), _U32),
            pltpu.VMEM((dm // 2, dm), _U32),
            pltpu.VMEM((dm // 2, dm), _U32),
            pltpu.VMEM((dm // 2, dm), _U32),
            pltpu.VMEM((64, 8, dm), _U32),
            pltpu.VMEM((seq, dm), _BF16),
            pltpu.VMEM((seq, dm), _BF16),
            q_buf, kv_buf, kv_buf, q_buf, kv_buf, kv_buf, o_buf, o_buf,
            pltpu.VMEM((rows, dm), _F32),
            pltpu.VMEM((8, 128), _U32),
            pltpu.SemaphoreType.DMA((10,)),
            pltpu.SemaphoreType.DMA((seq // (2 * _T),)),
            pltpu.SemaphoreType.DMA((seq // (2 * _T),)),
            pltpu.SemaphoreType.DMA((2,)),
        ],
        compiler_params=pltpu.CompilerParams(vmem_limit_bytes=110 * 1024 * 1024),
    )(
        A_x.reshape(seq, dm),
        A_mem0.reshape(n_mem, dm),
        A_Wq.reshape(dm // 2, 2 * heads, dh),
        A_Wk.reshape(dm // 2, 2 * heads, dh),
        A_Wv.reshape(dm // 2, 2 * heads, dh),
        A_Wo.reshape(heads * dh, dm),
        B_x.reshape(seq, dm),
        B_wqkv,
        B_wo.reshape(8, dm // 8, dm),
    )
    return out.reshape(1, seq, 2 * dm)
```

```python
import functools

import jax
import jax.numpy as jnp
from jax import lax
from jax.experimental import pallas as pl
from jax.experimental.pallas import tpu as pltpu

_F32 = jnp.float32
_BF16 = jnp.bfloat16
_U32 = jnp.uint32
_NT = (((1,), (1,)), ((), ()))
_LOG2E = 1.4426950408889634
_MASKED = -1000000000.0

_B_HEADS = 32
_B_WIN = 8
_B_DIL = 2
_HALO = 16
_T = 128
_SPAN = 0.85
_CH = 8

_A_UNROLL = 2


def _permute_b_columns(src_ref, dst_ref):
    rows, lag = 16, 2
    field = (lax.broadcasted_iota(jnp.int32, (rows, 128), 1) >> 1) & 7
    bits = [(field & (1 << b)) != 0 for b in range(3)]

    def spread(r):
        t = [src_ref[r:r + rows, c * 128:(c + 1) * 128] for c in range(8)]
        return [t[c] if c == 0 else pltpu.roll(t[c], 2 * c, 1) for c in range(8)]

    def exchange(t):
        t = [t[-c % 8] for c in range(8)]
        for b in range(3):
            t = [jnp.where(bits[b], t[(c - (1 << b)) % 8], t[c]) for c in range(8)]
        return [t[c] if c == 0 else pltpu.roll(t[c], 128 - 2 * c, 1) for c in range(8)]

    n = src_ref.shape[0] // rows
    first, second = {}, {}
    for i in range(n + 2 * lag):
        if i < n:
            first[i] = spread(i * rows)
        if 0 <= i - lag < n:
            second[i - lag] = exchange(first.pop(i - lag))
        if 0 <= i - 2 * lag < n:
            r = (i - 2 * lag) * rows
            for c, y in enumerate(second.pop(i - 2 * lag)):
                dst_ref[r:r + rows, c * 128:(c + 1) * 128] = y


def _b_logits(q_ref, k_ref, r, first_block, never):
    scale = (1024 // _B_HEADS) ** -0.5
    lane = lax.broadcasted_iota(jnp.int32, (_CH, 128), 1)
    row = lax.broadcasted_iota(jnp.int32, (_CH, 128), 0)
    bit0 = (lane & 1) != 0
    bit4 = (lane & 16) != 0
    logits = [None] * _B_WIN
    for c in range(8):
        q = q_ref[c, r:r + _CH, :]
        if never is not None:
            q = jnp.where(never, 0.0, q)
        for w in range(_B_WIN):
            a = _HALO + r - _B_DIL * w
            pr = q * k_ref[c, a:a + _CH, :]
            logits[w] = pr if logits[w] is None else logits[w] + pr
    for w in range(_B_WIN):
        x = logits[w]
        x = x + jnp.where(bit0, pltpu.roll(x, 1, 1), pltpu.roll(x, 127, 1))
        x = x + jnp.where(bit4, pltpu.roll(x, 16, 1), pltpu.roll(x, 112, 1))
        if first_block and r < _B_DIL * w:
            x = jnp.where(r + row >= _B_DIL * w, x, _MASKED / scale)
        logits[w] = x
    return logits


def _b_values(logits, v_ref, o_ref, r):
    scale = (1024 // _B_HEADS) ** -0.5
    m = logits[0]
    for w in range(1, _B_WIN):
        m = jnp.maximum(m, logits[w])
    es = [jnp.exp2((x - m) * (scale * _LOG2E)) for x in logits]
    den = es[0]
    for w in range(1, _B_WIN):
        den = den + es[w]
    inv = 1.0 / den
    ps = [e * inv for e in es]
    for c in range(8):
        acc = None
        for w in range(_B_WIN):
            a = _HALO + r - _B_DIL * w
            pr = ps[w] * v_ref[c, a:a + _CH, :]
            acc = pr if acc is None else acc + pr
        o_ref[r:r + _CH, c * 128:(c + 1) * 128] = acc


def _paced(zero_ref, mxu_jobs, *vpu_streams, span=1.0):
    jobs = [((i + 1.0) / len(mxu_jobs), 0, f) for i, f in enumerate(mxu_jobs)]
    jobs += [(span * (i + 0.5) / len(s), 1, f)
             for s in vpu_streams for i, f in enumerate(s)]
    never = None
    for _, is_vpu, f in sorted(jobs, key=lambda j: j[:2]):
        if is_vpu:
            f(never)
        else:
            y = pltpu.bitcast(f()[-8:, :], _U32)
            never = (y & zero_ref[...]) != 0


def _kernel(ax_hbm, mem_hbm, wq_hbm, wk_hbm, wv_hbm, awo_hbm, bx_hbm, bw_hbm, bwo_hbm,
            out_hbm,
            xa, mem_v, wqkv, awo, xb, bw_raw, bwq, bwkv, bwo, outa, outb,
            q_all, ka, va, kb, vb, oa, ob, hbuf, zero,
            sems, psems, wsems, xsems, osems, *, seq, seg, n_mem, heads, dh):
    dm = 1024
    n_blk = seq // _T
    half = heads // 2
    n_grp = n_blk // 2
    piece = bw_raw.shape[1]
    n_piece = dm // 2 // piece

    bx_u = bx_hbm.bitcast(_U32)
    bw_u = bw_hbm.bitcast(_U32)
    bwo_u = bwo_hbm.bitcast(_U32)
    ax_u = ax_hbm.bitcast(_U32)
    awo_u = awo_hbm.bitcast(_U32)

    def cp_xb(g):
        rows = pl.ds(pl.multiple_of(g * _T, _T), _T)
        return pltpu.make_async_copy(bx_u.at[rows], xb.at[rows], xsems.at[g])

    def cp_bw(j):
        rows = pl.ds(pl.multiple_of(j % n_piece * piece, piece), piece)
        cols = pl.ds(pl.multiple_of(j // n_piece * dm, dm), dm)
        return pltpu.make_async_copy(bw_u.at[rows, cols], bw_raw.at[j], psems.at[j])

    cp_bwo = [pltpu.make_async_copy(bwo_u.at[:, j, :],
                                    bwo.at[(j % 8) * 8 + (j // 16) * 2 + (j // 8) % 2],
                                    sems.at[0])
              for j in range(64)]
    cp_mem = pltpu.make_async_copy(mem_hbm, mem_v, sems.at[1])

    per_grp = half // n_grp

    def cp_w(g):
        return [pltpu.make_async_copy(
                    w.bitcast(_U32).at[:, par * half + g * per_grp + j, :],
                    wqkv.at[2 * (g * per_grp + j) + par, :, m * dh:(m + 1) * dh],
                    wsems.at[g])
                for j in range(per_grp) for par in range(2)
                for m, w in enumerate((wq_hbm, wk_hbm, wv_hbm))]

    def start_a_slice(g):
        for src_ref, dst_ref, sem in ((awo_u, awo, sems.at[2]), (ax_u, xa, sems.at[3])):
            n = dst_ref.shape[0] // n_grp
            rows = pl.ds(pl.multiple_of(g * n, n), n)
            pltpu.make_async_copy(src_ref.at[rows], dst_ref.at[rows], sem).start()

    def split_heads(g):
        def job(j, r, never):
            h = 2 * (g * per_grp + j)
            low = jnp.full((8, 128), 0xFFFF, _U32)
            sh = jnp.full((8, 128), 16, _U32)
            if never is not None:
                low = jnp.where(never, sh, low)
                sh = jnp.where(never, low, sh)
            for rr in range(r, r + 32, 8):
                for m in range(3):
                    even = wqkv[h, rr:rr + 8, m * dh:(m + 1) * dh]
                    odd = wqkv[h + 1, rr:rr + 8, m * dh:(m + 1) * dh]
                    wqkv[h, rr:rr + 8, m * dh:(m + 1) * dh] = (even & low) | (odd << sh)
                    wqkv[h + 1, rr:rr + 8, m * dh:(m + 1) * dh] = (
                        (even >> sh) | ((odd >> sh) << sh))
        return [functools.partial(job, j, r)
                for j in range(per_grp) for r in range(0, dm // 2, 32)]

    for j in range(n_piece):
        cp_bw(j).start()
    cp_xb(0).start()
    cp_bw(n_piece).start()
    cp_xb(1).start()
    cp_bw(n_piece + 1).start()
    zero[...] = jnp.zeros(zero.shape, _U32)

    def permute_q(j, carry):
        cp_bw(j).wait()
        _permute_b_columns(bw_raw.at[j], bwq.at[j])
        return carry

    lax.fori_loop(0, n_piece, permute_q, 0)

    def q_body(g, carry):
        @pl.when(g + 2 < n_grp)
        def _():
            cp_xb(g + 2).start()
            cp_bw(n_piece + g + 2).start()

        @pl.when(g + 2 == n_grp)
        def _():
            for cp in cp_bwo + cp_w(0):
                cp.start()

        cp_xb(g).wait()
        cp_bw(n_piece + g).wait()
        x = pltpu.bitcast(xb[pl.ds(pl.multiple_of(g * _T, _T), _T), :], _BF16)
        w = pltpu.bitcast(bwq[...].reshape(dm // 2, dm), _BF16)
        y = jnp.dot(x, w, preferred_element_type=_F32)
        for c in range(8):
            q_all[c, pl.ds(pl.multiple_of(g * 2 * _T, 2 * _T), 2 * _T), :] = (
                y[:, c * 128:(c + 1) * 128])
        _permute_b_columns(bw_raw.at[n_piece + g], bwkv.at[g])
        return carry

    lax.fori_loop(0, n_grp, q_body, 0)

    def b_proj(r0, s, dst):
        def job(c):
            x = xb[pl.ds(pl.multiple_of(r0 // 2, _T // 2), _T // 2), :]
            w = bwkv[s * n_piece:(s + 1) * n_piece, :, c * 128:(c + 1) * 128]
            y = jnp.dot(pltpu.bitcast(x, _BF16),
                        pltpu.bitcast(w.reshape(dm // 2, 128), _BF16),
                        preferred_element_type=_F32)
            dst[c, _HALO:_HALO + _T, :] = y
            return y
        return [functools.partial(job, c) for c in range(8)]

    def b_halo(src, dst):
        dst[:, 0:_HALO, :] = src[:, _T:_T + _HALO, :]

    def b_out(o_ref, r0):
        def job(c):
            w = bwo[:, :, c * 128:(c + 1) * 128].reshape(dm // 2, 128)
            y = jnp.dot(o_ref[...], pltpu.bitcast(w, _BF16), preferred_element_type=_F32)
            outb[pl.ds(pl.multiple_of(r0, _T), _T), c * 128:(c + 1) * 128] = y.astype(_BF16)
            return y
        return [functools.partial(job, c) for c in range(8)]

    def b_attention(r0, bufs, first_block):
        q_ref = q_all.at[:, pl.ds(pl.multiple_of(r0, _T), _T), :]
        pending = {}

        def logits(r, never):
            pending[r] = _b_logits(q_ref, bufs[0], r, first_block, never)

        def values(r, never):
            _b_values(pending.pop(r), bufs[1], bufs[2], r)

        starts = list(range(0, _T, _CH))
        jobs = []
        for i in range(len(starts) + 1):
            if i < len(starts):
                jobs.append(functools.partial(logits, starts[i]))
            if i >= 1:
                jobs.append(functools.partial(values, starts[i - 1]))
        return jobs

    for cp in cp_w(1):
        cp.start()
    cp_mem.start()
    _paced(zero, b_proj(0, 0, ka) + b_proj(0, 1, va))
    ka[:, 0:_HALO, :] = jnp.broadcast_to(ka[:, _HALO:_HALO + 1, :], (8, _HALO, 128))
    va[:, 0:_HALO, :] = jnp.broadcast_to(va[:, _HALO:_HALO + 1, :], (8, _HALO, 128))

    def b_step(r0, cur, nxt, extra=(), first_block=False, last_block=False):
        mxu = []
        if not first_block:
            mxu += b_out(nxt[2], r0 - _T)
        if not last_block:
            for s in range(2):
                b_halo(cur[s], nxt[s])
                mxu += b_proj(r0 + _T, s, nxt[s])
        _paced(zero, mxu, b_attention(r0, cur, first_block), list(extra), span=_SPAN)

    set_a = (ka, va, oa)
    set_b = (kb, vb, ob)
    b_step(0, set_a, set_b, first_block=True)
    for cp in cp_bwo:
        cp.wait()

    def b_body(i, carry):
        @pl.when(i + 2 < n_grp)
        def _():
            for cp in cp_w(i + 2):
                cp.start()

        start_a_slice(i)
        for cp in cp_w(i):
            cp.wait()
        r0 = (2 * i + 1) * _T
        split = split_heads(i)
        b_step(r0, set_b, set_a, split[:len(split) // 2])
        b_step(r0 + _T, set_a, set_b, split[len(split) // 2:])
        return carry

    lax.fori_loop(0, n_grp - 1, b_body, 0)
    start_a_slice(n_grp - 1)
    for cp in cp_w(n_grp - 1):
        cp.wait()
    b_step(seq - _T, set_b, set_a, split_heads(n_grp - 1), last_block=True)
    _paced(zero, b_out(ob, seq - _T))

    cp_outb = pltpu.make_async_copy(outb, out_hbm.at[:, dm:2 * dm], osems.at[0])
    cp_outb.start()

    pltpu.make_async_copy(awo_u, awo, sems.at[2]).wait()
    pltpu.make_async_copy(ax_u, xa, sems.at[3]).wait()
    cp_mem.wait()

    rows = n_mem + seg
    scale = dh ** -0.5
    hbuf[0:n_mem, :] = mem_v[...].astype(_F32)

    def a_step(s):
        qi = lax.broadcasted_iota(jnp.int32, (rows, 128), 0)
        ki = lax.broadcasted_iota(jnp.int32, (rows, 128), 1)
        real = ki < rows
        mask = ((qi < n_mem) | (qi >= ki)) & real
        fill = jnp.where(real, _MASKED, -jnp.inf).astype(_F32)
        pad = jnp.zeros((128 - rows, dh), _F32)

        xs = xa[pl.ds(pl.multiple_of(s * (seg // 2), seg // 2), seg // 2), :]
        hbuf[n_mem:rows, :] = pltpu.bitcast(xs, _BF16).astype(_F32)

        def project(h):
            return jnp.dot(hbuf[...], pltpu.bitcast(wqkv[h], _BF16),
                           preferred_element_type=_F32)

        def probs(qkv):
            k = jnp.concatenate([qkv[:, dh:2 * dh], pad], axis=0).astype(_BF16)
            sc = lax.dot_general(qkv[:, 0:dh], k, _NT, preferred_element_type=_F32)
            sc = jnp.where(mask, sc * scale, fill)
            e = jnp.exp(sc - jnp.max(sc, axis=-1, keepdims=True))
            return e / jnp.sum(e, axis=-1, keepdims=True)

        def values(p, qkv):
            v = jnp.concatenate([qkv[:, 2 * dh:3 * dh], pad], axis=0).astype(_BF16)
            return jnp.dot(p, v, preferred_element_type=_F32)

        def out_proj(g):
            h0, h1 = g * heads // 4, (g + 1) * heads // 4
            w = pltpu.bitcast(awo[h0 * dh // 2:h1 * dh // 2, :], _BF16)
            lhs = jnp.concatenate([o[h] for h in range(h0, h1)], axis=1)
            return jnp.dot(lhs, w, preferred_element_type=_F32)

        qkv, p, o = {}, {}, {}
        acc = None
        for t in range(heads + 3):
            if t < heads:
                qkv[t] = project(t)
            else:
                part = out_proj(t - heads)
                acc = part if acc is None else acc + part
            if 1 <= t <= heads:
                p[t - 1] = probs(qkv[t - 1])
            if t >= 3:
                o[t - 3] = values(p[t - 3], qkv[t - 3])
        acc = acc + out_proj(3)

        hbuf[0:n_mem, :] = acc[0:n_mem]
        outa[pl.ds(pl.multiple_of(s * seg, seg), seg), :] = acc[n_mem:rows].astype(_BF16)

    def a_body(i, carry):
        for u in range(_A_UNROLL):
            a_step(i * _A_UNROLL + u)
        n = _A_UNROLL * seg
        done = pl.ds(pl.multiple_of(i * n, n), n)
        pltpu.make_async_copy(outa.at[done], out_hbm.at[done, 0:dm], osems.at[1]).start()
        return carry

    lax.fori_loop(0, seq // (seg * _A_UNROLL), a_body, 0)
    cp_outb.wait()
    pltpu.make_async_copy(outa, out_hbm.at[:, 0:dm], osems.at[1]).wait()


@functools.partial(jax.jit, static_argnames=("A_seg_len",))
def pallas_concat_heads__memory_aug_recurrent_mem_tr__sliding_local_dilated__prompt_kernel(
    A_x: jax.Array,
    A_mem0: jax.Array,
    A_Wq: jax.Array,
    A_Wk: jax.Array,
    A_Wv: jax.Array,
    A_Wo: jax.Array,
    A_seg_len: int,
    B_x: jax.Array,
    B_wqkv: jax.Array,
    B_wo: jax.Array,
):
    batch, seq, dm = A_x.shape
    heads, dh = A_Wq.shape[1], A_Wq.shape[2]
    n_mem = A_mem0.shape[1]
    seg = int(A_seg_len)
    assert batch == 1 and dm == 1024 and dh == 128 and heads % 8 == 0
    assert B_x.shape == (1, seq, dm) and B_wqkv.shape == (dm, 3 * dm)
    assert seg % 16 == 0 and seq % (seg * _A_UNROLL) == 0 and n_mem % 8 == 0 and n_mem + seg <= 128
    assert seq % (2 * _T) == 0 and (heads // 2) % (seq // (2 * _T)) == 0
    rows = n_mem + seg

    n_grp = seq // (2 * _T)
    n_piece = n_grp // 2
    piece = dm // 2 // n_piece
    assert piece % 16 == 0 and piece * n_piece == dm // 2
    kv_buf = pltpu.VMEM((8, _HALO + _T, 128), _F32)
    o_buf = pltpu.VMEM((_T, dm), _F32)
    out = pl.pallas_call(
        functools.partial(_kernel, seq=seq, seg=seg, n_mem=n_mem, heads=heads, dh=dh),
        out_shape=jax.ShapeDtypeStruct((seq, 2 * dm), _BF16),
        in_specs=[pl.BlockSpec(memory_space=pl.ANY)] * 9,
        out_specs=pl.BlockSpec(memory_space=pl.ANY),
        scratch_shapes=[
            pltpu.VMEM((seq // 2, dm), _U32),
            pltpu.VMEM((n_mem, dm), _BF16),
            pltpu.VMEM((heads, dm // 2, 3 * dh), _U32),
            pltpu.VMEM((heads * dh // 2, dm), _U32),
            pltpu.VMEM((seq // 2, dm), _U32),
            pltpu.VMEM((3 * n_piece, piece, dm), _U32),
            pltpu.VMEM((n_piece, piece, dm), _U32),
            pltpu.VMEM((2 * n_piece, piece, dm), _U32),
            pltpu.VMEM((64, 8, dm), _U32),
            pltpu.VMEM((seq, dm), _BF16),
            pltpu.VMEM((seq, dm), _BF16),
            pltpu.VMEM((8, seq, 128), _F32),
            kv_buf, kv_buf, kv_buf, kv_buf, o_buf, o_buf,
            pltpu.VMEM((rows, dm), _F32),
            pltpu.VMEM((8, 128), _U32),
            pltpu.SemaphoreType.DMA((4,)),
            pltpu.SemaphoreType.DMA((3 * n_piece,)),
            pltpu.SemaphoreType.DMA((n_grp,)),
            pltpu.SemaphoreType.DMA((n_grp,)),
            pltpu.SemaphoreType.DMA((2,)),
        ],
        compiler_params=pltpu.CompilerParams(vmem_limit_bytes=110 * 1024 * 1024),
    )(
        A_x.reshape(seq, dm),
        A_mem0.reshape(n_mem, dm),
        A_Wq.reshape(dm // 2, 2 * heads, dh),
        A_Wk.reshape(dm // 2, 2 * heads, dh),
        A_Wv.reshape(dm // 2, 2 * heads, dh),
        A_Wo.reshape(heads * dh, dm),
        B_x.reshape(seq, dm),
        B_wqkv,
        B_wo.reshape(8, dm // 8, dm),
    )
    return out.reshape(1, seq, 2 * dm)
```

```python
import functools

import jax
import jax.numpy as jnp
from jax import lax
from jax.experimental import pallas as pl
from jax.experimental.pallas import tpu as pltpu

_F32 = jnp.float32
_BF16 = jnp.bfloat16
_U32 = jnp.uint32
_NT = (((1,), (1,)), ((), ()))
_LOG2E = 1.4426950408889634
_MASKED = -1000000000.0

_B_HEADS = 32
_B_WIN = 8
_B_DIL = 2
_HALO = 16
_T = 128
_SPAN = 0.95
_CH = 8

_PV_LAG = 3
_V_LAG = 1
_O_CUTS = (0, 8, 16, 24)
_A_UNROLL = 2


def _permute_b_columns(src_ref, dst_ref):
    rows, lag = 16, 2
    field = (lax.broadcasted_iota(jnp.int32, (rows, 128), 1) >> 1) & 7
    bits = [(field & (1 << b)) != 0 for b in range(3)]

    def spread(r):
        t = [src_ref[r:r + rows, c * 128:(c + 1) * 128] for c in range(8)]
        return [t[c] if c == 0 else pltpu.roll(t[c], 2 * c, 1) for c in range(8)]

    def exchange(t):
        t = [t[-c % 8] for c in range(8)]
        for b in range(3):
            t = [jnp.where(bits[b], t[(c - (1 << b)) % 8], t[c]) for c in range(8)]
        return [t[c] if c == 0 else pltpu.roll(t[c], 128 - 2 * c, 1) for c in range(8)]

    n = src_ref.shape[0] // rows
    first, second = {}, {}
    for i in range(n + 2 * lag):
        if i < n:
            first[i] = spread(i * rows)
        if 0 <= i - lag < n:
            second[i - lag] = exchange(first.pop(i - lag))
        if 0 <= i - 2 * lag < n:
            r = (i - 2 * lag) * rows
            for c, y in enumerate(second.pop(i - 2 * lag)):
                dst_ref[r:r + rows, c * 128:(c + 1) * 128] = y


def _b_products(q_ref, k_ref, r, never):
    logits = [None] * _B_WIN
    for c in range(8):
        q = q_ref[c, r:r + _CH, :]
        if never is not None:
            q = jnp.where(never, 0.0, q)
        for w in range(_B_WIN):
            a = _HALO + r - _B_DIL * w
            pr = q * k_ref[c, a:a + _CH, :]
            logits[w] = pr if logits[w] is None else logits[w] + pr
    return logits


def _b_lane_sum(xs, step):
    upper = (lax.broadcasted_iota(jnp.int32, (_CH, 128), 1) & step) != 0
    return [x + jnp.where(upper, pltpu.roll(x, step, 1), pltpu.roll(x, 128 - step, 1))
            for x in xs]


def _b_softmax(logits, r, first_block):
    scale = (1024 // _B_HEADS) ** -0.5
    if first_block:
        row = r + lax.broadcasted_iota(jnp.int32, (_CH, 128), 0)
        logits = [jnp.where(row >= _B_DIL * w, x, _MASKED / scale) if r < _B_DIL * w else x
                  for w, x in enumerate(logits)]
    m = functools.reduce(jnp.maximum, logits)
    es = [jnp.exp2((x - m) * (scale * _LOG2E)) for x in logits]
    inv = 1.0 / functools.reduce(jnp.add, es)
    return [e * inv for e in es]


def _b_values(ps, v_ref, o_ref, r):
    for c in range(8):
        acc = None
        for w in range(_B_WIN):
            a = _HALO + r - _B_DIL * w
            pr = ps[w] * v_ref[c, a:a + _CH, :]
            acc = pr if acc is None else acc + pr
        o_ref[r:r + _CH, c * 128:(c + 1) * 128] = acc


def _paced(zero_ref, mxu_jobs, *vpu_streams, span=1.0):
    jobs = [((i + 1.0) / len(mxu_jobs), 0, f) for i, f in enumerate(mxu_jobs)]
    jobs += [(span * (i + 0.5) / len(s), 1, f)
             for s in vpu_streams for i, f in enumerate(s)]
    never = None
    for _, is_vpu, f in sorted(jobs, key=lambda j: j[:2]):
        if is_vpu:
            f(never)
        else:
            y = pltpu.bitcast(f()[-8:, :], _U32)
            never = (y & zero_ref[...]) != 0


def _kernel(ax_hbm, mem_hbm, wq_hbm, wk_hbm, wv_hbm, awo_hbm, bx_hbm, bw_hbm, bwo_hbm,
            out_hbm,
            xa, mem_v, wqkv, awo, xb, bw_raw, bwq, bwkv, bwo, outa, outb,
            q_all, ka, va, kb, vb, oa, ob, hbuf, zero,
            sems, psems, x0sems, wsems, xsems, osems, *, seq, seg, n_mem, heads, dh):
    dm = 1024
    n_blk = seq // _T
    half = heads // 2
    n_grp = n_blk // 2
    piece = bw_raw.shape[1]
    n_piece = dm // 2 // piece

    bx_u = bx_hbm.bitcast(_U32)
    bw_u = bw_hbm.bitcast(_U32)
    bwo_u = bwo_hbm.bitcast(_U32)
    ax_u = ax_hbm.bitcast(_U32)
    awo_u = awo_hbm.bitcast(_U32)

    def cp_xb(g):
        rows = pl.ds(pl.multiple_of(g * _T, _T), _T)
        return pltpu.make_async_copy(bx_u.at[rows], xb.at[rows], xsems.at[g])

    def cp_bw(j):
        rows = pl.ds(pl.multiple_of(j % n_piece * piece, piece), piece)
        cols = pl.ds(pl.multiple_of(j // n_piece * dm, dm), dm)
        return pltpu.make_async_copy(bw_u.at[rows, cols], bw_raw.at[j], psems.at[j])

    cp_bwo = [pltpu.make_async_copy(bwo_u.at[:, j, :],
                                    bwo.at[(j % 8) * 8 + (j // 16) * 2 + (j // 8) % 2],
                                    sems.at[0])
              for j in range(64)]
    cp_mem = pltpu.make_async_copy(mem_hbm, mem_v, sems.at[1])

    per_grp = half // n_grp

    def cp_w(g):
        return [pltpu.make_async_copy(
                    w.bitcast(_U32).at[:, par * half + g * per_grp + j, :],
                    wqkv.at[2 * (g * per_grp + j) + par, :, m * dh:(m + 1) * dh],
                    wsems.at[g])
                for j in range(per_grp) for par in range(2)
                for m, w in enumerate((wq_hbm, wk_hbm, wv_hbm))]

    def start_a_slice(g):
        for src_ref, dst_ref, sem in ((awo_u, awo, sems.at[2]), (ax_u, xa, sems.at[3])):
            n = dst_ref.shape[0] // n_grp
            rows = pl.ds(pl.multiple_of(g * n, n), n)
            pltpu.make_async_copy(src_ref.at[rows], dst_ref.at[rows], sem).start()

    def split_heads(g):
        def job(j, r, never):
            h = 2 * (g * per_grp + j)
            low = jnp.full((8, 128), 0xFFFF, _U32)
            sh = jnp.full((8, 128), 16, _U32)
            if never is not None:
                low = jnp.where(never, sh, low)
                sh = jnp.where(never, low, sh)
            for rr in range(r, r + 32, 8):
                for m in range(3):
                    even = wqkv[h, rr:rr + 8, m * dh:(m + 1) * dh]
                    odd = wqkv[h + 1, rr:rr + 8, m * dh:(m + 1) * dh]
                    wqkv[h, rr:rr + 8, m * dh:(m + 1) * dh] = (even & low) | (odd << sh)
                    wqkv[h + 1, rr:rr + 8, m * dh:(m + 1) * dh] = (
                        (even >> sh) | ((odd >> sh) << sh))
        return [functools.partial(job, j, r)
                for j in range(per_grp) for r in range(0, dm // 2, 32)]

    def cp_x0(j):
        at = (pl.ds(0, _T), pl.ds(j * 2 * piece, 2 * piece))
        return pltpu.make_async_copy(bx_u.at[at], xb.at[at], x0sems.at[j])

    for j in range(n_piece):
        cp_bw(j).start()
        cp_x0(j).start()
    cp_bw(n_piece).start()
    zero[...] = jnp.zeros(zero.shape, _U32)

    def weight_piece(j):
        return bwq.at[j] if j < n_piece else bwkv.at[j - n_piece]

    cp_bw(0).wait()
    _permute_b_columns(bw_raw.at[0], weight_piece(0))
    for j in range(n_piece):
        if j == n_piece - 2:
            cp_xb(1).start()
            cp_bw(n_piece + 1).start()
        cp_x0(j).wait()
        cp_bw(j + 1).wait()
        x = pltpu.bitcast(xb[0:_T, j * 2 * piece:(j + 1) * 2 * piece], _BF16)
        y = jnp.dot(x, pltpu.bitcast(bwq[j], _BF16), preferred_element_type=_F32)
        for c in range(8):
            part = y[:, c * 128:(c + 1) * 128]
            q_all[c, 0:2 * _T, :] = part if j == 0 else q_all[c, 0:2 * _T, :] + part
        _permute_b_columns(bw_raw.at[j + 1], weight_piece(j + 1))

    def q_body(g, carry):
        @pl.when(g + 1 < n_grp)
        def _():
            cp_xb(g + 1).start()
            cp_bw(n_piece + g + 1).start()

        @pl.when(g + 2 == n_grp)
        def _():
            for cp in cp_bwo + cp_w(0):
                cp.start()

        cp_xb(g).wait()
        cp_bw(n_piece + g).wait()
        x = pltpu.bitcast(xb[pl.ds(pl.multiple_of(g * _T, _T), _T), :], _BF16)
        w = pltpu.bitcast(bwq[...].reshape(dm // 2, dm), _BF16)
        y = jnp.dot(x, w, preferred_element_type=_F32)
        for c in range(8):
            q_all[c, pl.ds(pl.multiple_of(g * 2 * _T, 2 * _T), 2 * _T), :] = (
                y[:, c * 128:(c + 1) * 128])
        _permute_b_columns(bw_raw.at[n_piece + g], bwkv.at[g])
        return carry

    lax.fori_loop(1, n_grp, q_body, 0)

    def b_proj(r0, s, dst):
        def job(c):
            x = xb[pl.ds(pl.multiple_of(r0 // 2, _T // 2), _T // 2), :]
            w = bwkv[s * n_piece:(s + 1) * n_piece, :, c * 128:(c + 1) * 128]
            y = jnp.dot(pltpu.bitcast(x, _BF16),
                        pltpu.bitcast(w.reshape(dm // 2, 128), _BF16),
                        preferred_element_type=_F32)
            dst[c, _HALO:_HALO + _T, :] = y
            return y
        return [functools.partial(job, c) for c in range(8)]

    def b_halo(src, dst):
        dst[:, 0:_HALO, :] = src[:, _T:_T + _HALO, :]

    def b_out(o_ref, r0):
        def job(c):
            w = bwo[:, :, c * 128:(c + 1) * 128].reshape(dm // 2, 128)
            y = jnp.dot(o_ref[...], pltpu.bitcast(w, _BF16), preferred_element_type=_F32)
            outb[pl.ds(pl.multiple_of(r0, _T), _T), c * 128:(c + 1) * 128] = y.astype(_BF16)
            return y
        return [functools.partial(job, c) for c in range(8)]

    def b_attention(r0, bufs, first_block):
        q_ref = q_all.at[:, pl.ds(pl.multiple_of(r0, _T), _T), :]
        stages = (
            lambda x, r, never: _b_lane_sum(_b_products(q_ref, bufs[0], r, never), 1),
            lambda x, r, never: _b_lane_sum(x, 16),
            lambda x, r, never: _b_softmax(x, r, first_block),
            lambda x, r, never: _b_values(x, bufs[1], bufs[2], r),
        )
        state = {}

        def job(stage, r, never):
            state[r] = stages[stage](state.get(r), r, never)

        order = sorted((i + s, -s, i) for i in range(_T // _CH) for s in range(4))
        return [functools.partial(job, -s, i * _CH) for _, s, i in order]

    for cp in cp_w(1):
        cp.start()
    cp_mem.start()
    _paced(zero, b_proj(0, 0, ka) + b_proj(0, 1, va))
    ka[:, 0:_HALO, :] = jnp.broadcast_to(ka[:, _HALO:_HALO + 1, :], (8, _HALO, 128))
    va[:, 0:_HALO, :] = jnp.broadcast_to(va[:, _HALO:_HALO + 1, :], (8, _HALO, 128))

    def b_step(r0, cur, nxt, extra=(), first_block=False, last_block=False):
        mxu = []
        if not first_block:
            mxu += b_out(nxt[2], r0 - _T)
        if not last_block:
            for s in range(2):
                b_halo(cur[s], nxt[s])
                mxu += b_proj(r0 + _T, s, nxt[s])
        _paced(zero, mxu, b_attention(r0, cur, first_block), list(extra), span=_SPAN)

    set_a = (ka, va, oa)
    set_b = (kb, vb, ob)
    b_step(0, set_a, set_b, first_block=True)
    for cp in cp_bwo:
        cp.wait()

    def b_body(i, carry):
        @pl.when(i + 2 < n_grp)
        def _():
            for cp in cp_w(i + 2):
                cp.start()

        start_a_slice(i)
        for cp in cp_w(i):
            cp.wait()
        r0 = (2 * i + 1) * _T
        split = split_heads(i)
        b_step(r0, set_b, set_a, split[:len(split) // 2])
        b_step(r0 + _T, set_a, set_b, split[len(split) // 2:])
        return carry

    lax.fori_loop(0, n_grp - 1, b_body, 0)
    start_a_slice(n_grp - 1)
    for cp in cp_w(n_grp - 1):
        cp.wait()
    b_step(seq - _T, set_b, set_a, split_heads(n_grp - 1), last_block=True)
    _paced(zero, b_out(ob, seq - _T))

    cp_outb = pltpu.make_async_copy(outb, out_hbm.at[:, dm:2 * dm], osems.at[0])
    cp_outb.start()

    pltpu.make_async_copy(awo_u, awo, sems.at[2]).wait()
    pltpu.make_async_copy(ax_u, xa, sems.at[3]).wait()
    cp_mem.wait()

    rows = n_mem + seg
    scale = dh ** -0.5
    hbuf[0:n_mem, :] = mem_v[...].astype(_F32)

    def a_step(s):
        qi = lax.broadcasted_iota(jnp.int32, (rows, 128), 0)
        ki = lax.broadcasted_iota(jnp.int32, (rows, 128), 1)
        real = ki < rows
        mask = ((qi < n_mem) | (qi >= ki)) & real
        fill = jnp.where(real, _MASKED, -jnp.inf).astype(_F32)
        pad = jnp.zeros((128 - rows, dh), _F32)

        xs = xa[pl.ds(pl.multiple_of(s * (seg // 2), seg // 2), seg // 2), :]
        hbuf[n_mem:rows, :] = pltpu.bitcast(xs, _BF16).astype(_F32)

        def project(h, c0, c1):
            w = wqkv[h, :, c0 * dh:c1 * dh]
            return jnp.dot(hbuf[...], pltpu.bitcast(w, _BF16), preferred_element_type=_F32)

        def probs(qk):
            k = jnp.concatenate([qk[:, dh:2 * dh], pad], axis=0).astype(_BF16)
            sc = lax.dot_general(qk[:, 0:dh], k, _NT, preferred_element_type=_F32)
            sc = jnp.where(mask, sc * scale, fill)
            e = jnp.exp(sc - jnp.max(sc, axis=-1, keepdims=True))
            return e / jnp.sum(e, axis=-1, keepdims=True)

        def values(p, v):
            v = jnp.concatenate([v, pad], axis=0).astype(_BF16)
            return jnp.dot(p, v, preferred_element_type=_F32)

        def out_proj(h0, h1):
            w = pltpu.bitcast(awo[h0 * dh // 2:h1 * dh // 2, :], _BF16)
            lhs = jnp.concatenate([o[h] for h in range(h0, h1)], axis=1)
            return jnp.dot(lhs, w, preferred_element_type=_F32)

        qk, v, p, o = {}, {}, {}, {}
        cuts = [c * heads // 32 for c in _O_CUTS]
        acc = None
        for t in range(heads + _PV_LAG):
            if t < heads:
                qk[t] = project(t, 0, 2)
            if 0 <= t - _V_LAG < heads:
                v[t - _V_LAG] = project(t - _V_LAG, 2, 3)
            if heads <= t < heads + len(cuts) - 1:
                part = out_proj(cuts[t - heads], cuts[t - heads + 1])
                acc = part if acc is None else acc + part
            if 1 <= t <= heads:
                p[t - 1] = probs(qk[t - 1])
            if t >= _PV_LAG:
                o[t - _PV_LAG] = values(p[t - _PV_LAG], v[t - _PV_LAG])
        acc = acc + out_proj(cuts[-1], heads)

        hbuf[0:n_mem, :] = acc[0:n_mem]
        outa[pl.ds(pl.multiple_of(s * seg, seg), seg), :] = acc[n_mem:rows].astype(_BF16)

    def a_body(i, carry):
        for u in range(_A_UNROLL):
            a_step(i * _A_UNROLL + u)
        n = _A_UNROLL * seg
        done = pl.ds(pl.multiple_of(i * n, n), n)
        pltpu.make_async_copy(outa.at[done], out_hbm.at[done, 0:dm], osems.at[1]).start()
        return carry

    lax.fori_loop(0, seq // (seg * _A_UNROLL), a_body, 0)
    cp_outb.wait()
    pltpu.make_async_copy(outa, out_hbm.at[:, 0:dm], osems.at[1]).wait()


@functools.partial(jax.jit, static_argnames=("A_seg_len",))
def pallas_concat_heads__memory_aug_recurrent_mem_tr__sliding_local_dilated__prompt_kernel(
    A_x: jax.Array,
    A_mem0: jax.Array,
    A_Wq: jax.Array,
    A_Wk: jax.Array,
    A_Wv: jax.Array,
    A_Wo: jax.Array,
    A_seg_len: int,
    B_x: jax.Array,
    B_wqkv: jax.Array,
    B_wo: jax.Array,
):
    batch, seq, dm = A_x.shape
    heads, dh = A_Wq.shape[1], A_Wq.shape[2]
    n_mem = A_mem0.shape[1]
    seg = int(A_seg_len)
    assert batch == 1 and dm == 1024 and dh == 128 and heads % 8 == 0
    assert B_x.shape == (1, seq, dm) and B_wqkv.shape == (dm, 3 * dm)
    assert seg % 16 == 0 and seq % (seg * _A_UNROLL) == 0 and n_mem % 8 == 0 and n_mem + seg <= 128
    assert seq % (2 * _T) == 0 and (heads // 2) % (seq // (2 * _T)) == 0
    rows = n_mem + seg

    n_grp = seq // (2 * _T)
    n_piece = n_grp // 2
    piece = dm // 2 // n_piece
    assert piece % 16 == 0 and piece * n_piece == dm // 2
    kv_buf = pltpu.VMEM((8, _HALO + _T, 128), _F32)
    o_buf = pltpu.VMEM((_T, dm), _F32)
    out = pl.pallas_call(
        functools.partial(_kernel, seq=seq, seg=seg, n_mem=n_mem, heads=heads, dh=dh),
        out_shape=jax.ShapeDtypeStruct((seq, 2 * dm), _BF16),
        in_specs=[pl.BlockSpec(memory_space=pl.ANY)] * 9,
        out_specs=pl.BlockSpec(memory_space=pl.ANY),
        scratch_shapes=[
            pltpu.VMEM((seq // 2, dm), _U32),
            pltpu.VMEM((n_mem, dm), _BF16),
            pltpu.VMEM((heads, dm // 2, 3 * dh), _U32),
            pltpu.VMEM((heads * dh // 2, dm), _U32),
            pltpu.VMEM((seq // 2, dm), _U32),
            pltpu.VMEM((3 * n_piece, piece, dm), _U32),
            pltpu.VMEM((n_piece, piece, dm), _U32),
            pltpu.VMEM((2 * n_piece, piece, dm), _U32),
            pltpu.VMEM((64, 8, dm), _U32),
            pltpu.VMEM((seq, dm), _BF16),
            pltpu.VMEM((seq, dm), _BF16),
            pltpu.VMEM((8, seq, 128), _F32),
            kv_buf, kv_buf, kv_buf, kv_buf, o_buf, o_buf,
            pltpu.VMEM((rows, dm), _F32),
            pltpu.VMEM((8, 128), _U32),
            pltpu.SemaphoreType.DMA((4,)),
            pltpu.SemaphoreType.DMA((3 * n_piece,)),
            pltpu.SemaphoreType.DMA((n_piece,)),
            pltpu.SemaphoreType.DMA((n_grp,)),
            pltpu.SemaphoreType.DMA((n_grp,)),
            pltpu.SemaphoreType.DMA((2,)),
        ],
        compiler_params=pltpu.CompilerParams(vmem_limit_bytes=110 * 1024 * 1024),
    )(
        A_x.reshape(seq, dm),
        A_mem0.reshape(n_mem, dm),
        A_Wq.reshape(dm // 2, 2 * heads, dh),
        A_Wk.reshape(dm // 2, 2 * heads, dh),
        A_Wv.reshape(dm // 2, 2 * heads, dh),
        A_Wo.reshape(heads * dh, dm),
        B_x.reshape(seq, dm),
        B_wqkv,
        B_wo.reshape(8, dm // 8, dm),
    )
    return out.reshape(1, seq, 2 * dm)
```

```python
import functools

import jax
import jax.numpy as jnp
from jax import lax
from jax.experimental import pallas as pl
from jax.experimental.pallas import tpu as pltpu

_F32 = jnp.float32
_BF16 = jnp.bfloat16
_U32 = jnp.uint32
_NT = (((1,), (1,)), ((), ()))
_LOG2E = 1.4426950408889634
_MASKED = -1000000000.0

_B_HEADS = 32
_B_WIN = 8
_B_DIL = 2
_HALO = 16
_T = 128
_SPAN = 0.95
_CH = 8

_PV_LAG = 3
_V_LAG = 1
_O_CUTS = (0, 8, 16, 24)
_A_UNROLL = 2


def _permute_b_columns(src_ref, dst_ref):
    rows, lag = 16, 2
    field = (lax.broadcasted_iota(jnp.int32, (rows, 128), 1) >> 1) & 7
    bits = [(field & (1 << b)) != 0 for b in range(3)]

    def spread(r):
        t = [src_ref[r:r + rows, c * 128:(c + 1) * 128] for c in range(8)]
        return [t[c] if c == 0 else pltpu.roll(t[c], 2 * c, 1) for c in range(8)]

    def exchange(t):
        t = [t[-c % 8] for c in range(8)]
        for b in range(3):
            t = [jnp.where(bits[b], t[(c - (1 << b)) % 8], t[c]) for c in range(8)]
        return [t[c] if c == 0 else pltpu.roll(t[c], 128 - 2 * c, 1) for c in range(8)]

    n = src_ref.shape[0] // rows
    first, second = {}, {}
    for i in range(n + 2 * lag):
        if i < n:
            first[i] = spread(i * rows)
        if 0 <= i - lag < n:
            second[i - lag] = exchange(first.pop(i - lag))
        if 0 <= i - 2 * lag < n:
            r = (i - 2 * lag) * rows
            for c, y in enumerate(second.pop(i - 2 * lag)):
                dst_ref[r:r + rows, c * 128:(c + 1) * 128] = y


def _b_products(q_ref, k_ref, r, never):
    logits = [None] * _B_WIN
    for c in range(8):
        q = q_ref[c, r:r + _CH, :]
        if never is not None:
            q = jnp.where(never, 0.0, q)
        for w in range(_B_WIN):
            a = _HALO + r - _B_DIL * w
            pr = q * k_ref[c, a:a + _CH, :]
            logits[w] = pr if logits[w] is None else logits[w] + pr
    return logits


def _b_lane_sum(xs, step):
    upper = (lax.broadcasted_iota(jnp.int32, (_CH, 128), 1) & step) != 0
    return [x + jnp.where(upper, pltpu.roll(x, step, 1), pltpu.roll(x, 128 - step, 1))
            for x in xs]


def _b_softmax(logits, r, first_block):
    scale = (1024 // _B_HEADS) ** -0.5
    if first_block:
        row = r + lax.broadcasted_iota(jnp.int32, (_CH, 128), 0)
        logits = [jnp.where(row >= _B_DIL * w, x, _MASKED / scale) if r < _B_DIL * w else x
                  for w, x in enumerate(logits)]
    m = functools.reduce(jnp.maximum, logits)
    es = [jnp.exp2((x - m) * (scale * _LOG2E)) for x in logits]
    inv = 1.0 / functools.reduce(jnp.add, es)
    return [e * inv for e in es]


def _b_values(ps, v_ref, o_ref, r):
    for c in range(8):
        acc = None
        for w in range(_B_WIN):
            a = _HALO + r - _B_DIL * w
            pr = ps[w] * v_ref[c, a:a + _CH, :]
            acc = pr if acc is None else acc + pr
        o_ref[r:r + _CH, c * 128:(c + 1) * 128] = acc


def _paced(zero_ref, mxu_jobs, *vpu_streams, span=1.0):
    jobs = [((i + 1.0) / len(mxu_jobs), 0, f) for i, f in enumerate(mxu_jobs)]
    jobs += [(span * (i + 0.5) / len(s), 1, f)
             for s in vpu_streams for i, f in enumerate(s)]
    never = None
    for _, is_vpu, f in sorted(jobs, key=lambda j: j[:2]):
        if is_vpu:
            f(never)
        else:
            y = pltpu.bitcast(f()[-8:, :], _U32)
            never = (y & zero_ref[...]) != 0


def _kernel(ax_hbm, mem_hbm, wq_hbm, wk_hbm, wv_hbm, awo_hbm, bx_hbm, bw_hbm, bwo_hbm,
            out_hbm,
            xa, mem_v, wqkv, awo, xb, bw_raw, bwq, bwkv, bwo, outa, outb,
            q_all, ka, va, kb, vb, oa, ob, hbuf, zero,
            sems, psems, x0sems, wsems, xsems, osems, *, seq, seg, n_mem, heads, dh):
    dm = 1024
    n_blk = seq // _T
    half = heads // 2
    n_grp = n_blk // 2
    piece = bw_raw.shape[1]
    n_piece = dm // 2 // piece

    bx_u = bx_hbm.bitcast(_U32)
    bw_u = bw_hbm.bitcast(_U32)
    bwo_u = bwo_hbm.bitcast(_U32)
    ax_u = ax_hbm.bitcast(_U32)
    awo_u = awo_hbm.bitcast(_U32)

    def cp_xb(g):
        rows = pl.ds(pl.multiple_of(g * _T, _T), _T)
        return pltpu.make_async_copy(bx_u.at[rows], xb.at[rows], xsems.at[g])

    def cp_bw(j):
        rows = pl.ds(pl.multiple_of(j % n_piece * piece, piece), piece)
        cols = pl.ds(pl.multiple_of(j // n_piece * dm, dm), dm)
        return pltpu.make_async_copy(bw_u.at[rows, cols], bw_raw.at[j], psems.at[j])

    cp_bwo = [pltpu.make_async_copy(bwo_u.at[:, j, :],
                                    bwo.at[(j % 8) * 8 + (j // 16) * 2 + (j // 8) % 2],
                                    sems.at[0])
              for j in range(64)]
    cp_mem = pltpu.make_async_copy(mem_hbm, mem_v, sems.at[1])

    per_grp = half // n_grp

    def cp_w(g):
        return [pltpu.make_async_copy(
                    w.bitcast(_U32).at[:, par * half + g * per_grp + j, :],
                    wqkv.at[2 * (g * per_grp + j) + par, :, m * dh:(m + 1) * dh],
                    wsems.at[g])
                for j in range(per_grp) for par in range(2)
                for m, w in enumerate((wq_hbm, wk_hbm, wv_hbm))]

    def start_a_slice(g):
        for src_ref, dst_ref, sem in ((awo_u, awo, sems.at[2]), (ax_u, xa, sems.at[3])):
            n = dst_ref.shape[0] // n_grp
            rows = pl.ds(pl.multiple_of(g * n, n), n)
            pltpu.make_async_copy(src_ref.at[rows], dst_ref.at[rows], sem).start()

    def split_heads(g):
        def job(j, r, never):
            h = 2 * (g * per_grp + j)
            low = jnp.full((8, 128), 0xFFFF, _U32)
            sh = jnp.full((8, 128), 16, _U32)
            if never is not None:
                low = jnp.where(never, sh, low)
                sh = jnp.where(never, low, sh)
            for rr in range(r, r + 32, 8):
                for m in range(3):
                    even = wqkv[h, rr:rr + 8, m * dh:(m + 1) * dh]
                    odd = wqkv[h + 1, rr:rr + 8, m * dh:(m + 1) * dh]
                    wqkv[h, rr:rr + 8, m * dh:(m + 1) * dh] = (even & low) | (odd << sh)
                    wqkv[h + 1, rr:rr + 8, m * dh:(m + 1) * dh] = (
                        (even >> sh) | ((odd >> sh) << sh))
        return [functools.partial(job, j, r)
                for j in range(per_grp) for r in range(0, dm // 2, 32)]

    def cp_x0(j):
        at = (pl.ds(0, _T), pl.ds(j * 2 * piece, 2 * piece))
        return pltpu.make_async_copy(bx_u.at[at], xb.at[at], x0sems.at[j])

    for j in range(n_piece):
        cp_bw(j).start()
        cp_x0(j).start()
    cp_bw(n_piece).start()
    zero[...] = jnp.zeros(zero.shape, _U32)

    def weight_piece(j):
        return bwq.at[j] if j < n_piece else bwkv.at[j - n_piece]

    cp_bw(0).wait()
    _permute_b_columns(bw_raw.at[0], weight_piece(0))
    for j in range(n_piece):
        if j >= n_piece - 2:
            cp_xb(j - n_piece + 3).start()
            cp_bw(j + 3).start()
        cp_x0(j).wait()
        cp_bw(j + 1).wait()
        x = pltpu.bitcast(xb[0:_T, j * 2 * piece:(j + 1) * 2 * piece], _BF16)
        y = jnp.dot(x, pltpu.bitcast(bwq[j], _BF16), preferred_element_type=_F32)
        for c in range(8):
            part = y[:, c * 128:(c + 1) * 128]
            q_all[c, 0:2 * _T, :] = part if j == 0 else q_all[c, 0:2 * _T, :] + part
        _permute_b_columns(bw_raw.at[j + 1], weight_piece(j + 1))

    def q_body(g, carry):
        @pl.when(g + 2 < n_grp)
        def _():
            cp_xb(g + 2).start()
            cp_bw(n_piece + g + 2).start()

        @pl.when(g + 1 == n_grp)
        def _():
            for cp in cp_bwo + cp_w(0):
                cp.start()

        cp_xb(g).wait()
        cp_bw(n_piece + g).wait()
        x = pltpu.bitcast(xb[pl.ds(pl.multiple_of(g * _T, _T), _T), :], _BF16)
        w = pltpu.bitcast(bwq[...].reshape(dm // 2, dm), _BF16)
        y = jnp.dot(x, w, preferred_element_type=_F32)
        for c in range(8):
            q_all[c, pl.ds(pl.multiple_of(g * 2 * _T, 2 * _T), 2 * _T), :] = (
                y[:, c * 128:(c + 1) * 128])
        _permute_b_columns(bw_raw.at[n_piece + g], bwkv.at[g])
        return carry

    lax.fori_loop(1, n_grp, q_body, 0)

    def b_proj(r0, s, dst):
        def job(c):
            x = xb[pl.ds(pl.multiple_of(r0 // 2, _T // 2), _T // 2), :]
            w = bwkv[s * n_piece:(s + 1) * n_piece, :, c * 128:(c + 1) * 128]
            y = jnp.dot(pltpu.bitcast(x, _BF16),
                        pltpu.bitcast(w.reshape(dm // 2, 128), _BF16),
                        preferred_element_type=_F32)
            dst[c, _HALO:_HALO + _T, :] = y
            return y
        return [functools.partial(job, c) for c in range(8)]

    def b_halo(src, dst):
        dst[:, 0:_HALO, :] = src[:, _T:_T + _HALO, :]

    def b_out(o_ref, r0):
        def job(c):
            w = bwo[:, :, c * 128:(c + 1) * 128].reshape(dm // 2, 128)
            y = jnp.dot(o_ref[...], pltpu.bitcast(w, _BF16), preferred_element_type=_F32)
            outb[pl.ds(pl.multiple_of(r0, _T), _T), c * 128:(c + 1) * 128] = y.astype(_BF16)
            return y
        return [functools.partial(job, c) for c in range(8)]

    def b_attention(r0, bufs, first_block):
        q_ref = q_all.at[:, pl.ds(pl.multiple_of(r0, _T), _T), :]
        stages = (
            lambda x, r, never: _b_lane_sum(_b_products(q_ref, bufs[0], r, never), 1),
            lambda x, r, never: _b_lane_sum(x, 16),
            lambda x, r, never: _b_softmax(x, r, first_block),
            lambda x, r, never: _b_values(x, bufs[1], bufs[2], r),
        )
        state = {}

        def job(stage, r, never):
            state[r] = stages[stage](state.get(r), r, never)

        order = sorted((i + s, -s, i) for i in range(_T // _CH) for s in range(4))
        return [functools.partial(job, -s, i * _CH) for _, s, i in order]

    for cp in cp_w(1):
        cp.start()
    cp_mem.start()
    _paced(zero, b_proj(0, 0, ka) + b_proj(0, 1, va))
    ka[:, 0:_HALO, :] = jnp.broadcast_to(ka[:, _HALO:_HALO + 1, :], (8, _HALO, 128))
    va[:, 0:_HALO, :] = jnp.broadcast_to(va[:, _HALO:_HALO + 1, :], (8, _HALO, 128))

    def b_step(r0, cur, nxt, extra=(), first_block=False, last_block=False):
        mxu = []
        if not first_block:
            mxu += b_out(nxt[2], r0 - _T)
        if not last_block:
            for s in range(2):
                b_halo(cur[s], nxt[s])
                mxu += b_proj(r0 + _T, s, nxt[s])
        _paced(zero, mxu, b_attention(r0, cur, first_block), list(extra), span=_SPAN)

    set_a = (ka, va, oa)
    set_b = (kb, vb, ob)
    b_step(0, set_a, set_b, first_block=True)
    for cp in cp_bwo:
        cp.wait()

    def b_body(i, carry):
        @pl.when(i + 2 < n_grp)
        def _():
            for cp in cp_w(i + 2):
                cp.start()

        start_a_slice(i)
        for cp in cp_w(i):
            cp.wait()
        r0 = (2 * i + 1) * _T
        split = split_heads(i)
        b_step(r0, set_b, set_a, split[:len(split) // 2])
        b_step(r0 + _T, set_a, set_b, split[len(split) // 2:])
        return carry

    lax.fori_loop(0, n_grp - 1, b_body, 0)
    start_a_slice(n_grp - 1)
    for cp in cp_w(n_grp - 1):
        cp.wait()
    b_step(seq - _T, set_b, set_a, split_heads(n_grp - 1), last_block=True)
    _paced(zero, b_out(ob, seq - _T))

    cp_outb = pltpu.make_async_copy(outb, out_hbm.at[:, dm:2 * dm], osems.at[0])
    cp_outb.start()

    pltpu.make_async_copy(awo_u, awo, sems.at[2]).wait()
    pltpu.make_async_copy(ax_u, xa, sems.at[3]).wait()
    cp_mem.wait()

    rows = n_mem + seg
    scale = dh ** -0.5
    hbuf[0:n_mem, :] = mem_v[...].astype(_F32)

    def a_step(s):
        qi = lax.broadcasted_iota(jnp.int32, (rows, 128), 0)
        ki = lax.broadcasted_iota(jnp.int32, (rows, 128), 1)
        real = ki < rows
        mask = ((qi < n_mem) | (qi >= ki)) & real
        fill = jnp.where(real, _MASKED, -jnp.inf).astype(_F32)
        pad = jnp.zeros((128 - rows, dh), _F32)

        xs = xa[pl.ds(pl.multiple_of(s * (seg // 2), seg // 2), seg // 2), :]
        hbuf[n_mem:rows, :] = pltpu.bitcast(xs, _BF16).astype(_F32)

        def project(h, c0, c1):
            w = wqkv[h, :, c0 * dh:c1 * dh]
            return jnp.dot(hbuf[...], pltpu.bitcast(w, _BF16), preferred_element_type=_F32)

        def probs(qk):
            k = jnp.concatenate([qk[:, dh:2 * dh], pad], axis=0).astype(_BF16)
            sc = lax.dot_general(qk[:, 0:dh], k, _NT, preferred_element_type=_F32)
            sc = jnp.where(mask, sc * scale, fill)
            e = jnp.exp(sc - jnp.max(sc, axis=-1, keepdims=True))
            return e / jnp.sum(e, axis=-1, keepdims=True)

        def values(p, v):
            v = jnp.concatenate([v, pad], axis=0).astype(_BF16)
            return jnp.dot(p, v, preferred_element_type=_F32)

        def out_proj(h0, h1):
            w = pltpu.bitcast(awo[h0 * dh // 2:h1 * dh // 2, :], _BF16)
            lhs = jnp.concatenate([o[h] for h in range(h0, h1)], axis=1)
            return jnp.dot(lhs, w, preferred_element_type=_F32)

        qk, v, p, o = {}, {}, {}, {}
        cuts = [c * heads // 32 for c in _O_CUTS]
        acc = None
        for t in range(heads + _PV_LAG):
            if t < heads:
                qk[t] = project(t, 0, 2)
            if 0 <= t - _V_LAG < heads:
                v[t - _V_LAG] = project(t - _V_LAG, 2, 3)
            if heads <= t < heads + len(cuts) - 1:
                part = out_proj(cuts[t - heads], cuts[t - heads + 1])
                acc = part if acc is None else acc + part
            if 1 <= t <= heads:
                p[t - 1] = probs(qk[t - 1])
            if t >= _PV_LAG:
                o[t - _PV_LAG] = values(p[t - _PV_LAG], v[t - _PV_LAG])
        acc = acc + out_proj(cuts[-1], heads)

        hbuf[0:n_mem, :] = acc[0:n_mem]
        outa[pl.ds(pl.multiple_of(s * seg, seg), seg), :] = acc[n_mem:rows].astype(_BF16)

    def a_body(i, carry):
        for u in range(_A_UNROLL):
            a_step(i * _A_UNROLL + u)
        n = _A_UNROLL * seg
        done = pl.ds(pl.multiple_of(i * n, n), n)
        pltpu.make_async_copy(outa.at[done], out_hbm.at[done, 0:dm], osems.at[1]).start()
        return carry

    lax.fori_loop(0, seq // (seg * _A_UNROLL), a_body, 0)
    cp_outb.wait()
    pltpu.make_async_copy(outa, out_hbm.at[:, 0:dm], osems.at[1]).wait()


@functools.partial(jax.jit, static_argnames=("A_seg_len",))
def pallas_concat_heads__memory_aug_recurrent_mem_tr__sliding_local_dilated__prompt_kernel(
    A_x: jax.Array,
    A_mem0: jax.Array,
    A_Wq: jax.Array,
    A_Wk: jax.Array,
    A_Wv: jax.Array,
    A_Wo: jax.Array,
    A_seg_len: int,
    B_x: jax.Array,
    B_wqkv: jax.Array,
    B_wo: jax.Array,
):
    batch, seq, dm = A_x.shape
    heads, dh = A_Wq.shape[1], A_Wq.shape[2]
    n_mem = A_mem0.shape[1]
    seg = int(A_seg_len)
    assert batch == 1 and dm == 1024 and dh == 128 and heads % 8 == 0
    assert B_x.shape == (1, seq, dm) and B_wqkv.shape == (dm, 3 * dm)
    assert seg % 16 == 0 and seq % (seg * _A_UNROLL) == 0 and n_mem % 8 == 0 and n_mem + seg <= 128
    assert seq % (2 * _T) == 0 and (heads // 2) % (seq // (2 * _T)) == 0
    rows = n_mem + seg

    n_grp = seq // (2 * _T)
    n_piece = n_grp // 2
    piece = dm // 2 // n_piece
    assert piece % 16 == 0 and piece * n_piece == dm // 2
    kv_buf = pltpu.VMEM((8, _HALO + _T, 128), _F32)
    o_buf = pltpu.VMEM((_T, dm), _F32)
    out = pl.pallas_call(
        functools.partial(_kernel, seq=seq, seg=seg, n_mem=n_mem, heads=heads, dh=dh),
        out_shape=jax.ShapeDtypeStruct((seq, 2 * dm), _BF16),
        in_specs=[pl.BlockSpec(memory_space=pl.ANY)] * 9,
        out_specs=pl.BlockSpec(memory_space=pl.ANY),
        scratch_shapes=[
            pltpu.VMEM((seq // 2, dm), _U32),
            pltpu.VMEM((n_mem, dm), _BF16),
            pltpu.VMEM((heads, dm // 2, 3 * dh), _U32),
            pltpu.VMEM((heads * dh // 2, dm), _U32),
            pltpu.VMEM((seq // 2, dm), _U32),
            pltpu.VMEM((3 * n_piece, piece, dm), _U32),
            pltpu.VMEM((n_piece, piece, dm), _U32),
            pltpu.VMEM((2 * n_piece, piece, dm), _U32),
            pltpu.VMEM((64, 8, dm), _U32),
            pltpu.VMEM((seq, dm), _BF16),
            pltpu.VMEM((seq, dm), _BF16),
            pltpu.VMEM((8, seq, 128), _F32),
            kv_buf, kv_buf, kv_buf, kv_buf, o_buf, o_buf,
            pltpu.VMEM((rows, dm), _F32),
            pltpu.VMEM((8, 128), _U32),
            pltpu.SemaphoreType.DMA((4,)),
            pltpu.SemaphoreType.DMA((3 * n_piece,)),
            pltpu.SemaphoreType.DMA((n_piece,)),
            pltpu.SemaphoreType.DMA((n_grp,)),
            pltpu.SemaphoreType.DMA((n_grp,)),
            pltpu.SemaphoreType.DMA((2,)),
        ],
        compiler_params=pltpu.CompilerParams(vmem_limit_bytes=110 * 1024 * 1024),
    )(
        A_x.reshape(seq, dm),
        A_mem0.reshape(n_mem, dm),
        A_Wq.reshape(dm // 2, 2 * heads, dh),
        A_Wk.reshape(dm // 2, 2 * heads, dh),
        A_Wv.reshape(dm // 2, 2 * heads, dh),
        A_Wo.reshape(heads * dh, dm),
        B_x.reshape(seq, dm),
        B_wqkv,
        B_wo.reshape(8, dm // 8, dm),
    )
    return out.reshape(1, seq, 2 * dm)
```

```python
import functools

import jax
import jax.numpy as jnp
from jax import lax
from jax.experimental import pallas as pl
from jax.experimental.pallas import tpu as pltpu

_F32 = jnp.float32
_BF16 = jnp.bfloat16
_U32 = jnp.uint32
_NT = (((1,), (1,)), ((), ()))
_LOG2E = 1.4426950408889634
_MASKED = -1000000000.0

_B_HEADS = 32
_B_WIN = 8
_B_DIL = 2
_HALO = 16
_T = 128
_SPAN = 0.95
_CH = 8

_PV_LAG = 3
_V_LAG = 1
_O_CUTS = (0, 8, 16, 24)
_A_UNROLL = 2


def _permute_b_columns(src_ref, dst_ref):
    rows, lag = 16, 2
    field = (lax.broadcasted_iota(jnp.int32, (rows, 128), 1) >> 1) & 7
    bits = [(field & (1 << b)) != 0 for b in range(3)]

    def spread(r):
        t = [src_ref[r:r + rows, c * 128:(c + 1) * 128] for c in range(8)]
        return [t[c] if c == 0 else pltpu.roll(t[c], 2 * c, 1) for c in range(8)]

    def exchange(t):
        t = [t[-c % 8] for c in range(8)]
        for b in range(3):
            t = [jnp.where(bits[b], t[(c - (1 << b)) % 8], t[c]) for c in range(8)]
        return [t[c] if c == 0 else pltpu.roll(t[c], 128 - 2 * c, 1) for c in range(8)]

    n = src_ref.shape[0] // rows
    first, second = {}, {}
    for i in range(n + 2 * lag):
        if i < n:
            first[i] = spread(i * rows)
        if 0 <= i - lag < n:
            second[i - lag] = exchange(first.pop(i - lag))
        if 0 <= i - 2 * lag < n:
            r = (i - 2 * lag) * rows
            for c, y in enumerate(second.pop(i - 2 * lag)):
                dst_ref[r:r + rows, c * 128:(c + 1) * 128] = y


def _b_products(q_ref, k_ref, r, never):
    logits = [None] * _B_WIN
    for c in range(8):
        q = q_ref[c, r:r + _CH, :]
        if never is not None and c % 4 == 0:
            q = jnp.where(never, 0.0, q)
        for w in range(_B_WIN):
            a = _HALO + r - _B_DIL * w
            pr = q * k_ref[c, a:a + _CH, :]
            logits[w] = pr if logits[w] is None else logits[w] + pr
    return logits


def _b_lane_sum(xs, step):
    upper = (lax.broadcasted_iota(jnp.int32, (_CH, 128), 1) & step) != 0
    return [x + jnp.where(upper, pltpu.roll(x, step, 1), pltpu.roll(x, 128 - step, 1))
            for x in xs]


def _b_softmax(logits, r, first_block):
    scale = (1024 // _B_HEADS) ** -0.5
    if first_block:
        row = r + lax.broadcasted_iota(jnp.int32, (_CH, 128), 0)
        logits = [jnp.where(row >= _B_DIL * w, x, _MASKED / scale) if r < _B_DIL * w else x
                  for w, x in enumerate(logits)]
    m = functools.reduce(jnp.maximum, logits)
    es = [jnp.exp2((x - m) * (scale * _LOG2E)) for x in logits]
    inv = 1.0 / functools.reduce(jnp.add, es)
    return [e * inv for e in es]


def _b_values(ps, v_ref, o_ref, r):
    for c in range(8):
        acc = None
        for w in range(_B_WIN):
            a = _HALO + r - _B_DIL * w
            pr = ps[w] * v_ref[c, a:a + _CH, :]
            acc = pr if acc is None else acc + pr
        o_ref[r:r + _CH, c * 128:(c + 1) * 128] = acc


def _paced(zero_ref, mxu_jobs, *vpu_streams, span=1.0):
    jobs = [((i + 1.0) / len(mxu_jobs), 0, f) for i, f in enumerate(mxu_jobs)]
    jobs += [(span * (i + 0.5) / len(s), 1, f)
             for s in vpu_streams for i, f in enumerate(s)]
    never = None
    for _, is_vpu, f in sorted(jobs, key=lambda j: j[:2]):
        if is_vpu:
            f(never)
        else:
            y = pltpu.bitcast(f()[-8:, :], _U32)
            never = (y & zero_ref[...]) != 0


def _kernel(ax_hbm, mem_hbm, wq_hbm, wk_hbm, wv_hbm, awo_hbm, bx_hbm, bw_hbm, bwo_hbm,
            out_hbm,
            xa, mem_v, wqkv, awo, xb, bw_raw, bwq, bwkv, bwo, outa, outb,
            q_all, ka, va, kb, vb, oa, ob, hbuf, zero,
            sems, psems, x0sems, wsems, xsems, osems, *, seq, seg, n_mem, heads, dh):
    dm = 1024
    n_blk = seq // _T
    half = heads // 2
    n_grp = n_blk // 2
    piece = bw_raw.shape[1]
    n_piece = dm // 2 // piece

    bx_u = bx_hbm.bitcast(_U32)
    bw_u = bw_hbm.bitcast(_U32)
    bwo_u = bwo_hbm.bitcast(_U32)
    ax_u = ax_hbm.bitcast(_U32)
    awo_u = awo_hbm.bitcast(_U32)

    q_head = seq // 4
    q_rest = (seq - q_head) // n_piece

    def cp_x0(j):
        at = (pl.ds(0, q_head // 2), pl.ds(j * 2 * piece, 2 * piece))
        return pltpu.make_async_copy(bx_u.at[at], xb.at[at], x0sems.at[j])

    def cp_xb(g):
        rows = pl.ds(pl.multiple_of((q_head + g * q_rest) // 2, _T // 2), q_rest // 2)
        return pltpu.make_async_copy(bx_u.at[rows], xb.at[rows], xsems.at[g])

    def cp_bw(j):
        rows = pl.ds(pl.multiple_of(j % n_piece * piece, piece), piece)
        cols = pl.ds(pl.multiple_of(j // n_piece * dm, dm), dm)
        return pltpu.make_async_copy(bw_u.at[rows, cols], bw_raw.at[j], psems.at[j])

    cp_bwo = [pltpu.make_async_copy(bwo_u.at[:, j, :],
                                    bwo.at[(j % 8) * 8 + (j // 16) * 2 + (j // 8) % 2],
                                    sems.at[0])
              for j in range(64)]
    cp_mem = pltpu.make_async_copy(mem_hbm, mem_v, sems.at[1])

    per_grp = half // n_grp

    def cp_w(g):
        return [pltpu.make_async_copy(
                    w.bitcast(_U32).at[:, par * half + g * per_grp + j, :],
                    wqkv.at[2 * (g * per_grp + j) + par, :, m * dh:(m + 1) * dh],
                    wsems.at[g])
                for j in range(per_grp) for par in range(2)
                for m, w in enumerate((wq_hbm, wk_hbm, wv_hbm))]

    def start_a_slice(g):
        for src_ref, dst_ref, sem in ((awo_u, awo, sems.at[2]), (ax_u, xa, sems.at[3])):
            n = dst_ref.shape[0] // n_grp
            rows = pl.ds(pl.multiple_of(g * n, n), n)
            pltpu.make_async_copy(src_ref.at[rows], dst_ref.at[rows], sem).start()

    def split_heads(g):
        def job(j, r, never):
            h = 2 * (g * per_grp + j)
            low = jnp.full((8, 128), 0xFFFF, _U32)
            sh = jnp.full((8, 128), 16, _U32)
            if never is not None:
                low = jnp.where(never, sh, low)
                sh = jnp.where(never, low, sh)
            for rr in range(r, r + 32, 8):
                for m in range(3):
                    even = wqkv[h, rr:rr + 8, m * dh:(m + 1) * dh]
                    odd = wqkv[h + 1, rr:rr + 8, m * dh:(m + 1) * dh]
                    wqkv[h, rr:rr + 8, m * dh:(m + 1) * dh] = (even & low) | (odd << sh)
                    wqkv[h + 1, rr:rr + 8, m * dh:(m + 1) * dh] = (
                        (even >> sh) | ((odd >> sh) << sh))
        return [functools.partial(job, j, r)
                for j in range(per_grp) for r in range(0, dm // 2, 32)]

    def q_group_copies(g):
        return (cp_xb(g), cp_bw(n_piece + 2 * g), cp_bw(n_piece + 2 * g + 1))

    for j in range(n_piece):
        cp_bw(j).start()
        cp_x0(j).start()
    zero[...] = jnp.zeros(zero.shape, _U32)

    cp_bw(0).wait()
    _permute_b_columns(bw_raw.at[0], bwq.at[0])
    for j in range(n_piece):
        cp_x0(j).wait()
        if j + 1 < n_piece:
            cp_bw(j + 1).wait()
        if j >= n_piece - 2:
            for cp in q_group_copies(j - n_piece + 2):
                cp.start()
        x = pltpu.bitcast(xb[0:q_head // 2, j * 2 * piece:(j + 1) * 2 * piece], _BF16)
        y = jnp.dot(x, pltpu.bitcast(bwq[j], _BF16), preferred_element_type=_F32)
        for c in range(8):
            part = y[:, c * 128:(c + 1) * 128]
            q_all[c, 0:q_head, :] = part if j == 0 else q_all[c, 0:q_head, :] + part
        if j + 1 < n_piece:
            _permute_b_columns(bw_raw.at[j + 1], bwq.at[j + 1])

    def q_body(g, carry):
        @pl.when(g + 2 < n_piece)
        def _():
            for cp in q_group_copies(g + 2):
                cp.start()

        @pl.when(g + 1 == n_piece)
        def _():
            for cp in cp_bwo + cp_w(0):
                cp.start()

        for cp in q_group_copies(g):
            cp.wait()
        r0 = pl.multiple_of(q_head + g * q_rest, _T)
        x = pltpu.bitcast(xb[pl.ds(pl.multiple_of(r0 // 2, _T // 2), q_rest // 2), :], _BF16)
        w = pltpu.bitcast(bwq[...].reshape(dm // 2, dm), _BF16)
        y = jnp.dot(x, w, preferred_element_type=_F32)
        for c in range(8):
            q_all[c, pl.ds(r0, q_rest), :] = y[:, c * 128:(c + 1) * 128]
        for j in (2 * g, 2 * g + 1):
            _permute_b_columns(bw_raw.at[n_piece + j], bwkv.at[j])
        return carry

    lax.fori_loop(0, n_piece, q_body, 0)

    def b_proj(r0, s, dst):
        def job(c):
            x = xb[pl.ds(pl.multiple_of(r0 // 2, _T // 2), _T // 2), :]
            w = bwkv[s * n_piece:(s + 1) * n_piece, :, c * 128:(c + 1) * 128]
            y = jnp.dot(pltpu.bitcast(x, _BF16),
                        pltpu.bitcast(w.reshape(dm // 2, 128), _BF16),
                        preferred_element_type=_F32)
            dst[c, _HALO:_HALO + _T, :] = y
            return y
        return [functools.partial(job, c) for c in range(8)]

    def b_halo(src, dst):
        dst[:, 0:_HALO, :] = src[:, _T:_T + _HALO, :]

    def b_out(o_ref, r0):
        def job(c):
            w = bwo[:, :, c * 128:(c + 1) * 128].reshape(dm // 2, 128)
            y = jnp.dot(o_ref[...], pltpu.bitcast(w, _BF16), preferred_element_type=_F32)
            outb[pl.ds(pl.multiple_of(r0, _T), _T), c * 128:(c + 1) * 128] = y.astype(_BF16)
            return y
        return [functools.partial(job, c) for c in range(8)]

    def b_attention(r0, bufs, first_block):
        q_ref = q_all.at[:, pl.ds(pl.multiple_of(r0, _T), _T), :]
        stages = (
            lambda x, r, never: _b_lane_sum(_b_products(q_ref, bufs[0], r, never), 1),
            lambda x, r, never: _b_lane_sum(x, 16),
            lambda x, r, never: _b_softmax(x, r, first_block),
            lambda x, r, never: _b_values(x, bufs[1], bufs[2], r),
        )
        state = {}

        def job(stage, r, never):
            state[r] = stages[stage](state.get(r), r, never)

        order = sorted((i + s, -s, i) for i in range(_T // _CH) for s in range(4))
        return [functools.partial(job, -s, i * _CH) for _, s, i in order]

    for cp in cp_w(1):
        cp.start()
    cp_mem.start()
    _paced(zero, b_proj(0, 0, ka) + b_proj(0, 1, va))
    ka[:, 0:_HALO, :] = jnp.broadcast_to(ka[:, _HALO:_HALO + 1, :], (8, _HALO, 128))
    va[:, 0:_HALO, :] = jnp.broadcast_to(va[:, _HALO:_HALO + 1, :], (8, _HALO, 128))

    def b_step(r0, cur, nxt, extra=(), first_block=False, last_block=False):
        mxu = []
        if not first_block:
            mxu += b_out(nxt[2], r0 - _T)
        if not last_block:
            for s in range(2):
                b_halo(cur[s], nxt[s])
                mxu += b_proj(r0 + _T, s, nxt[s])
        _paced(zero, mxu, b_attention(r0, cur, first_block), list(extra), span=_SPAN)

    set_a = (ka, va, oa)
    set_b = (kb, vb, ob)
    b_step(0, set_a, set_b, first_block=True)
    for cp in cp_bwo:
        cp.wait()

    def b_body(i, carry):
        @pl.when(i + 2 < n_grp)
        def _():
            for cp in cp_w(i + 2):
                cp.start()

        start_a_slice(i)
        for cp in cp_w(i):
            cp.wait()
        r0 = (2 * i + 1) * _T
        split = split_heads(i)
        b_step(r0, set_b, set_a, split[:len(split) // 2])
        b_step(r0 + _T, set_a, set_b, split[len(split) // 2:])
        return carry

    lax.fori_loop(0, n_grp - 1, b_body, 0)
    start_a_slice(n_grp - 1)
    for cp in cp_w(n_grp - 1):
        cp.wait()
    b_step(seq - _T, set_b, set_a, split_heads(n_grp - 1), last_block=True)
    _paced(zero, b_out(ob, seq - _T))

    cp_outb = pltpu.make_async_copy(outb, out_hbm.at[:, dm:2 * dm], osems.at[0])
    cp_outb.start()

    pltpu.make_async_copy(awo_u, awo, sems.at[2]).wait()
    pltpu.make_async_copy(ax_u, xa, sems.at[3]).wait()
    cp_mem.wait()

    rows = n_mem + seg
    scale = dh ** -0.5
    hbuf[0:n_mem, :] = mem_v[...].astype(_F32)

    def a_step(s):
        qi = lax.broadcasted_iota(jnp.int32, (rows, 128), 0)
        ki = lax.broadcasted_iota(jnp.int32, (rows, 128), 1)
        real = ki < rows
        mask = ((qi < n_mem) | (qi >= ki)) & real
        fill = jnp.where(real, _MASKED, -jnp.inf).astype(_F32)
        pad = jnp.zeros((128 - rows, dh), _F32)

        xs = xa[pl.ds(pl.multiple_of(s * (seg // 2), seg // 2), seg // 2), :]
        hbuf[n_mem:rows, :] = pltpu.bitcast(xs, _BF16).astype(_F32)

        def project(h, c0, c1):
            w = wqkv[h, :, c0 * dh:c1 * dh]
            return jnp.dot(hbuf[...], pltpu.bitcast(w, _BF16), preferred_element_type=_F32)

        def probs(qk):
            k = jnp.concatenate([qk[:, dh:2 * dh], pad], axis=0).astype(_BF16)
            sc = lax.dot_general(qk[:, 0:dh], k, _NT, preferred_element_type=_F32)
            sc = jnp.where(mask, sc * scale, fill)
            e = jnp.exp(sc - jnp.max(sc, axis=-1, keepdims=True))
            return e / jnp.sum(e, axis=-1, keepdims=True)

        def values(p, v):
            v = jnp.concatenate([v, pad], axis=0).astype(_BF16)
            return jnp.dot(p, v, preferred_element_type=_F32)

        def out_proj(h0, h1):
            w = pltpu.bitcast(awo[h0 * dh // 2:h1 * dh // 2, :], _BF16)
            lhs = jnp.concatenate([o[h] for h in range(h0, h1)], axis=1)
            return jnp.dot(lhs, w, preferred_element_type=_F32)

        qk, v, p, o = {}, {}, {}, {}
        cuts = [c * heads // 32 for c in _O_CUTS]
        acc = None
        for t in range(heads + _PV_LAG):
            if t < heads:
                qk[t] = project(t, 0, 2)
            if 0 <= t - _V_LAG < heads:
                v[t - _V_LAG] = project(t - _V_LAG, 2, 3)
            if heads <= t < heads + len(cuts) - 1:
                part = out_proj(cuts[t - heads], cuts[t - heads + 1])
                acc = part if acc is None else acc + part
            if 1 <= t <= heads:
                p[t - 1] = probs(qk[t - 1])
            if t >= _PV_LAG:
                o[t - _PV_LAG] = values(p[t - _PV_LAG], v[t - _PV_LAG])
        acc = acc + out_proj(cuts[-1], heads)

        hbuf[0:n_mem, :] = acc[0:n_mem]
        outa[pl.ds(pl.multiple_of(s * seg, seg), seg), :] = acc[n_mem:rows].astype(_BF16)

    def a_body(i, carry):
        for u in range(_A_UNROLL):
            a_step(i * _A_UNROLL + u)
        n = _A_UNROLL * seg
        done = pl.ds(pl.multiple_of(i * n, n), n)
        pltpu.make_async_copy(outa.at[done], out_hbm.at[done, 0:dm], osems.at[1]).start()
        return carry

    lax.fori_loop(0, seq // (seg * _A_UNROLL), a_body, 0)
    cp_outb.wait()
    pltpu.make_async_copy(outa, out_hbm.at[:, 0:dm], osems.at[1]).wait()


@functools.partial(jax.jit, static_argnames=("A_seg_len",))
def pallas_concat_heads__memory_aug_recurrent_mem_tr__sliding_local_dilated__prompt_kernel(
    A_x: jax.Array,
    A_mem0: jax.Array,
    A_Wq: jax.Array,
    A_Wk: jax.Array,
    A_Wv: jax.Array,
    A_Wo: jax.Array,
    A_seg_len: int,
    B_x: jax.Array,
    B_wqkv: jax.Array,
    B_wo: jax.Array,
):
    batch, seq, dm = A_x.shape
    heads, dh = A_Wq.shape[1], A_Wq.shape[2]
    n_mem = A_mem0.shape[1]
    seg = int(A_seg_len)
    assert batch == 1 and dm == 1024 and dh == 128 and heads % 8 == 0
    assert B_x.shape == (1, seq, dm) and B_wqkv.shape == (dm, 3 * dm)
    assert seg % 16 == 0 and seq % (seg * _A_UNROLL) == 0 and n_mem % 8 == 0 and n_mem + seg <= 128
    assert seq % (2 * _T) == 0 and (heads // 2) % (seq // (2 * _T)) == 0
    rows = n_mem + seg

    n_grp = seq // (2 * _T)
    n_piece = 4
    piece = dm // 2 // n_piece
    assert seq % (4 * n_piece * _T) == 0
    kv_buf = pltpu.VMEM((8, _HALO + _T, 128), _F32)
    o_buf = pltpu.VMEM((_T, dm), _F32)
    out = pl.pallas_call(
        functools.partial(_kernel, seq=seq, seg=seg, n_mem=n_mem, heads=heads, dh=dh),
        out_shape=jax.ShapeDtypeStruct((seq, 2 * dm), _BF16),
        in_specs=[pl.BlockSpec(memory_space=pl.ANY)] * 9,
        out_specs=pl.BlockSpec(memory_space=pl.ANY),
        scratch_shapes=[
            pltpu.VMEM((seq // 2, dm), _U32),
            pltpu.VMEM((n_mem, dm), _BF16),
            pltpu.VMEM((heads, dm // 2, 3 * dh), _U32),
            pltpu.VMEM((heads * dh // 2, dm), _U32),
            pltpu.VMEM((seq // 2, dm), _U32),
            pltpu.VMEM((3 * n_piece, piece, dm), _U32),
            pltpu.VMEM((n_piece, piece, dm), _U32),
            pltpu.VMEM((2 * n_piece, piece, dm), _U32),
            pltpu.VMEM((64, 8, dm), _U32),
            pltpu.VMEM((seq, dm), _BF16),
            pltpu.VMEM((seq, dm), _BF16),
            pltpu.VMEM((8, seq, 128), _F32),
            kv_buf, kv_buf, kv_buf, kv_buf, o_buf, o_buf,
            pltpu.VMEM((rows, dm), _F32),
            pltpu.VMEM((8, 128), _U32),
            pltpu.SemaphoreType.DMA((4,)),
            pltpu.SemaphoreType.DMA((3 * n_piece,)),
            pltpu.SemaphoreType.DMA((n_piece,)),
            pltpu.SemaphoreType.DMA((n_grp,)),
            pltpu.SemaphoreType.DMA((n_piece,)),
            pltpu.SemaphoreType.DMA((2,)),
        ],
        compiler_params=pltpu.CompilerParams(vmem_limit_bytes=110 * 1024 * 1024),
    )(
        A_x.reshape(seq, dm),
        A_mem0.reshape(n_mem, dm),
        A_Wq.reshape(dm // 2, 2 * heads, dh),
        A_Wk.reshape(dm // 2, 2 * heads, dh),
        A_Wv.reshape(dm // 2, 2 * heads, dh),
        A_Wo.reshape(heads * dh, dm),
        B_x.reshape(seq, dm),
        B_wqkv,
        B_wo.reshape(8, dm // 8, dm),
    )
    return out.reshape(1, seq, 2 * dm)
```

```python
import functools

import jax
import jax.numpy as jnp
from jax import lax
from jax.experimental import pallas as pl
from jax.experimental.pallas import tpu as pltpu

_F32 = jnp.float32
_BF16 = jnp.bfloat16
_U32 = jnp.uint32
_NT = (((1,), (1,)), ((), ()))
_LOG2E = 1.4426950408889634
_MASKED = -1000000000.0

_B_HEADS = 32
_B_WIN = 8
_B_DIL = 2
_HALO = 16
_T = 256
_CH = 8

_PV_LAG = 3
_V_LAG = 1
_SIDE_LAG = 1
_MID = 0
_O_CUTS = (0, 8, 16, 24)


def _permute_b_columns(src_ref, dst_ref):
    rows, lag = 16, 2
    field = (lax.broadcasted_iota(jnp.int32, (rows, 128), 1) >> 1) & 7
    bits = [(field & (1 << b)) != 0 for b in range(3)]

    def spread(r):
        t = [src_ref[r:r + rows, c * 128:(c + 1) * 128] for c in range(8)]
        return [t[c] if c == 0 else pltpu.roll(t[c], 2 * c, 1) for c in range(8)]

    def exchange(t):
        t = [t[-c % 8] for c in range(8)]
        for b in range(3):
            t = [jnp.where(bits[b], t[(c - (1 << b)) % 8], t[c]) for c in range(8)]
        return [t[c] if c == 0 else pltpu.roll(t[c], 128 - 2 * c, 1) for c in range(8)]

    n = src_ref.shape[0] // rows
    first, second = {}, {}
    for i in range(n + 2 * lag):
        if i < n:
            first[i] = spread(i * rows)
        if 0 <= i - lag < n:
            second[i - lag] = exchange(first.pop(i - lag))
        if 0 <= i - 2 * lag < n:
            r = (i - 2 * lag) * rows
            for c, y in enumerate(second.pop(i - 2 * lag)):
                dst_ref[r:r + rows, c * 128:(c + 1) * 128] = y


def _b_products(q_ref, k_ref, r, never):
    logits = [None] * _B_WIN
    for c in range(8):
        q = q_ref[c, r:r + _CH, :]
        if c % 4 == 0:
            q = jnp.where(never, 0.0, q)
        for w in range(_B_WIN):
            a = _HALO + r - _B_DIL * w
            pr = q * k_ref[c, a:a + _CH, :]
            logits[w] = pr if logits[w] is None else logits[w] + pr
    return logits


def _b_lane_sum(xs, step):
    upper = (lax.broadcasted_iota(jnp.int32, (_CH, 128), 1) & step) != 0
    return [x + jnp.where(upper, pltpu.roll(x, step, 1), pltpu.roll(x, 128 - step, 1))
            for x in xs]


def _b_softmax(logits, t0, r):
    scale = (1024 // _B_HEADS) ** -0.5
    if r < _B_DIL * (_B_WIN - 1):
        tok = t0 + r + lax.broadcasted_iota(jnp.int32, (_CH, 128), 0)
        logits = [jnp.where(tok >= _B_DIL * w, x, _MASKED / scale) if r < _B_DIL * w else x
                  for w, x in enumerate(logits)]
    m = functools.reduce(jnp.maximum, logits)
    es = [jnp.exp2((x - m) * (scale * _LOG2E)) for x in logits]
    inv = 1.0 / functools.reduce(jnp.add, es)
    return [e * inv for e in es]


def _b_values(ps, v_ref, o_ref, r):
    for c in range(8):
        acc = None
        for w in range(_B_WIN):
            a = _HALO + r - _B_DIL * w
            pr = ps[w] * v_ref[c, a:a + _CH, :]
            acc = pr if acc is None else acc + pr
        o_ref[r:r + _CH, c * 128:(c + 1) * 128] = acc.astype(o_ref.dtype)
    return [acc]


def _never(zero_ref, y):
    return (pltpu.bitcast(y[-8:, -128:], _U32) & zero_ref[...]) != 0


def _kernel(ax_hbm, mem_hbm, wq_hbm, wk_hbm, wv_hbm, awo_hbm, bx_hbm, bw_hbm, bwo_hbm,
            out_hbm,
            xa, mem_v, wqkv, awo, xb, bw_raw, bwq, bwkv, bwo, res,
            q_all, k_all, v_all, ob, hbuf, zero,
            sems, psems, x0sems, wsems, xsems, *, seq, seg, n_mem, heads, dh):
    dm = 1024
    half = heads // 2
    n_grp = seq // _T
    piece = bw_raw.shape[1]
    n_piece = dm // 2 // piece

    bx_u = bx_hbm.bitcast(_U32)
    bw_u = bw_hbm.bitcast(_U32)
    bwo_u = bwo_hbm.bitcast(_U32)
    ax_u = ax_hbm.bitcast(_U32)
    awo_u = awo_hbm.bitcast(_U32)

    q_head = seq // 4
    q_rest = (seq - q_head) // n_piece

    def cp_x0(j):
        at = (pl.ds(0, q_head // 2), pl.ds(j * 2 * piece, 2 * piece))
        return pltpu.make_async_copy(bx_u.at[at], xb.at[at], x0sems.at[j])

    def cp_xb(g):
        rows = pl.ds(pl.multiple_of((q_head + g * q_rest) // 2, 64), q_rest // 2)
        return pltpu.make_async_copy(bx_u.at[rows], xb.at[rows], xsems.at[g])

    def cp_bw(j):
        rows = pl.ds(pl.multiple_of(j % n_piece * piece, piece), piece)
        cols = pl.ds(pl.multiple_of(j // n_piece * dm, dm), dm)
        return pltpu.make_async_copy(bw_u.at[rows, cols], bw_raw.at[j], psems.at[j])

    cp_bwo = [pltpu.make_async_copy(bwo_u.at[:, j, :],
                                    bwo.at[(j % 8) * 8 + (j // 16) * 2 + (j // 8) % 2],
                                    sems.at[0])
              for j in range(64)]
    cp_mem = pltpu.make_async_copy(mem_hbm, mem_v, sems.at[1])

    per_grp = half // n_grp

    def cp_w(g):
        return [pltpu.make_async_copy(
                    w.bitcast(_U32).at[:, par * half + g * per_grp + j, :],
                    wqkv.at[2 * (g * per_grp + j) + par, :, m * dh:(m + 1) * dh],
                    wsems.at[g])
                for j in range(per_grp) for par in range(2)
                for m, w in enumerate((wq_hbm, wk_hbm, wv_hbm))]

    def start_a_slice(g):
        for src_ref, dst_ref, sem in ((awo_u, awo, sems.at[2]), (ax_u, xa, sems.at[3])):
            n = dst_ref.shape[0] // n_grp
            rows = pl.ds(pl.multiple_of(g * n, n), n)
            pltpu.make_async_copy(src_ref.at[rows], dst_ref.at[rows], sem).start()

    def split_heads(g):
        def job(j, r, never):
            h = 2 * (g * per_grp + j)
            low = jnp.where(never, 16, jnp.full((8, 128), 0xFFFF, _U32))
            sh = jnp.where(never, low, 16)
            for rr in range(r, r + 64, 8):
                for m in range(3):
                    even = wqkv[h, rr:rr + 8, m * dh:(m + 1) * dh]
                    odd = wqkv[h + 1, rr:rr + 8, m * dh:(m + 1) * dh]
                    wqkv[h, rr:rr + 8, m * dh:(m + 1) * dh] = (even & low) | (odd << sh)
                    wqkv[h + 1, rr:rr + 8, m * dh:(m + 1) * dh] = (
                        (even >> sh) | ((odd >> sh) << sh))
        return [functools.partial(job, j, r)
                for j in range(per_grp) for r in range(0, dm // 2, 64)]

    def q_group_copies(g):
        return (cp_xb(g), cp_bw(n_piece + 2 * g), cp_bw(n_piece + 2 * g + 1))

    for j in range(n_piece):
        cp_bw(j).start()
        cp_x0(j).start()
    zero[...] = jnp.zeros(zero.shape, _U32)

    cp_bw(0).wait()
    _permute_b_columns(bw_raw.at[0], bwq.at[0])
    for j in range(n_piece):
        cp_x0(j).wait()
        if j + 1 < n_piece:
            cp_bw(j + 1).wait()
        if j >= n_piece - 2:
            for cp in q_group_copies(j - n_piece + 2):
                cp.start()
        x = pltpu.bitcast(xb[0:q_head // 2, j * 2 * piece:(j + 1) * 2 * piece], _BF16)
        y = jnp.dot(x, pltpu.bitcast(bwq[j], _BF16), preferred_element_type=_F32)
        for c in range(8):
            part = y[:, c * 128:(c + 1) * 128]
            q_all[c, 0:q_head, :] = part if j == 0 else q_all[c, 0:q_head, :] + part
        if j + 1 < n_piece:
            _permute_b_columns(bw_raw.at[j + 1], bwq.at[j + 1])

    def q_body(g, carry):
        @pl.when(g + 2 < n_piece)
        def _():
            for cp in q_group_copies(g + 2):
                cp.start()

        @pl.when((g >= 1) & (g <= 2))
        def _():
            for cp in cp_w(g - 1):
                cp.start()

        @pl.when(g + 1 == n_piece)
        def _():
            for cp in cp_bwo + [cp_mem]:
                cp.start()

        for cp in q_group_copies(g):
            cp.wait()
        r0 = pl.multiple_of(q_head + g * q_rest, 128)
        x = pltpu.bitcast(xb[pl.ds(pl.multiple_of(r0 // 2, 64), q_rest // 2), :], _BF16)
        w = pltpu.bitcast(bwq[...].reshape(dm // 2, dm), _BF16)
        y = jnp.dot(x, w, preferred_element_type=_F32)
        for c in range(8):
            q_all[c, pl.ds(r0, q_rest), :] = y[:, c * 128:(c + 1) * 128]
        for j in (2 * g, 2 * g + 1):
            _permute_b_columns(bw_raw.at[n_piece + j], bwkv.at[j])
        return carry

    lax.fori_loop(0, n_piece, q_body, 0)

    def kv_body(g, carry):
        @pl.when(g + 2 < n_grp)
        def _():
            for cp in cp_w(g + 2):
                cp.start()

        start_a_slice(g)
        for cp in cp_w(g):
            cp.wait()
        split = split_heads(g)
        r0 = pl.multiple_of(g * _T, _T)
        for j in range(16):
            s, c = divmod(j, 8)
            x = xb[pl.ds(pl.multiple_of(r0 // 2, _T // 2), _T // 2), :]
            w = bwkv[s * n_piece:(s + 1) * n_piece, :, c * 128:(c + 1) * 128]
            y = jnp.dot(pltpu.bitcast(x, _BF16),
                        pltpu.bitcast(w.reshape(dm // 2, 128), _BF16),
                        preferred_element_type=_F32)
            (k_all, v_all)[s][c, pl.ds(_HALO + r0, _T), :] = y
            if j < 15:
                never = _never(zero, y)
                for job in split[j * len(split) // 15:(j + 1) * len(split) // 15]:
                    job(never)
        return carry

    lax.fori_loop(0, n_grp, kv_body, 0)
    for ref in (k_all, v_all):
        ref[:, 0:_HALO, :] = jnp.broadcast_to(ref[:, _HALO:_HALO + 1, :], (8, _HALO, 128))

    def b_attention(t0, n):
        q_ref = q_all.at[:, pl.ds(t0, n), :]
        k_ref = k_all.at[:, pl.ds(t0, _HALO + n), :]
        v_ref = v_all.at[:, pl.ds(t0, _HALO + n), :]
        stages = (
            lambda x, r, never: _b_lane_sum(_b_products(q_ref, k_ref, r, never), 1),
            lambda x, r, never: _b_lane_sum(x, 16),
            lambda x, r, never: _b_softmax(x, t0, r),
            lambda x, r, never: _b_values(x, v_ref, ob, r),
        )
        state = {}

        def job(stage, r, never):
            state[r] = stages[stage](state.get(r), r, never)
            return state[r][-1]

        return [functools.partial(job, s, r) for r in range(0, n, _CH) for s in range(4)]

    pltpu.make_async_copy(awo_u, awo, sems.at[2]).wait()
    pltpu.make_async_copy(ax_u, xa, sems.at[3]).wait()
    for cp in cp_bwo + [cp_mem]:
        cp.wait()

    rows = n_mem + seg
    scale = dh ** -0.5
    hbuf[0:n_mem, :] = mem_v[...].astype(_F32)

    def a_step(s, side_jobs=(), mid=None):
        qi = lax.broadcasted_iota(jnp.int32, (rows, 128), 0)
        ki = lax.broadcasted_iota(jnp.int32, (rows, 128), 1)
        real = ki < rows
        mask = ((qi < n_mem) | (qi >= ki)) & real
        fill = jnp.where(real, _MASKED, -jnp.inf).astype(_F32)
        pad = jnp.zeros((128 - rows, dh), _F32)

        xs = xa[pl.ds(pl.multiple_of(s * (seg // 2), seg // 2), seg // 2), :]
        hbuf[n_mem:rows, :] = pltpu.bitcast(xs, _BF16).astype(_F32)

        def project(h, c0, c1):
            w = wqkv[h, :, c0 * dh:c1 * dh]
            return jnp.dot(hbuf[...], pltpu.bitcast(w, _BF16), preferred_element_type=_F32)

        def probs(qk, after):
            k = jnp.concatenate([qk[:, dh:2 * dh], pad], axis=0).astype(_BF16)
            sc = lax.dot_general(qk[:, 0:dh], k, _NT, preferred_element_type=_F32)
            low = fill
            if after is not None:
                low = jnp.concatenate(
                    [jnp.where(_never(zero, after), 0.0, fill[0:8])] * (rows // 8), axis=0)
            sc = jnp.where(mask, sc * scale, low)
            e = jnp.exp(sc - jnp.max(sc, axis=-1, keepdims=True))
            return e / jnp.sum(e, axis=-1, keepdims=True)

        def values(p, v):
            v = jnp.concatenate([v, pad], axis=0).astype(_BF16)
            return jnp.dot(p, v, preferred_element_type=_F32)

        def out_proj(h0, h1):
            w = pltpu.bitcast(awo[h0 * dh // 2:h1 * dh // 2, :], _BF16)
            lhs = jnp.concatenate([o[h] for h in range(h0, h1)], axis=1)
            return jnp.dot(lhs, w, preferred_element_type=_F32)

        qk, v, p, o, side = {}, {}, {}, {}, {}
        cuts = [c * heads // 32 for c in _O_CUTS]
        acc = None
        for t in range(heads + _PV_LAG):
            if t < heads:
                qk[t] = project(t, 0, 2)
            if 0 <= t - _V_LAG < heads:
                v[t - _V_LAG] = project(t - _V_LAG, 2, 3)
            if heads <= t < heads + len(cuts) - 1:
                part = out_proj(cuts[t - heads], cuts[t - heads + 1])
                acc = part if acc is None else acc + part
            if 1 <= t <= heads:
                p[t - 1] = probs(qk[t - 1], side.get(t - _SIDE_LAG))
            if t >= _PV_LAG:
                o[t - _PV_LAG] = values(p[t - _PV_LAG], v[t - _PV_LAG])
            if t < heads:
                for job in side_jobs[t * len(side_jobs) // heads:
                                     (t + 1) * len(side_jobs) // heads]:
                    side[t] = job(_never(zero, qk[t]))
        if mid is not None:
            mid()
        acc = acc + out_proj(cuts[-1], heads)

        hbuf[0:n_mem, :] = acc[0:n_mem]
        res[pl.ds(pl.multiple_of(s * seg, seg), seg), 0:dm] = acc[n_mem:rows].astype(_BF16)

    def a_body(i, carry):
        toks = pl.ds(pl.multiple_of(i * 2 * seg, 2 * seg), 2 * seg)

        def b_out(c0, c1):
            if c1 > c0:
                w = bwo[:, :, c0 * 128:c1 * 128].reshape(dm // 2, (c1 - c0) * 128)
                y = jnp.dot(ob[...], pltpu.bitcast(w, _BF16), preferred_element_type=_F32)
                res[toks, dm + c0 * 128:dm + c1 * 128] = y.astype(_BF16)

        a_step(2 * i, b_attention(toks.start, 2 * seg), functools.partial(b_out, 0, _MID))
        b_out(_MID, 8)
        a_step(2 * i + 1)
        pltpu.make_async_copy(res.at[toks], out_hbm.at[toks], sems.at[4]).start()
        return carry

    lax.fori_loop(0, seq // (2 * seg), a_body, 0)
    pltpu.make_async_copy(res, out_hbm, sems.at[4]).wait()


@functools.partial(jax.jit, static_argnames=("A_seg_len",))
def pallas_concat_heads__memory_aug_recurrent_mem_tr__sliding_local_dilated__prompt_kernel(
    A_x: jax.Array,
    A_mem0: jax.Array,
    A_Wq: jax.Array,
    A_Wk: jax.Array,
    A_Wv: jax.Array,
    A_Wo: jax.Array,
    A_seg_len: int,
    B_x: jax.Array,
    B_wqkv: jax.Array,
    B_wo: jax.Array,
):
    batch, seq, dm = A_x.shape
    heads, dh = A_Wq.shape[1], A_Wq.shape[2]
    n_mem = A_mem0.shape[1]
    seg = int(A_seg_len)
    assert batch == 1 and dm == 1024 and dh == 128 and heads % 8 == 0
    assert B_x.shape == (1, seq, dm) and B_wqkv.shape == (dm, 3 * dm)
    assert seg % 16 == 0 and seq % (2 * seg) == 0 and n_mem % 8 == 0 and n_mem + seg <= 128
    assert seq % _T == 0 and (heads // 2) % (seq // _T) == 0
    rows = n_mem + seg

    n_grp = seq // _T
    n_piece = 4
    piece = dm // 2 // n_piece
    assert seq % (4 * n_piece * 128) == 0
    out = pl.pallas_call(
        functools.partial(_kernel, seq=seq, seg=seg, n_mem=n_mem, heads=heads, dh=dh),
        out_shape=jax.ShapeDtypeStruct((seq, 2 * dm), _BF16),
        in_specs=[pl.BlockSpec(memory_space=pl.ANY)] * 9,
        out_specs=pl.BlockSpec(memory_space=pl.ANY),
        scratch_shapes=[
            pltpu.VMEM((seq // 2, dm), _U32),
            pltpu.VMEM((n_mem, dm), _BF16),
            pltpu.VMEM((heads, dm // 2, 3 * dh), _U32),
            pltpu.VMEM((heads * dh // 2, dm), _U32),
            pltpu.VMEM((seq // 2, dm), _U32),
            pltpu.VMEM((3 * n_piece, piece, dm), _U32),
            pltpu.VMEM((n_piece, piece, dm), _U32),
            pltpu.VMEM((2 * n_piece, piece, dm), _U32),
            pltpu.VMEM((64, 8, dm), _U32),
            pltpu.VMEM((seq, 2 * dm), _BF16),
            pltpu.VMEM((8, seq, 128), _F32),
            pltpu.VMEM((8, _HALO + seq, 128), _F32),
            pltpu.VMEM((8, _HALO + seq, 128), _F32),
            pltpu.VMEM((2 * seg, dm), _F32),
            pltpu.VMEM((rows, dm), _F32),
            pltpu.VMEM((8, 128), _U32),
            pltpu.SemaphoreType.DMA((5,)),
            pltpu.SemaphoreType.DMA((3 * n_piece,)),
            pltpu.SemaphoreType.DMA((n_piece,)),
            pltpu.SemaphoreType.DMA((n_grp,)),
            pltpu.SemaphoreType.DMA((n_piece,)),
        ],
        compiler_params=pltpu.CompilerParams(vmem_limit_bytes=110 * 1024 * 1024),
    )(
        A_x.reshape(seq, dm),
        A_mem0.reshape(n_mem, dm),
        A_Wq.reshape(dm // 2, 2 * heads, dh),
        A_Wk.reshape(dm // 2, 2 * heads, dh),
        A_Wv.reshape(dm // 2, 2 * heads, dh),
        A_Wo.reshape(heads * dh, dm),
        B_x.reshape(seq, dm),
        B_wqkv,
        B_wo.reshape(8, dm // 8, dm),
    )
    return out.reshape(1, seq, 2 * dm)
```

```python
import functools

import jax
import jax.numpy as jnp
from jax import lax
from jax.experimental import pallas as pl
from jax.experimental.pallas import tpu as pltpu

_F32 = jnp.float32
_BF16 = jnp.bfloat16
_U32 = jnp.uint32
_NT = (((1,), (1,)), ((), ()))
_LOG2E = 1.4426950408889634
_MASKED = -1000000000.0

_B_HEADS = 32
_B_WIN = 8
_B_DIL = 2
_HALO = 16
_T = 256
_CH = 8

_V_LAG = 1
_PV_LAG = 3


def _permute_b_columns(src_ref, dst_ref):
    rows, lag = 16, 2
    field = (lax.broadcasted_iota(jnp.int32, (rows, 128), 1) >> 1) & 7
    bits = [(field & (1 << b)) != 0 for b in range(3)]

    def spread(r):
        t = [src_ref[r:r + rows, c * 128:(c + 1) * 128] for c in range(8)]
        return [t[c] if c == 0 else pltpu.roll(t[c], 2 * c, 1) for c in range(8)]

    def exchange(t):
        t = [t[-c % 8] for c in range(8)]
        for b in range(3):
            t = [jnp.where(bits[b], t[(c - (1 << b)) % 8], t[c]) for c in range(8)]
        return [t[c] if c == 0 else pltpu.roll(t[c], 128 - 2 * c, 1) for c in range(8)]

    n = src_ref.shape[0] // rows
    first, second = {}, {}
    for i in range(n + 2 * lag):
        if i < n:
            first[i] = spread(i * rows)
        if 0 <= i - lag < n:
            second[i - lag] = exchange(first.pop(i - lag))
        if 0 <= i - 2 * lag < n:
            r = (i - 2 * lag) * rows
            for c, y in enumerate(second.pop(i - 2 * lag)):
                dst_ref[r:r + rows, c * 128:(c + 1) * 128] = y


def _b_products(q_ref, k_ref, r, never):
    logits = [None] * _B_WIN
    for c in range(8):
        q = q_ref[c, r:r + _CH, :]
        if c % 4 == 0:
            q = jnp.where(never, 0.0, q)
        for w in range(_B_WIN):
            a = _HALO + r - _B_DIL * w
            pr = q * k_ref[c, a:a + _CH, :]
            logits[w] = pr if logits[w] is None else logits[w] + pr
    return logits


def _b_lane_sum(xs, step):
    upper = (lax.broadcasted_iota(jnp.int32, (_CH, 128), 1) & step) != 0
    return [x + jnp.where(upper, pltpu.roll(x, step, 1), pltpu.roll(x, 128 - step, 1))
            for x in xs]


def _b_softmax(logits, t0, r):
    scale = (1024 // _B_HEADS) ** -0.5
    if r < _B_DIL * (_B_WIN - 1):
        tok = t0 + r + lax.broadcasted_iota(jnp.int32, (_CH, 128), 0)
        logits = [jnp.where(tok >= _B_DIL * w, x, _MASKED / scale) if r < _B_DIL * w else x
                  for w, x in enumerate(logits)]
    m = functools.reduce(jnp.maximum, logits)
    es = [jnp.exp2((x - m) * (scale * _LOG2E)) for x in logits]
    inv = 1.0 / functools.reduce(jnp.add, es)
    return [e * inv for e in es]


def _b_values(ps, v_ref, o_ref, r):
    for c in range(8):
        acc = None
        for w in range(_B_WIN):
            a = _HALO + r - _B_DIL * w
            pr = ps[w] * v_ref[c, a:a + _CH, :]
            acc = pr if acc is None else acc + pr
        o_ref[r:r + _CH, c * 128:(c + 1) * 128] = acc
    return [acc]


def _never(zero_ref, y):
    return (pltpu.bitcast(y[-8:, -128:], _U32) & zero_ref[...]) != 0


def _kernel(ax_hbm, mem_hbm, wq_hbm, wk_hbm, wv_hbm, awo_hbm, bx_hbm, bw_hbm, bwo_hbm,
            out_hbm,
            xa, mem_v, wqkv, awo, xb, bw_raw, bwq, bwkv, bwo, res,
            q_all, k_all, v_all, ob, hbuf, zero,
            sems, psems, x0sems, wsems, xsems, *, seq, seg, n_mem, heads, dh):
    dm = 1024
    half = heads // 2
    n_grp = seq // _T
    piece = bw_raw.shape[1]
    n_piece = dm // 2 // piece

    bx_u = bx_hbm.bitcast(_U32)
    bw_u = bw_hbm.bitcast(_U32)
    bwo_u = bwo_hbm.bitcast(_U32)
    ax_u = ax_hbm.bitcast(_U32)
    awo_u = awo_hbm.bitcast(_U32)

    q_head = seq // 4
    q_rest = (seq - q_head) // n_piece

    def cp_x0(j):
        at = (pl.ds(0, q_head // 2), pl.ds(j * 2 * piece, 2 * piece))
        return pltpu.make_async_copy(bx_u.at[at], xb.at[at], x0sems.at[j])

    def cp_xb(g):
        rows = pl.ds(pl.multiple_of((q_head + g * q_rest) // 2, 64), q_rest // 2)
        return pltpu.make_async_copy(bx_u.at[rows], xb.at[rows], xsems.at[g])

    def cp_bw(j):
        rows = pl.ds(pl.multiple_of(j % n_piece * piece, piece), piece)
        cols = pl.ds(pl.multiple_of(j // n_piece * dm, dm), dm)
        return pltpu.make_async_copy(bw_u.at[rows, cols], bw_raw.at[j], psems.at[j])

    cp_bwo = [pltpu.make_async_copy(bwo_u.at[:, j, :],
                                    bwo.at[(j % 8) * 8 + (j // 16) * 2 + (j // 8) % 2],
                                    sems.at[0])
              for j in range(64)]
    cp_mem = pltpu.make_async_copy(mem_hbm, mem_v, sems.at[1])

    per_grp = half // n_grp

    def cp_w(g):
        return [pltpu.make_async_copy(
                    w.bitcast(_U32).at[:, par * half + g * per_grp + j, :],
                    wqkv.at[2 * (g * per_grp + j) + par, :, m * dh:(m + 1) * dh],
                    wsems.at[g])
                for j in range(per_grp) for par in range(2)
                for m, w in enumerate((wq_hbm, wk_hbm, wv_hbm))]

    def start_a_slice(g):
        for src_ref, dst_ref, sem in ((awo_u, awo, sems.at[2]), (ax_u, xa, sems.at[3])):
            n = dst_ref.shape[0] // n_grp
            rows = pl.ds(pl.multiple_of(g * n, n), n)
            pltpu.make_async_copy(src_ref.at[rows], dst_ref.at[rows], sem).start()

    def split_heads(g):
        def job(j, r, never):
            h = 2 * (g * per_grp + j)
            low = jnp.where(never, 16, jnp.full((8, 128), 0xFFFF, _U32))
            sh = jnp.where(never, low, 16)
            for rr in range(r, r + 64, 8):
                for m in range(3):
                    even = wqkv[h, rr:rr + 8, m * dh:(m + 1) * dh]
                    odd = wqkv[h + 1, rr:rr + 8, m * dh:(m + 1) * dh]
                    wqkv[h, rr:rr + 8, m * dh:(m + 1) * dh] = (even & low) | (odd << sh)
                    wqkv[h + 1, rr:rr + 8, m * dh:(m + 1) * dh] = (
                        (even >> sh) | ((odd >> sh) << sh))
        return [functools.partial(job, j, r)
                for j in range(per_grp) for r in range(0, dm // 2, 64)]

    def q_group_copies(g):
        return (cp_xb(g), cp_bw(n_piece + 2 * g), cp_bw(n_piece + 2 * g + 1))

    for j in range(n_piece):
        cp_bw(j).start()
        cp_x0(j).start()
    zero[...] = jnp.zeros(zero.shape, _U32)

    cp_bw(0).wait()
    _permute_b_columns(bw_raw.at[0], bwq.at[0])
    for j in range(n_piece):
        cp_x0(j).wait()
        if j + 1 < n_piece:
            cp_bw(j + 1).wait()
        if j >= n_piece - 2:
            for cp in q_group_copies(j - n_piece + 2):
                cp.start()
        x = pltpu.bitcast(xb[0:q_head // 2, j * 2 * piece:(j + 1) * 2 * piece], _BF16)
        y = jnp.dot(x, pltpu.bitcast(bwq[j], _BF16), preferred_element_type=_F32)
        for c in range(8):
            part = y[:, c * 128:(c + 1) * 128]
            q_all[c, 0:q_head, :] = part if j == 0 else q_all[c, 0:q_head, :] + part
        if j + 1 < n_piece:
            _permute_b_columns(bw_raw.at[j + 1], bwq.at[j + 1])

    def q_body(g, carry):
        @pl.when(g + 2 < n_piece)
        def _():
            for cp in q_group_copies(g + 2):
                cp.start()

        @pl.when((g >= 1) & (g <= 2))
        def _():
            for cp in cp_w(g - 1):
                cp.start()

        @pl.when(g + 1 == n_piece)
        def _():
            for cp in cp_bwo + [cp_mem]:
                cp.start()

        for cp in q_group_copies(g):
            cp.wait()
        r0 = pl.multiple_of(q_head + g * q_rest, 128)
        x = pltpu.bitcast(xb[pl.ds(pl.multiple_of(r0 // 2, 64), q_rest // 2), :], _BF16)
        w = pltpu.bitcast(bwq[...].reshape(dm // 2, dm), _BF16)
        y = jnp.dot(x, w, preferred_element_type=_F32)
        for c in range(8):
            q_all[c, pl.ds(r0, q_rest), :] = y[:, c * 128:(c + 1) * 128]
        for j in (2 * g, 2 * g + 1):
            _permute_b_columns(bw_raw.at[n_piece + j], bwkv.at[j])
        return carry

    lax.fori_loop(0, n_piece, q_body, 0)

    def kv_body(g, carry):
        @pl.when(g + 2 < n_grp)
        def _():
            for cp in cp_w(g + 2):
                cp.start()

        start_a_slice(g)
        for cp in cp_w(g):
            cp.wait()
        split = split_heads(g)
        r0 = pl.multiple_of(g * _T, _T)
        for j in range(16):
            s, c = divmod(j, 8)
            x = xb[pl.ds(pl.multiple_of(r0 // 2, _T // 2), _T // 2), :]
            w = bwkv[s * n_piece:(s + 1) * n_piece, :, c * 128:(c + 1) * 128]
            y = jnp.dot(pltpu.bitcast(x, _BF16),
                        pltpu.bitcast(w.reshape(dm // 2, 128), _BF16),
                        preferred_element_type=_F32)
            (k_all, v_all)[s][c, pl.ds(_HALO + r0, _T), :] = y
            if j < 15:
                never = _never(zero, y)
                for job in split[j * len(split) // 15:(j + 1) * len(split) // 15]:
                    job(never)
        return carry

    lax.fori_loop(0, n_grp, kv_body, 0)
    for ref in (k_all, v_all):
        ref[:, 0:_HALO, :] = jnp.broadcast_to(ref[:, _HALO:_HALO + 1, :], (8, _HALO, 128))

    def b_attention(t0, n):
        q_ref = q_all.at[:, pl.ds(t0, n), :]
        k_ref = k_all.at[:, pl.ds(t0, _HALO + n), :]
        v_ref = v_all.at[:, pl.ds(t0, _HALO + n), :]
        stages = (
            lambda x, r, never: _b_lane_sum(_b_products(q_ref, k_ref, r, never), 1),
            lambda x, r, never: _b_lane_sum(x, 16),
            lambda x, r, never: _b_softmax(x, t0, r),
            lambda x, r, never: _b_values(x, v_ref, ob, r),
        )
        state = {}

        def job(stage, r, never):
            state[r] = stages[stage](state.get(r), r, never)
            return state[r][-1]

        return [functools.partial(job, s, r) for r in range(0, n, _CH) for s in range(4)]

    pltpu.make_async_copy(awo_u, awo, sems.at[2]).wait()
    pltpu.make_async_copy(ax_u, xa, sems.at[3]).wait()
    for cp in cp_bwo + [cp_mem]:
        cp.wait()

    rows = n_mem + seg
    scale = dh ** -0.5
    hbuf[0:n_mem, :] = mem_v[...].astype(_F32)

    def a_step(s, side_jobs=()):
        qi = lax.broadcasted_iota(jnp.int32, (rows, 128), 0)
        ki = lax.broadcasted_iota(jnp.int32, (rows, 128), 1)
        real = ki < rows
        mask = ((qi < n_mem) | (qi >= ki)) & real
        fill = jnp.where(real, _MASKED, -jnp.inf).astype(_F32)
        pad = jnp.zeros((128 - rows, dh), _F32)

        xs = xa[pl.ds(pl.multiple_of(s * (seg // 2), seg // 2), seg // 2), :]
        hbuf[n_mem:rows, :] = pltpu.bitcast(xs, _BF16).astype(_F32)

        def project(h, c0, c1):
            w = wqkv[h, :, c0 * dh:c1 * dh]
            return jnp.dot(hbuf[...], pltpu.bitcast(w, _BF16), preferred_element_type=_F32)

        def probs(qk, after):
            k = jnp.concatenate([qk[:, dh:2 * dh], pad], axis=0).astype(_BF16)
            sc = lax.dot_general(qk[:, 0:dh], k, _NT, preferred_element_type=_F32)
            low = fill
            if after is not None:
                low = jnp.concatenate(
                    [jnp.where(_never(zero, after), 0.0, fill[0:8])] * (rows // 8), axis=0)
            sc = jnp.where(mask, sc * scale, low)
            e = jnp.exp(sc - jnp.max(sc, axis=-1, keepdims=True))
            return e / jnp.sum(e, axis=-1, keepdims=True)

        def values(p, v):
            v = jnp.concatenate([v, pad], axis=0).astype(_BF16)
            return jnp.dot(p, v, preferred_element_type=_F32)

        def out_proj(h0, h1):
            w = pltpu.bitcast(awo[h0 * dh // 2:h1 * dh // 2, :], _BF16)
            lhs = jnp.concatenate([o[h] for h in range(h0, h1)], axis=1)
            return jnp.dot(lhs, w, preferred_element_type=_F32)

        qk, v, p, o, side = {}, {}, {}, {}, {}
        quarter = heads // (_PV_LAG + 1)
        acc = None
        for t in range(heads + _PV_LAG):
            if t < heads:
                qk[t] = project(t, 0, 2)
            if 0 <= t - _V_LAG < heads:
                v[t - _V_LAG] = project(t - _V_LAG, 2, 3)
            if t >= heads:
                part = out_proj((t - heads) * quarter, (t - heads + 1) * quarter)
                acc = part if acc is None else acc + part
            if 1 <= t <= heads:
                p[t - 1] = probs(qk[t - 1], side.get(t - 1) if t % 4 == 3 else None)
            if t >= _PV_LAG:
                o[t - _PV_LAG] = values(p[t - _PV_LAG], v[t - _PV_LAG])
            if t < heads:
                for job in side_jobs[t * len(side_jobs) // heads:
                                     (t + 1) * len(side_jobs) // heads]:
                    side[t] = job(_never(zero, qk[max(t - 1, 0)]))
        acc = acc + out_proj(_PV_LAG * quarter, heads)

        hbuf[0:n_mem, :] = acc[0:n_mem]
        res[pl.ds(pl.multiple_of(s * seg, seg), seg), 0:dm] = acc[n_mem:rows].astype(_BF16)

    def a_body(i, carry):
        toks = pl.ds(pl.multiple_of(i * 2 * seg, 2 * seg), 2 * seg)
        a_step(2 * i, b_attention(toks.start, 2 * seg))
        w = pltpu.bitcast(bwo[...].reshape(dm // 2, dm), _BF16)
        y = jnp.dot(ob[...], w, preferred_element_type=_F32)
        res[toks, dm:2 * dm] = y.astype(_BF16)
        a_step(2 * i + 1)
        pltpu.make_async_copy(res.at[toks], out_hbm.at[toks], sems.at[4]).start()
        return carry

    lax.fori_loop(0, seq // (2 * seg), a_body, 0)
    pltpu.make_async_copy(res, out_hbm, sems.at[4]).wait()


@functools.partial(jax.jit, static_argnames=("A_seg_len",))
def pallas_concat_heads__memory_aug_recurrent_mem_tr__sliding_local_dilated__prompt_kernel(
    A_x: jax.Array,
    A_mem0: jax.Array,
    A_Wq: jax.Array,
    A_Wk: jax.Array,
    A_Wv: jax.Array,
    A_Wo: jax.Array,
    A_seg_len: int,
    B_x: jax.Array,
    B_wqkv: jax.Array,
    B_wo: jax.Array,
):
    batch, seq, dm = A_x.shape
    heads, dh = A_Wq.shape[1], A_Wq.shape[2]
    n_mem = A_mem0.shape[1]
    seg = int(A_seg_len)
    assert batch == 1 and dm == 1024 and dh == 128 and heads % 8 == 0
    assert B_x.shape == (1, seq, dm) and B_wqkv.shape == (dm, 3 * dm)
    assert seg % 16 == 0 and seq % (2 * seg) == 0 and n_mem % 8 == 0 and n_mem + seg <= 128
    assert seq % _T == 0 and (heads // 2) % (seq // _T) == 0
    rows = n_mem + seg

    n_grp = seq // _T
    n_piece = 4
    piece = dm // 2 // n_piece
    assert seq % (4 * n_piece * 128) == 0
    out = pl.pallas_call(
        functools.partial(_kernel, seq=seq, seg=seg, n_mem=n_mem, heads=heads, dh=dh),
        out_shape=jax.ShapeDtypeStruct((seq, 2 * dm), _BF16),
        in_specs=[pl.BlockSpec(memory_space=pl.ANY)] * 9,
        out_specs=pl.BlockSpec(memory_space=pl.ANY),
        scratch_shapes=[
            pltpu.VMEM((seq // 2, dm), _U32),
            pltpu.VMEM((n_mem, dm), _BF16),
            pltpu.VMEM((heads, dm // 2, 3 * dh), _U32),
            pltpu.VMEM((heads * dh // 2, dm), _U32),
            pltpu.VMEM((seq // 2, dm), _U32),
            pltpu.VMEM((3 * n_piece, piece, dm), _U32),
            pltpu.VMEM((n_piece, piece, dm), _U32),
            pltpu.VMEM((2 * n_piece, piece, dm), _U32),
            pltpu.VMEM((64, 8, dm), _U32),
            pltpu.VMEM((seq, 2 * dm), _BF16),
            pltpu.VMEM((8, seq, 128), _F32),
            pltpu.VMEM((8, _HALO + seq, 128), _F32),
            pltpu.VMEM((8, _HALO + seq, 128), _F32),
            pltpu.VMEM((2 * seg, dm), _F32),
            pltpu.VMEM((rows, dm), _F32),
            pltpu.VMEM((8, 128), _U32),
            pltpu.SemaphoreType.DMA((5,)),
            pltpu.SemaphoreType.DMA((3 * n_piece,)),
            pltpu.SemaphoreType.DMA((n_piece,)),
            pltpu.SemaphoreType.DMA((n_grp,)),
            pltpu.SemaphoreType.DMA((n_piece,)),
        ],
        compiler_params=pltpu.CompilerParams(vmem_limit_bytes=110 * 1024 * 1024),
    )(
        A_x.reshape(seq, dm),
        A_mem0.reshape(n_mem, dm),
        A_Wq.reshape(dm // 2, 2 * heads, dh),
        A_Wk.reshape(dm // 2, 2 * heads, dh),
        A_Wv.reshape(dm // 2, 2 * heads, dh),
        A_Wo.reshape(heads * dh, dm),
        B_x.reshape(seq, dm),
        B_wqkv,
        B_wo.reshape(8, dm // 8, dm),
    )
    return out.reshape(1, seq, 2 * dm)
```
